```python
import jax
import jax.numpy as jnp

def _softmax(x, axis=-1):
    return jax.nn.softmax(x, axis=axis)
def _gelu(x):
    return jax.nn.gelu(x, approximate=True)
def _silu(x):
    return jax.nn.silu(x)
def _sigmoid(x):
    return jax.nn.sigmoid(x)
def _layernorm(x, axis=-1, eps=1e-5):
    m = jnp.mean(x, axis=axis, keepdims=True)
    v = jnp.var(x, axis=axis, keepdims=True)
    return (x - m) / jnp.sqrt(v + eps)
def _scatter_add(tgt, idx, src, axis=0):
    return tgt.at[idx].add(src)
def _segment_sum(src, seg, n):
    return jax.ops.segment_sum(src, seg, n)
class _Rng:
    def __init__(self, key):
        self._k = key
    def _next(self):
        self._k, sub = jax.random.split(self._k)
        return sub
    def normal(self, shape):
        return jax.random.normal(self._next(), shape, dtype=jnp.bfloat16)
    def randint(self, lo, hi, shape):
        return jax.random.randint(self._next(), shape, lo, hi, dtype=jnp.int32)
    def uniform(self, shape, lo=0.0, hi=1.0):
        return jax.random.uniform(self._next(), shape, jnp.bfloat16, lo, hi)
    def permutation(self, n):
        return jax.random.permutation(self._next(), n)


kernel_name = 'standalone__dcn_v2_cross__recsys'

def setup_inputs():
    _rng = _Rng(jax.random.key(int.from_bytes(__import__("os").urandom(4), "little")))
    _w = (lambda a: (lambda t: t.astype(jnp.bfloat16) if jnp.issubdtype(t.dtype, jnp.floating) else t)(jnp.asarray(a)))
    B, F, D, L = 16384, 26, 128, 6
    Din = min(F * D, 1024)
    return {
        "x0": _w((lambda *s: _rng.normal(s) * 0.05)(B, Din)),
        "ws": _w((lambda *s: _rng.normal(s) * 0.05)(L, Din, Din)),
        "bs": _w((lambda *s: _rng.normal(s) * 0.05)(L, Din)),
    }

def reference(x0, ws, bs):
    x = x0
    for l in range(ws.shape[0]):
        x = x0 * (x @ ws[l] + bs[l]) + x
    return x
```

```python
import functools

import jax
import jax.numpy as jnp
import jax.experimental.pallas as pl
import jax.experimental.pallas.tpu as pltpu


def _kernel(x0_ref, w_ref, b_ref, o_ref, *, num_layers):
    x0 = x0_ref[...].astype(jnp.float32)
    x = x0
    xb = x0_ref[...]
    for l in range(num_layers):
        y = jnp.dot(xb, w_ref[l], preferred_element_type=jnp.float32)
        y = y + b_ref[l].astype(jnp.float32)
        x = x0 * y + x
        xb = x.astype(jnp.bfloat16)
    o_ref[...] = xb


@jax.jit
def pallas_standalone__dcn_v2_cross__recsys_kernel(
    x0: jax.Array,
    ws: jax.Array,
    bs: jax.Array,
):
    B, D = x0.shape
    L = ws.shape[0]
    TM = 512
    bs3 = bs.reshape(L, 1, D)
    return pl.pallas_call(
        functools.partial(_kernel, num_layers=L),
        grid=(B // TM,),
        in_specs=[
            pl.BlockSpec((TM, D), lambda i: (i, 0)),
            pl.BlockSpec((L, D, D), lambda i: (0, 0, 0)),
            pl.BlockSpec((L, 1, D), lambda i: (0, 0, 0)),
        ],
        out_specs=pl.BlockSpec((TM, D), lambda i: (i, 0)),
        out_shape=jax.ShapeDtypeStruct((B, D), x0.dtype),
        compiler_params=pltpu.CompilerParams(
            dimension_semantics=("arbitrary",),
            vmem_limit_bytes=100 * 1024 * 1024,
        ),
    )(x0, ws, bs3)
```

```python
import functools
import itertools
import jax
import jax.numpy as jnp
import jax.experimental.pallas as pl
import jax.experimental.pallas.tpu as pltpu

F32 = jnp.float32
BF16 = jnp.bfloat16

S1 = [1.0, 0.5, 2.0, 1.0]
LAM = [[(1, 0)], [(1, 1)], [(1, 0), (-1, 2)], [(1, 2), (-1, 1)], [(1, 2)], [(1, 2), (1, 3)], [(1, 3), (-1, 2)]]


def fwd(a, g, h, d):
    return [a + g, a - g, a + d, g + h]


def inv(u, v, e, f):
    a = (u + v) * 0.5
    g = (u - v) * 0.5
    return [a, g, f - g, e - a]


def rhs7(u, v, e, f):
    return [v - e, u - e, e + f, f - e, e + e, v, u]


class Q:
    def __init__(self, qs):
        self.q = list(qs)
    def __add__(self, o):
        return Q(a + b for a, b in zip(self.q, o.q))
    def __sub__(self, o):
        return Q(a - b for a, b in zip(self.q, o.q))
    def __mul__(self, s):
        return Q(a * s for a in self.q)


def scl(x, s):
    return x if s == 1.0 else x * s


def rc(Qd, q):
    return 2 * (Qd // 2) + q // 2, 2 * (Qd % 2) + q % 2


def t_orders():
    used = set()
    terms = {(i, j): [(s1 * s2, (a, b)) for s1, a in LAM[i] for s2, b in LAM[j]] for i in range(7) for j in range(7)}
    out = {}
    for k, t in sorted(terms.items(), key=lambda kv: len(kv[1])):
        for perm in itertools.permutations(t):
            if perm[0][0] < 0:
                continue
            pre = [frozenset(perm[:n]) for n in range(2, len(perm) + 1)]
            if not any(p in used for p in pre):
                used.update(pre)
                out[k] = perm
                break
        else:
            raise AssertionError(k)
    return out
T_ORD = t_orders()


def _kernel(x0_hbm, w_hbm, b_hbm, o_hbm,
            wbuf, s_ref, m_ref, xin, ost, sp_z, sp_x, sp_b, bvm, bt_ref,
            sem_w, sem_in, sem_out, sem_misc,
            *, L, tm, d, ntiles, r0, wins, wins_last, pfrac, pshift):
    d4 = d // 4
    r4 = tm // 4
    H = tm // 2
    nc = d4 // 128
    N = ntiles
    ids = {}
    for nm in ([("C21", k) for k in range(7)] + [("C22", k) for k in range(7)]
               + [("X", a, (L - 1) % 2, k) for a in range(4) for k in range(4)]
               + [("z", Qd, k) for Qd in (2, 3) for k in range(4)]):
        ids[nm] = len(ids)
    nzero = len(ids)

    def put(name, v):
        i = ids.setdefault(name, len(ids))
        for c in range(nc):
            m_ref[i, c * r4:(c + 1) * r4, :] = v[:, c * 128:(c + 1) * 128]

    def get(name):
        i = ids.setdefault(name, len(ids))
        return jnp.concatenate([m_ref[i, c * r4:(c + 1) * r4, :] for c in range(nc)], axis=1)

    def putq(name, vs):
        for k, v in enumerate(vs):
            put(name + (k,), v)

    def getq(name, n=4):
        return Q(get(name + (k,)) for k in range(n))

    dot = functools.partial(jnp.dot, preferred_element_type=F32)

    def slio(Qd, q):
        r, cc = rc(Qd, q)
        r = (r + 2) % 4
        return (slice(r * r4, (r + 1) * r4), slice(cc * d4, (cc + 1) * d4))

    CN = {0: "E", 1: "F", 2: "C21", 3: "C22"}

    def delta(l, Qd, gate):
        c = [get((CN[Qd], k)) for k in range(7)]
        for k in (1, 5, 6):
            c[k] = gate(c[k])
        f = c[1] - c[0]
        e = c[1] + c[0] + c[2] + c[3] + c[4]
        v = c[5] + c[3]
        u = c[6] - c[2]
        y = [e, f, u + v + f, u - v + e]
        return [get(("z", Qd, q)) * (y[q] + bt_ref[l, 4 * Qd + q, 0:1, :]) for q in range(4)]

    def fin(Qd, gate, slot):
        par = (L - 1) % 2
        D = delta(L - 1, Qd, gate)
        xu = Q(gate(x) for x in getq(("X", 0, par)).q)
        xv = getq(("X", 1, par))
        t = ((xu + xv) if Qd in (0, 3) else (xu - xv)) * 0.5
        if Qd == 3:
            t = getq(("X", 2, par)) - t
        if Qd == 2:
            t = getq(("X", 3, par)) - t
        xs = inv(*t.q)
        for q in range(4):
            ost[(slot,) + slio(Qd, q)] = scl(xs[q] + D[q], 1.0 / (S1[Qd] * S1[q])).astype(ost.dtype)

    def start(Qd, gate, slot):
        zs = [gate(xin[(slot,) + slio(Qd, q)].astype(F32)) for q in range(4)]
        putq(("z", Qd), zs)
        return Q(fwd(*[scl(zs[q], S1[Qd] * S1[q]) for q in range(4)]))

    def update(l, Qd, gate, slot, do_fin=True):
        last = l == L - 1
        par, npar = l % 2, (l + 1) % 2
        if last:
            if do_fin:
                fin(Qd, gate, slot)
            Dn = start(Qd, gate, slot)
        else:
            Dn = Q(fwd(*delta(l, Qd, gate)))
        old = (lambda a, t: t) if last else (lambda a, t: t + getq(("X", a, par)))
        if Qd == 1:
            putq(("D12", par), Dn.q)
        elif Qd == 0:
            D12 = getq(("D12", par))
            putq(("X", 0, npar), (old(0, Dn) + D12).q)
            putq(("X", 1, npar), (old(1, Dn) - D12).q)
            putq(("D11", par), Dn.q)
        elif Qd == 3:
            putq(("X", 2, npar), (old(2, Dn) + getq(("D11", par))).q)
        else:
            putq(("X", 3, npar), (old(3, Dn) + getq(("D12", par))).q)

    ident = lambda x: x

    def w_copy(l, slot):
        return pltpu.make_async_copy(w_hbm.at[l], wbuf.at[slot], sem_w.at[slot])

    def in_bot(s, slot):
        return pltpu.make_async_copy(x0_hbm.at[pl.ds(pl.multiple_of(s * tm + H, 16), H)], xin.at[slot, pl.ds(0, H)], sem_in.at[slot, 0])

    def in_top(s, slot):
        return pltpu.make_async_copy(x0_hbm.at[pl.ds(pl.multiple_of(s * tm, 16), H)], xin.at[slot, pl.ds(H, H)], sem_in.at[slot, 1])

    def out_bot(s, slot):
        return pltpu.make_async_copy(ost.at[slot, pl.ds(0, H)], o_hbm.at[pl.ds(pl.multiple_of(s * tm + H, 16), H)], sem_out.at[slot, 0])

    def out_top(s, slot):
        return pltpu.make_async_copy(ost.at[slot, pl.ds(H, H)], o_hbm.at[pl.ds(pl.multiple_of(s * tm, 16), H)], sem_out.at[slot, 1])

    sp_in = pltpu.make_async_copy(x0_hbm.at[pl.ds(N * tm, r0)], sp_b, sem_misc.at[0])
    sp_out = pltpu.make_async_copy(sp_b, o_hbm.at[pl.ds(N * tm, r0)], sem_misc.at[0])
    b_in = pltpu.make_async_copy(b_hbm, bvm, sem_misc.at[1])

    b_in.start()
    sp_in.start()
    w_copy(0, 0).start()

    def zero(i, c):
        m_ref[i] = jnp.zeros(m_ref.shape[1:], F32)
        return c
    jax.lax.fori_loop(0, nzero, zero, 0)

    b_in.wait()
    ball = bvm[...].astype(F32)
    for l in range(L):
        for Qd in range(4):
            for q in range(4):
                cc = rc(Qd, q)[1]
                row = scl(ball[l:l + 1, cc * d4:(cc + 1) * d4], S1[Qd] * S1[q])
                bt_ref[l, 4 * Qd + q] = jnp.broadcast_to(row, (8, d4))
    sp_in.wait()
    z0 = sp_b[...].astype(F32)
    sp_z[...] = z0
    sp_x[...] = z0

    def layer_body(l, c):
        slot = l % 2
        w_copy(l, slot).wait()

        @pl.when(l + 1 < L)
        def _():
            w_copy(l + 1, 1 - slot).start()

        @pl.when(l + 1 == L)
        def _():
            in_top(0, 1).start()
            in_bot(0, 0).start()
            in_top(min(1, N - 1), 0).start()

        never = jnp.full((16, 128), l, jnp.int32) < 0
        xb = sp_b[...]
        trig = []
        news = []
        for n in range(d // 128):
            cs = slice(n * 128, (n + 1) * 128)
            cb = n * 128 // d4
            Qd, q = 3 * (cb // 2), 3 * (cb % 2)
            off = n * 128 - cb * d4
            y1 = dot(xb[:, :d // 2], wbuf[slot, :d // 2, cs]) + bt_ref[l, 4 * Qd + q, 0:1, off:off + 128]
            y2 = dot(xb[:, d // 2:], wbuf[slot, d // 2:, cs]) + y1
            trig += [y[k * 16:(k + 1) * 16] for y in (y1, y2) for k in range(r0 // 16)]
            news.append(sp_z[:, cs] * y2 + sp_x[:, cs])
        for n in range(d // 128):
            cs = slice(n * 128, (n + 1) * 128)
            sp_x[:, cs] = news[n]
            sp_b[:, cs] = news[n].astype(BF16)

        nch = (d4 // 16) * nc
        for ch in range(nch):
            rr, h = (ch // nc) * 16, ch % nc
            per = len(trig) // nch

            def blk(Qd, q):
                ti = (ch - 1) * per + (pfrac[Qd] * per) // 8 + pshift
                r, cb = rc(Qd, q)
                w = wbuf[slot, r * d4 + rr:r * d4 + rr + 16, cb * d4 + h * 128:cb * d4 + (h + 1) * 128].astype(F32)
                if q < 2 and ti >= 0:
                    w = jnp.where(never, trig[ti], w)
                return scl(w, 0.25 * S1[Qd] * S1[q])
            bb = fwd(*[Q(fwd(*[blk(Qd, q) for q in range(4)])) for Qd in range(4)])
            for i, t in enumerate(rhs7(*bb)):
                for j, u in enumerate(rhs7(*t.q)):
                    s_ref[l, i * 7 + j, h, rr:rr + 16, :] = u.astype(BF16)
        return c
    jax.lax.fori_loop(0, L, layer_body, 0)

    sp_out.start()
    in_top(0, 1).wait()
    update(L - 1, 1, ident, 1, do_fin=False)
    update(L - 1, 0, ident, 1, do_fin=False)

    def tile_body(s, carry):
        slot = s % 2
        in_bot(0, slot).wait()
        in_top(0, slot).wait()
        in_bot(jnp.minimum(s + 1, N - 1), 1 - slot).start()
        in_top(jnp.minimum(s + 2, N - 1), 1 - slot).start()

        never = jnp.full((r4, d4), s, jnp.int32) < 0
        s_u32 = s_ref.bitcast(jnp.uint32)
        allp = []

        def gate_on(lo, hi):
            prods = allp[lo:hi]
            assert len(prods) == hi - lo
            nr = r4 // 8
            n = nr * nc
            rows = []
            for r in range(nr):
                cols = []
                for c in range(nc):
                    pos = (r * nc + c) * len(prods)
                    k, rem = pos // n, pos % n
                    rr, cc = rem // nc, rem % nc
                    cols.append(prods[k][rr * 8:(rr + 1) * 8, cc * 128:(cc + 1) * 128])
                rows.append(jnp.concatenate(cols, axis=1))
            trig = jnp.concatenate(rows, axis=0)
            return lambda x: jnp.where(never, trig, x)

        for l in range(L):
            base = 49 * l
            par = l % 2
            pl_ = (l - 1) % L

            def outer(i):
                for j in range(7):
                    terms = T_ORD[i, j]
                    t = get(("X", terms[0][1][0], par, terms[0][1][1]))
                    for sg, (a, b) in terms[1:]:
                        x = get(("X", a, par, b))
                        t = t + x if sg > 0 else t - x
                    w = pltpu.bitcast(jnp.concatenate([s_u32[l, i * 7 + j, h] for h in range(nc)], axis=1), BF16)
                    p = dot(t.astype(BF16), w)
                    allp.append(p)
                    if i == 0:
                        put(("P0", j), p)
                    elif i == 1:
                        p0 = get(("P0", j))
                        put(("F", j), p - p0)
                        put(("G", j), p + p0)
                    elif i in (2, 3):
                        put(("P%d" % i, j), p)
                    elif i == 4:
                        put(("E", j), p + get(("G", j)) + get(("P2", j)) + get(("P3", j)))
                    elif i == 5:
                        put(("V", j), p + get(("P3", j)))
                    else:
                        u = p - get(("P2", j))
                        v = get(("V", j))
                        put(("C21", j), u + v + get(("F", j)))
                        put(("C22", j), u - v + get(("E", j)))

            def win(k, lay):
                ww = wins_last if lay == L - 1 else wins
                return gate_on(base + ww[k][0], base + ww[k][1])

            outer(0)
            outer(1)
            update(pl_, 3, win(2, pl_), slot)
            outer(2)
            outer(3)
            outer(4)
            update(pl_, 2, win(3, pl_), slot)
            update(l, 1, win(0, l), slot)
            outer(5)
            outer(6)
            update(l, 0, win(1, l), slot)

        @pl.when(s > 0)
        def _():
            out_top(0, 1 - slot).wait()
            out_bot(s - 1, slot).start()

        @pl.when(s > 1)
        def _():
            out_bot(0, 1 - slot).wait()

        out_top(s, slot).start()
        return carry
    jax.lax.fori_loop(0, N, tile_body, 0)

    slot = N % 2
    fin(3, ident, slot)
    fin(2, ident, slot)
    out_bot(N - 1, slot).start()
    in_bot(0, slot).wait()
    in_top(0, slot).wait()
    sp_out.wait()
    out_top(0, 1 - slot).wait()
    if N > 1:
        out_bot(0, 1 - slot).wait()
    out_bot(0, slot).wait()
    assert len(ids) <= m_ref.shape[0], len(ids)


W0 = ((24, 34), (35, 47), (0, 12), (12, 24))


@jax.jit
def pallas_standalone__dcn_v2_cross__recsys_kernel(x0: jax.Array, ws: jax.Array, bs: jax.Array):
    TM, R0, pad = 576, 256, 1
    B, D = x0.shape
    L = ws.shape[0]
    N = (B - R0) // TM
    assert R0 + N * TM == B and L % 2 == 0
    return pl.pallas_call(
        functools.partial(_kernel, L=L, tm=TM, d=D, ntiles=N, r0=R0, wins=W0, wins_last=W0,
                          pfrac=(0, 1, 6, 3), pshift=0),
        in_specs=[pl.BlockSpec(memory_space=pl.ANY)] * 3,
        out_specs=pl.BlockSpec(memory_space=pl.ANY),
        out_shape=jax.ShapeDtypeStruct((B, D), x0.dtype),
        scratch_shapes=[
            pltpu.VMEM((2, D, D), BF16),
            pltpu.VMEM((L, 49, D // 512, D // 4, 128), BF16),
            pltpu.VMEM((128, TM // 4 * (D // 512) + 8 * pad, 128), F32),
            pltpu.VMEM((2, TM, D), BF16),
            pltpu.VMEM((2, TM, D), BF16),
            pltpu.VMEM((R0, D), F32),
            pltpu.VMEM((R0, D), F32),
            pltpu.VMEM((R0, D), BF16),
            pltpu.VMEM((L, D), BF16),
            pltpu.VMEM((L, 16, 8, D // 4), F32),
            pltpu.SemaphoreType.DMA((2,)),
            pltpu.SemaphoreType.DMA((2, 2)),
            pltpu.SemaphoreType.DMA((2, 2)),
            pltpu.SemaphoreType.DMA((2,)),
        ],
        compiler_params=pltpu.CompilerParams(vmem_limit_bytes=120 * 1024 * 1024),
    )(x0, ws, bs)
```

```python
import functools

import jax
import jax.numpy as jnp
import jax.experimental.pallas as pl
import jax.experimental.pallas.tpu as pltpu

F32 = jnp.float32
BF16 = jnp.bfloat16
LANES = 128

_SCALE = (1.0, 0.5, 2.0, 1.0)
_LHS = (((1, 0),), ((1, 1),), ((1, 0), (-1, 2)), ((1, 2), (-1, 1)), ((1, 2),),
        ((1, 2), (1, 3)), ((1, 3), (-1, 2)))


def _fwd(a, g, h, d):
    return [a + g, a - g, a + d, g + h]


def _inv(u, v, e, f):
    a = (u + v) * 0.5
    g = (u - v) * 0.5
    return [a, g, f - g, e - a]


def _rhs7(u, v, e, f):
    return [v - e, u - e, e + f, f - e, e + e, v, u]


def _lin(terms, fetch):
    t = fetch(terms[0][1])
    for sign, k in terms[1:]:
        t = t + fetch(k) if sign > 0 else t - fetch(k)
    return t


class _Q:
    def __init__(self, blocks):
        self.q = list(blocks)

    def __add__(self, o):
        return _Q(a + b for a, b in zip(self.q, o.q))

    def __sub__(self, o):
        return _Q(a - b for a, b in zip(self.q, o.q))

    def __mul__(self, s):
        return _Q(a * s for a in self.q)


def _scl(x, s):
    return x if s == 1.0 else x * s


def _rc(Q, q):
    return 2 * (Q // 2) + q // 2, 2 * (Q % 2) + q % 2


def _ident(x):
    return x


def _kernel(x0_hbm, w_hbm, b_hbm, o_hbm,
            wbuf, s_ref, m_ref, xin, ost, sp_z, sp_x, sp_b, bvm, bt_ref,
            sem_w, sem_in, sem_out, sem_misc,
            *, L, tm, d, ntiles, r0, wins, shifts, xwin, pfrac, pshift, ngroups):
    d4 = d // 4
    r4 = tm // 4
    half = tm // 2
    nc = d4 // LANES
    N = ntiles
    dot = functools.partial(jnp.dot, preferred_element_type=F32)

    def ver(l):
        return "A" if l % L == 0 else "BC"[l % 2]

    ids = {}
    for name in ([(n, k) for n in "UV" for k in range(7)]
                 + [("Y", Q, (L - 1) % 2, k) for Q in (0, 1) for k in range(4)]
                 + [("X", a, ver(L - 1), k) for a in range(4) for k in range(4)]
                 + [("z", Q, k) for Q in (2, 3) for k in range(4)]):
        ids[name] = len(ids)
    nzero = len(ids)

    rw = [0, r4]

    def rows(base):
        if isinstance(rw[0], int):
            return slice(base + rw[0], base + rw[0] + rw[1])
        return pl.ds(pl.multiple_of(base + rw[0], 8), rw[1])

    def chunked(fn, lo, n):
        def body(k, c):
            rw[:] = [lo + k * 8, 8]
            fn()
            rw[:] = [0, r4]
            return c
        jax.lax.fori_loop(0, n // 8, body, 0)

    def put(name, v):
        i = ids.setdefault(name, len(ids))
        for c in range(nc):
            m_ref[i, rows(c * r4), :] = v[:, c * LANES:(c + 1) * LANES]

    def get(name):
        i = ids.setdefault(name, len(ids))
        return jnp.concatenate([m_ref[i, rows(c * r4), :] for c in range(nc)], axis=1)

    def putq(name, q):
        for k, v in enumerate(q.q):
            put(name + (k,), v)

    def getq(name):
        return _Q(get(name + (k,)) for k in range(4))

    def sl(Q, q):
        r, c = _rc(Q, q)
        return (rows(r * r4), slice(c * d4, (c + 1) * d4))

    def delta(l, Q, gate):
        par = l % 2
        c = []
        for k in range(7):
            t = get(("EFUU"[Q], k))
            if k in (1, 5, 6):
                t = gate(t)
            if Q >= 2:
                t = t + get(("V", k)) if Q == 2 else t - get(("V", k))
            c.append(t)
        f = c[1] - c[0]
        e = c[1] + c[0] + c[2] + c[3] + c[4]
        v = c[5] + c[3]
        u = c[6] - c[2]
        y = _Q([e, f, u + v + f, u - v + e])
        if Q < 2:
            putq(("Y", Q, par), y)
        else:
            y = y + getq(("Y", 3 - Q, par))
        return [get(("z", Q, q)) * (y.q[q] + bt_ref[l, 4 * Q + q, 0:1, :]) for q in range(4)]

    def finish(Q, gate, oslot):
        vr = ver(L - 1)
        dq = delta(L - 1, Q, gate)
        xu = _Q(gate(x) for x in getq(("X", 0, vr)).q)
        xv = getq(("X", 1, vr))
        t = ((xu + xv) if Q in (0, 3) else (xu - xv)) * 0.5
        if Q >= 2:
            t = getq(("X", 5 - Q, vr)) - t
        xs = _inv(*t.q)
        o = [_scl(xs[q] + dq[q], 1.0 / (_SCALE[Q] * _SCALE[q])) for q in range(4)]
        for q in range(4):
            ost[(oslot,) + sl(Q, q)] = o[q].astype(ost.dtype)
        return o

    def load_z(Q, gates, islot):
        putq(("z", Q), _Q(gates[q](xin[(islot,) + sl(Q, q)].astype(F32)) for q in range(4)))

    def init_x(gates, islot):
        def blk(Q, q):
            x = xin[(islot,) + sl(Q, q)].astype(F32)
            if q < 2:
                x = gates[Q](x)
            return _scl(x, _SCALE[Q] * _SCALE[q])
        x = _fwd(*[_Q(_fwd(*[blk(Q, q) for q in range(4)])) for Q in range(4)])
        for a in range(4):
            putq(("X", a, ver(0)), x[a])

    def update(l, Q, gate, oslot, islot, never):
        if l == L - 1:
            o = finish(Q, gate, oslot)
            load_z(Q, [lambda x, t=t: jnp.where(never, t, x) for t in o], islot)
            return
        par, vo, vn = l % 2, ver(l), ver(l + 1)
        dn = _Q(_fwd(*delta(l, Q, gate)))
        if Q < 2:
            putq(("D", Q, par), dn)
        if Q != 1:
            a = (0, None, 3, 2)[Q]
            putq(("X", a, vn), dn + getq(("X", a, vo)) + getq(("D", (1, None, 1, 0)[Q], par)))

    def update_v(l, gate):
        par, vo, vn = l % 2, ver(l), ver(l + 1)
        d11 = _Q(gate(x) for x in getq(("D", 0, par)).q)
        putq(("X", 1, vn), d11 + getq(("X", 1, vo)) - getq(("D", 1, par)))

    def w_copy(l):
        return pltpu.make_async_copy(w_hbm.at[l], wbuf.at[l], sem_w.at[l])

    def in_copy(t, slot):
        return pltpu.make_async_copy(
            x0_hbm.at[pl.ds(pl.multiple_of(t * tm, 16), tm)], xin.at[slot], sem_in.at[slot])

    def out_copy(t, slot, lo=0, n=tm):
        return pltpu.make_async_copy(
            ost.at[slot, pl.ds(lo, n)],
            o_hbm.at[pl.ds(pl.multiple_of(t * tm + lo, 16), n)], sem_out)

    sp_in = pltpu.make_async_copy(x0_hbm.at[pl.ds(N * tm, r0)], sp_b, sem_misc.at[0])
    sp_out = pltpu.make_async_copy(sp_b, o_hbm.at[pl.ds(N * tm, r0)], sem_misc.at[0])
    b_in = pltpu.make_async_copy(b_hbm, bvm, sem_misc.at[1])

    b_in.start()
    sp_in.start()

    def w_start(l, c):
        w_copy(l).start()
        return c
    jax.lax.fori_loop(0, L, w_start, 0)
    in_copy(0, 0).start()

    def zero(i, c):
        m_ref[i] = jnp.zeros(m_ref.shape[1:], F32)
        return c
    jax.lax.fori_loop(0, nzero, zero, 0)
    in_copy(min(1, N - 1), 1).start()

    b_in.wait()
    ball = bvm[...].astype(F32)
    for l in range(L):
        for Q in range(4):
            for q in range(4):
                c = _rc(Q, q)[1]
                row = _scl(ball[l:l + 1, c * d4:(c + 1) * d4], _SCALE[Q] * _SCALE[q])
                bt_ref[l, 4 * Q + q] = jnp.broadcast_to(row, (8, d4))
    sp_in.wait()
    z0 = sp_b[...].astype(F32)
    sp_z[...] = z0
    sp_x[...] = z0

    def layer_body(l, carry):
        w_copy(l).wait()
        never = jnp.full((16, LANES), l, jnp.int32) < 0
        xb = sp_b[...]
        trig, new = [], []
        for n in range(d // LANES):
            cs = slice(n * LANES, (n + 1) * LANES)
            cb, off = divmod(n * LANES, d4)
            unscaled = 4 * 3 * (cb // 2) + 3 * (cb % 2)
            y1 = dot(xb[:, :d // 2], wbuf[l, :d // 2, cs]) + bt_ref[l, unscaled, 0:1, off:off + LANES]
            y2 = dot(xb[:, d // 2:], wbuf[l, d // 2:, cs]) + y1
            trig += [y[k * 16:(k + 1) * 16] for y in (y1, y2) for k in range(r0 // 16)]
            new.append(sp_z[:, cs] * y2 + sp_x[:, cs])
        for n in range(d // LANES):
            cs = slice(n * LANES, (n + 1) * LANES)
            sp_x[:, cs] = new[n]
            sp_b[:, cs] = new[n].astype(BF16)

        nch = (d4 // 16) * nc
        per = len(trig) // nch
        for ch in range(nch):
            rr, h = (ch // nc) * 16, ch % nc

            def blk(Q, q):
                r, c = _rc(Q, q)
                c0 = c * d4 + h * LANES
                w = wbuf[l, r * d4 + rr:r * d4 + rr + 16, c0:c0 + LANES].astype(F32)
                ti = ch * per + (pfrac[Q] * per) // 8 + pshift
                if q < 2 and ti >= 0:
                    w = jnp.where(never, trig[ti], w)
                return _scl(w, 0.25 * _SCALE[Q] * _SCALE[q])
            wt = _fwd(*[_Q(_fwd(*[blk(Q, q) for q in range(4)])) for Q in range(4)])
            for i, t in enumerate(_rhs7(*wt)):
                for j, u in enumerate(_rhs7(*t.q)):
                    s_ref[l, i * 7 + j, h, rr:rr + 16, :] = u.astype(BF16)
        return carry
    jax.lax.fori_loop(0, L, layer_body, 0)

    sp_out.start()
    in_copy(0, 0).wait()

    def first():
        init_x([_ident] * 4, 0)
        load_z(0, [_ident] * 4, 0)
        load_z(1, [_ident] * 4, 0)
    chunked(first, 0, r4)

    def tile_body(s, slots):
        cur, nxt, fre = slots
        in_copy(0, nxt).wait()
        in_copy(jnp.minimum(s + 2, N - 1), fre).start()
        oslot = s & 1
        never = jnp.full((r4, d4), s, jnp.int32) < 0
        s_u32 = s_ref.bitcast(jnp.uint32)
        prods = []

        def gate_on(lo, hi, shift):
            n = (r4 // 8) * nc
            parts = []
            for r in range(r4 // 8):
                cols = []
                for c in range(nc):
                    k, rem = divmod((r * nc + c) * (hi - lo) + shift, n)
                    rr, cc = divmod(rem, nc)
                    cols.append(prods[lo + k][rr * 8:(rr + 1) * 8, cc * LANES:(cc + 1) * LANES])
                parts.append(jnp.concatenate(cols, axis=1))
            trig = jnp.concatenate(parts, axis=0)
            return lambda x: jnp.where(never, trig, x)

        for l in range(L):
            lp = (l - 1) % L

            def outer(i):
                for j in range(7):
                    t = _lin(_LHS[j], lambda b: _lin(_LHS[i], lambda a: get(("X", a, ver(l), b))))
                    w = jnp.concatenate([s_u32[l, i * 7 + j, h] for h in range(nc)], axis=1)
                    p = dot(t.astype(BF16), pltpu.bitcast(w, BF16))
                    prods.append(p)
                    if i in (0, 2, 3):
                        put(("P", i, j), p)
                    elif i == 1:
                        p0 = get(("P", 0, j))
                        put(("F", j), p - p0)
                        put(("G", j), p + p0)
                    elif i == 4:
                        put(("E", j), p + get(("G", j)) + get(("P", 2, j)) + get(("P", 3, j)))
                    elif i == 5:
                        put(("V", j), p + get(("P", 3, j)))
                    else:
                        put(("U", j), p - get(("P", 2, j)))

            def win(k):
                return gate_on(49 * l + wins[k][0], 49 * l + wins[k][1], shifts[k])

            outer(0)
            if l > 0:
                update_v(lp, win(4))
            outer(1)
            update(lp, 3, win(3), 1 - oslot, cur, never)
            outer(2)
            outer(3)
            outer(4)
            update(lp, 2, win(2), 1 - oslot, cur, never)
            update(l, 1, win(1), oslot, nxt, never)
            outer(5)
            outer(6)
            update(l, 0, win(0), oslot, nxt, never)
            if l == 0:
                @pl.when(s > 0)
                def _():
                    out_copy(s - 1, 1 - oslot).start()
            if l == L - 2:
                init_x([gate_on(xwin[0], xwin[1], sh) for sh in xwin[2]], nxt)

        @pl.when(s > 0)
        def _():
            out_copy(0, 0).wait()
        return nxt, fre, cur
    jax.lax.fori_loop(0, N, tile_body, (0, 1, 2))

    oslot = (N - 1) % 2
    out_copy(N - 1, oslot, 0, half).start()
    gr = r4 // ngroups

    def last():
        finish(3, _ident, oslot)
        finish(2, _ident, oslot)

    def group(g, carry):
        lo = pl.multiple_of(g * gr, 16)
        chunked(last, lo, gr)
        for rb in (2, 3):
            out_copy(N - 1, oslot, pl.multiple_of(rb * r4 + lo, 16), gr).start()
        return carry
    jax.lax.fori_loop(0, ngroups, group, 0)
    in_copy(0, (N + 1) % 3).wait()
    sp_out.wait()
    out_copy(0, 0).wait()
    assert len(ids) <= m_ref.shape[0]


def _build(x0, ws, bs, *, TM=576, R0=256, pad=1, ngroups=3, nobc=False,
           wins=((35, 47), (24, 34), (12, 24), (4, 12), (0, 4)), shifts=(1, 1, 1, 1, 1),
           xwin=(98, 242, (0, 4, 12, 8)), pfrac=(0, 1, 6, 3), pshift=0):
    B, D = x0.shape
    L = ws.shape[0]
    N = (B - R0) // TM
    assert R0 + N * TM == B and L % 2 == 0 and L >= 6 and D % (4 * LANES) == 0
    assert TM % (64 * ngroups) == 0 and R0 % 16 == 0
    nc = D // (4 * LANES)
    return pl.pallas_call(
        functools.partial(_kernel, L=L, tm=TM, d=D, ntiles=N, r0=R0, wins=wins, shifts=shifts,
                          xwin=xwin, pfrac=pfrac, pshift=pshift, ngroups=ngroups),
        in_specs=[pl.BlockSpec(memory_space=pl.ANY)] * 3,
        out_specs=pl.BlockSpec(memory_space=pl.ANY),
        out_shape=jax.ShapeDtypeStruct((B, D), x0.dtype),
        scratch_shapes=[
            pltpu.VMEM((L, D, D), BF16),
            pltpu.VMEM((L, 49, nc, D // 4, LANES), BF16),
            pltpu.VMEM((152, TM // 4 * nc + 8 * pad, LANES), F32),
            pltpu.VMEM((3, TM, D), BF16),
            pltpu.VMEM((2, TM, D), BF16),
            pltpu.VMEM((R0, D), F32),
            pltpu.VMEM((R0, D), F32),
            pltpu.VMEM((R0, D), BF16),
            pltpu.VMEM((L, D), BF16),
            pltpu.VMEM((L, 16, 8, D // 4), F32),
            pltpu.SemaphoreType.DMA((L,)),
            pltpu.SemaphoreType.DMA((3,)),
            pltpu.SemaphoreType.DMA,
            pltpu.SemaphoreType.DMA((2,)),
        ],
        compiler_params=pltpu.CompilerParams(
            vmem_limit_bytes=120 * 1024 * 1024,
            disable_bounds_checks=nobc,
        ),
    )(x0, ws, bs)


@jax.jit
def pallas_standalone__dcn_v2_cross__recsys_kernel(
    x0: jax.Array,
    ws: jax.Array,
    bs: jax.Array,
):
    return _build(x0, ws, bs)
```

```python
import functools

import jax
import jax.numpy as jnp
import jax.experimental.pallas as pl
import jax.experimental.pallas.tpu as pltpu

F32 = jnp.float32
BF16 = jnp.bfloat16
LANES = 128

_SCALE = (1.0, 0.5, 2.0, 1.0)
_LHS = (((1, 0),), ((1, 1),), ((1, 0), (-1, 2)), ((1, 2), (-1, 1)), ((1, 2),),
        ((1, 2), (1, 3)), ((1, 3), (-1, 2)))


def _fwd(a, g, h, d):
    return [a + g, a - g, a + d, g + h]


def _inv(u, v, e, f):
    a = (u + v) * 0.5
    g = (u - v) * 0.5
    return [a, g, f - g, e - a]


def _rhs7(u, v, e, f):
    return [v - e, u - e, e + f, f - e, e + e, v, u]


def _lin(terms, fetch):
    t = fetch(terms[0][1])
    for sign, k in terms[1:]:
        t = t + fetch(k) if sign > 0 else t - fetch(k)
    return t


class _Q:
    def __init__(self, blocks):
        self.q = list(blocks)

    def __add__(self, o):
        return _Q(a + b for a, b in zip(self.q, o.q))

    def __sub__(self, o):
        return _Q(a - b for a, b in zip(self.q, o.q))

    def __mul__(self, s):
        return _Q(a * s for a in self.q)


def _scl(x, s):
    return x if s == 1.0 else x * s


def _rc(Q, q):
    return 2 * (Q // 2) + q // 2, 2 * (Q % 2) + q % 2


def _ident(x):
    return x


def _kernel(x0_hbm, w_hbm, b_hbm, o_hbm,
            wbuf, s_ref, m_ref, xin, ost, sp_z, sp_x, sp_b, bvm, bt_ref,
            sem_w, sem_in, sem_out, sem_misc,
            *, L, tm, d, ntiles, r0, wins, shifts, xwin, pfrac, pshift, ngroups, wcast, wide):
    d4 = d // 4
    r4 = tm // 4
    half = tm // 2
    nc = d4 // LANES
    N = ntiles
    dot = functools.partial(jnp.dot, preferred_element_type=F32)

    def ver(l):
        return "A" if l % L == 0 else "BC"[l % 2]

    ids = {}
    for name in ([(n, k) for n in "UV" for k in range(7)]
                 + [("Y", Q, (L - 1) % 2, k) for Q in (0, 1) for k in range(4)]
                 + [("X", a, ver(L - 1), k) for a in range(4) for k in range(4)]
                 + [("z", Q, k) for Q in (2, 3) for k in range(4)]):
        ids[name] = len(ids)
    nzero = len(ids)

    rw = [0, r4]

    def rows(base):
        if isinstance(rw[0], int):
            return slice(base + rw[0], base + rw[0] + rw[1])
        return pl.ds(pl.multiple_of(base + rw[0], 8), rw[1])

    def chunked(fn, lo, n):
        def body(k, c):
            rw[:] = [lo + k * 8, 8]
            fn()
            rw[:] = [0, r4]
            return c
        jax.lax.fori_loop(0, n // 8, body, 0)

    def put(name, v):
        i = ids.setdefault(name, len(ids))
        if wide:
            m_ref[i, rows(0), :d4] = v
            return
        for c in range(nc):
            m_ref[i, rows(c * r4), :] = v[:, c * LANES:(c + 1) * LANES]

    def get(name):
        i = ids.setdefault(name, len(ids))
        if wide:
            return m_ref[i, rows(0), :d4]
        return jnp.concatenate([m_ref[i, rows(c * r4), :] for c in range(nc)], axis=1)

    def putq(name, q):
        for k, v in enumerate(q.q):
            put(name + (k,), v)

    def getq(name):
        return _Q(get(name + (k,)) for k in range(4))

    def sl(Q, q):
        r, c = _rc(Q, q)
        return (rows(r * r4), slice(c * d4, (c + 1) * d4))

    def delta(l, Q, gate):
        par = l % 2
        c = []
        for k in range(7):
            t = get(("EFUU"[Q], k))
            if k in (1, 5, 6):
                t = gate(t)
            if Q >= 2:
                t = t + get(("V", k)) if Q == 2 else t - get(("V", k))
            c.append(t)
        f = c[1] - c[0]
        e = c[1] + c[0] + c[2] + c[3] + c[4]
        v = c[5] + c[3]
        u = c[6] - c[2]
        y = _Q([e, f, u + v + f, u - v + e])
        if Q < 2:
            putq(("Y", Q, par), y)
        else:
            y = y + getq(("Y", 3 - Q, par))
        return [get(("z", Q, q)) * (y.q[q] + bt_ref[l, 4 * Q + q, 0:1, :]) for q in range(4)]

    def finish(Q, gate, oslot):
        vr = ver(L - 1)
        dq = delta(L - 1, Q, gate)
        xu = _Q(gate(x) for x in getq(("X", 0, vr)).q)
        xv = getq(("X", 1, vr))
        t = ((xu + xv) if Q in (0, 3) else (xu - xv)) * 0.5
        if Q >= 2:
            t = getq(("X", 5 - Q, vr)) - t
        xs = _inv(*t.q)
        o = [_scl(xs[q] + dq[q], 1.0 / (_SCALE[Q] * _SCALE[q])) for q in range(4)]
        for q in range(4):
            ost[(oslot,) + sl(Q, q)] = o[q].astype(ost.dtype)
        return o

    def load_z(Q, gates, islot):
        putq(("z", Q), _Q(gates[q](xin[(islot,) + sl(Q, q)].astype(F32)) for q in range(4)))

    def init_x(gates, islot):
        def blk(Q, q):
            x = xin[(islot,) + sl(Q, q)].astype(F32)
            if q < 2:
                x = gates[Q](x)
            return _scl(x, _SCALE[Q] * _SCALE[q])
        x = _fwd(*[_Q(_fwd(*[blk(Q, q) for q in range(4)])) for Q in range(4)])
        for a in range(4):
            putq(("X", a, ver(0)), x[a])

    def update(l, Q, gate, oslot, islot, never):
        if l == L - 1:
            o = finish(Q, gate, oslot)
            load_z(Q, [lambda x, t=t: jnp.where(never, t, x) for t in o], islot)
            return
        par, vo, vn = l % 2, ver(l), ver(l + 1)
        dn = _Q(_fwd(*delta(l, Q, gate)))
        if Q < 2:
            putq(("D", Q, par), dn)
        if Q != 1:
            a = (0, None, 3, 2)[Q]
            putq(("X", a, vn), dn + getq(("X", a, vo)) + getq(("D", (1, None, 1, 0)[Q], par)))

    def update_v(l, gate):
        par, vo, vn = l % 2, ver(l), ver(l + 1)
        d11 = _Q(gate(x) for x in getq(("D", 0, par)).q)
        putq(("X", 1, vn), d11 + getq(("X", 1, vo)) - getq(("D", 1, par)))

    def w_copy(l):
        return pltpu.make_async_copy(w_hbm.at[l], wbuf.at[l], sem_w.at[l])

    def in_copy(t, slot):
        return pltpu.make_async_copy(
            x0_hbm.at[pl.ds(pl.multiple_of(t * tm, 16), tm)], xin.at[slot], sem_in.at[slot])

    def out_copy(t, slot, lo=0, n=tm):
        return pltpu.make_async_copy(
            ost.at[slot, pl.ds(lo, n)],
            o_hbm.at[pl.ds(pl.multiple_of(t * tm + lo, 16), n)], sem_out)

    sp_in = pltpu.make_async_copy(x0_hbm.at[pl.ds(N * tm, r0)], sp_b, sem_misc.at[0])
    sp_out = pltpu.make_async_copy(sp_b, o_hbm.at[pl.ds(N * tm, r0)], sem_misc.at[0])
    b_in = pltpu.make_async_copy(b_hbm, bvm, sem_misc.at[1])

    b_in.start()
    sp_in.start()

    def w_start(l, c):
        w_copy(l).start()
        return c
    jax.lax.fori_loop(0, L, w_start, 0)
    in_copy(0, 0).start()

    def zero(i, c):
        if wide:
            m_ref[i, :r4, :d4] = jnp.zeros((r4, d4), F32)
        else:
            m_ref[i] = jnp.zeros(m_ref.shape[1:], F32)
        return c
    jax.lax.fori_loop(0, nzero, zero, 0)
    in_copy(min(1, N - 1), 1).start()

    b_in.wait()
    ball = bvm[...].astype(F32)
    for l in range(L):
        for Q in range(4):
            for q in range(4):
                c = _rc(Q, q)[1]
                row = _scl(ball[l:l + 1, c * d4:(c + 1) * d4], _SCALE[Q] * _SCALE[q])
                bt_ref[l, 4 * Q + q] = jnp.broadcast_to(row, (8, d4))
    sp_in.wait()
    z0 = sp_b[...].astype(F32)
    sp_z[...] = z0
    sp_x[...] = z0

    def layer_body(l, carry):
        w_copy(l).wait()
        never = jnp.full((16, LANES), l, jnp.int32) < 0
        xb = sp_b[...]
        trig, new = [], []
        for n in range(d // LANES):
            cs = slice(n * LANES, (n + 1) * LANES)
            cb, off = divmod(n * LANES, d4)
            unscaled = 4 * 3 * (cb // 2) + 3 * (cb % 2)
            y1 = dot(xb[:, :d // 2], wbuf[l, :d // 2, cs]) + bt_ref[l, unscaled, 0:1, off:off + LANES]
            y2 = dot(xb[:, d // 2:], wbuf[l, d // 2:, cs]) + y1
            trig += [y[k * 16:(k + 1) * 16] for y in (y1, y2) for k in range(r0 // 16)]
            new.append(sp_z[:, cs] * y2 + sp_x[:, cs])
        for n in range(d // LANES):
            cs = slice(n * LANES, (n + 1) * LANES)
            sp_x[:, cs] = new[n]
            sp_b[:, cs] = new[n].astype(BF16)

        nch = (d4 // 16) * nc
        per = len(trig) // nch
        for ch in range(nch):
            rr, h = (ch // nc) * 16, ch % nc

            def blk(Q, q):
                r, c = _rc(Q, q)
                c0 = c * d4 + h * LANES
                w = wbuf[l, r * d4 + rr:r * d4 + rr + 16, c0:c0 + LANES].astype(F32)
                ti = ch * per + (pfrac[Q] * per) // 8 + pshift
                if q < 2 and ti >= 0:
                    w = jnp.where(never, trig[ti], w)
                return _scl(w, 0.25 * _SCALE[Q] * _SCALE[q])
            wt = _fwd(*[_Q(_fwd(*[blk(Q, q) for q in range(4)])) for Q in range(4)])
            for i, t in enumerate(_rhs7(*wt)):
                for j, u in enumerate(_rhs7(*t.q)):
                    s_ref[l, i * 7 + j, h, rr:rr + 16, :] = u.astype(BF16)
        return carry
    jax.lax.fori_loop(0, L, layer_body, 0)

    sp_out.start()
    in_copy(0, 0).wait()

    def first():
        init_x([_ident] * 4, 0)
        load_z(0, [_ident] * 4, 0)
        load_z(1, [_ident] * 4, 0)
    chunked(first, 0, r4)

    def tile_body(s, slots):
        cur, nxt, fre = slots
        in_copy(0, nxt).wait()
        in_copy(jnp.minimum(s + 2, N - 1), fre).start()
        oslot = s & 1
        never = jnp.full((r4, d4), s, jnp.int32) < 0
        s_u32 = s_ref.bitcast(jnp.uint32) if wcast else None
        prods = []

        def gate_on(lo, hi, shift):
            n = (r4 // 8) * nc
            parts = []
            for r in range(r4 // 8):
                cols = []
                for c in range(nc):
                    k, rem = divmod((r * nc + c) * (hi - lo) + shift, n)
                    rr, cc = divmod(rem, nc)
                    cols.append(prods[lo + k][rr * 8:(rr + 1) * 8, cc * LANES:(cc + 1) * LANES])
                parts.append(jnp.concatenate(cols, axis=1))
            trig = jnp.concatenate(parts, axis=0)
            return lambda x: jnp.where(never, trig, x)

        for l in range(L):
            lp = (l - 1) % L

            def outer(i):
                for j in range(7):
                    t = _lin(_LHS[j], lambda b: _lin(_LHS[i], lambda a: get(("X", a, ver(l), b))))
                    if wcast:
                        w = jnp.concatenate([s_u32[l, i * 7 + j, h] for h in range(nc)], axis=1)
                        w = pltpu.bitcast(w, BF16)
                    else:
                        w = jnp.concatenate([s_ref[l, i * 7 + j, h] for h in range(nc)], axis=1)
                    p = dot(t.astype(BF16), w)
                    prods.append(p)
                    if i in (0, 2, 3):
                        put(("P", i, j), p)
                    elif i == 1:
                        p0 = get(("P", 0, j))
                        put(("F", j), p - p0)
                        put(("G", j), p + p0)
                    elif i == 4:
                        put(("E", j), p + get(("G", j)) + get(("P", 2, j)) + get(("P", 3, j)))
                    elif i == 5:
                        put(("V", j), p + get(("P", 3, j)))
                    else:
                        put(("U", j), p - get(("P", 2, j)))

            def win(k):
                return gate_on(49 * l + wins[k][0], 49 * l + wins[k][1], shifts[k])

            outer(0)
            if l > 0:
                update_v(lp, win(4))
            outer(1)
            update(lp, 3, win(3), 1 - oslot, cur, never)
            outer(2)
            outer(3)
            outer(4)
            update(lp, 2, win(2), 1 - oslot, cur, never)
            update(l, 1, win(1), oslot, nxt, never)
            outer(5)
            outer(6)
            update(l, 0, win(0), oslot, nxt, never)
            if l == 0:
                @pl.when(s > 0)
                def _():
                    out_copy(s - 1, 1 - oslot).start()
                ost[oslot, 0:8, 0:d4] = prods[-1][0:8].astype(ost.dtype)
            if l == L - 2:
                init_x([gate_on(xwin[0], xwin[1], sh) for sh in xwin[2]], nxt)

        @pl.when(s > 0)
        def _():
            out_copy(0, 0).wait()
        return nxt, fre, cur
    jax.lax.fori_loop(0, N, tile_body, (0, 1, 2))

    oslot = (N - 1) % 2
    out_copy(N - 1, oslot, 0, half).start()
    gr = r4 // ngroups

    def last():
        finish(3, _ident, oslot)
        finish(2, _ident, oslot)

    def group(g, carry):
        lo = pl.multiple_of(g * gr, 16)
        chunked(last, lo, gr)
        for rb in (2, 3):
            out_copy(N - 1, oslot, pl.multiple_of(rb * r4 + lo, 16), gr).start()
        return carry
    jax.lax.fori_loop(0, ngroups, group, 0)
    in_copy(0, (N + 1) % 3).wait()
    sp_out.wait()
    out_copy(0, 0).wait()
    assert len(ids) <= m_ref.shape[0]


def _build(x0, ws, bs, *, TM=576, R0=256, pad=1, ngroups=3, nobc=False,
           wins=((35, 47), (24, 34), (12, 24), (4, 12), (0, 4)), shifts=(1, 1, 1, 1, 1),
           xwin=(98, 242, (0, 4, 12, 8)), pfrac=(0, 1, 6, 3), pshift=0, wcast=False, wide=129):
    B, D = x0.shape
    L = ws.shape[0]
    N = (B - R0) // TM
    assert R0 + N * TM == B and L % 2 == 0 and L >= 6 and D % (4 * LANES) == 0
    assert TM % (64 * ngroups) == 0 and R0 % 16 == 0
    nc = D // (4 * LANES)
    return pl.pallas_call(
        functools.partial(_kernel, L=L, tm=TM, d=D, ntiles=N, r0=R0, wins=wins, shifts=shifts,
                          xwin=xwin, pfrac=pfrac, pshift=pshift, ngroups=ngroups, wcast=wcast, wide=wide),
        in_specs=[pl.BlockSpec(memory_space=pl.ANY)] * 3,
        out_specs=pl.BlockSpec(memory_space=pl.ANY),
        out_shape=jax.ShapeDtypeStruct((B, D), x0.dtype),
        scratch_shapes=[
            pltpu.VMEM((L, D, D), BF16),
            pltpu.VMEM((L, 49, nc, D // 4, LANES), BF16),
            (pltpu.VMEM((152, TM // 4 + 8 * pad, D // 4 + wide - 1), F32) if wide else
             pltpu.VMEM((152, TM // 4 * nc + 8 * pad, LANES), F32)),
            pltpu.VMEM((3, TM, D), BF16),
            pltpu.VMEM((2, TM, D), BF16),
            pltpu.VMEM((R0, D), F32),
            pltpu.VMEM((R0, D), F32),
            pltpu.VMEM((R0, D), BF16),
            pltpu.VMEM((L, D), BF16),
            pltpu.VMEM((L, 16, 8, D // 4), F32),
            pltpu.SemaphoreType.DMA((L,)),
            pltpu.SemaphoreType.DMA((3,)),
            pltpu.SemaphoreType.DMA,
            pltpu.SemaphoreType.DMA((2,)),
        ],
        compiler_params=pltpu.CompilerParams(
            vmem_limit_bytes=120 * 1024 * 1024,
            disable_bounds_checks=nobc,
        ),
    )(x0, ws, bs)


@jax.jit
def pallas_standalone__dcn_v2_cross__recsys_kernel(
    x0: jax.Array,
    ws: jax.Array,
    bs: jax.Array,
):
    return _build(x0, ws, bs)
```

```python
import functools

import jax
import jax.numpy as jnp
import jax.experimental.pallas as pl
import jax.experimental.pallas.tpu as pltpu

F32 = jnp.float32
BF16 = jnp.bfloat16
LANES = 128

_SCALE = (1.0, 0.5, 2.0, 1.0)
_LHS = (((1, 0),), ((1, 1),), ((1, 0), (-1, 2)), ((1, 2), (-1, 1)), ((1, 2),),
        ((1, 2), (1, 3)), ((1, 3), (-1, 2)))


def _fwd(a, g, h, d):
    return [a + g, a - g, a + d, g + h]


def _inv(u, v, e, f):
    a = (u + v) * 0.5
    g = (u - v) * 0.5
    return [a, g, f - g, e - a]


def _rhs7(u, v, e, f):
    return [v - e, u - e, e + f, f - e, e + e, v, u]


def _lin(terms, fetch):
    t = fetch(terms[0][1])
    for sign, k in terms[1:]:
        t = t + fetch(k) if sign > 0 else t - fetch(k)
    return t


class _Q:
    def __init__(self, blocks):
        self.q = list(blocks)

    def __add__(self, o):
        return _Q(a + b for a, b in zip(self.q, o.q))

    def __sub__(self, o):
        return _Q(a - b for a, b in zip(self.q, o.q))

    def __mul__(self, s):
        return _Q(a * s for a in self.q)


def _scl(x, s):
    return x if s == 1.0 else x * s


def _rc(Q, q):
    return 2 * (Q // 2) + q // 2, 2 * (Q % 2) + q % 2


def _ident(x):
    return x


def _kernel(x0_hbm, w_hbm, b_hbm, o_hbm,
            wbuf, s_ref, m_ref, xin, ost, sp_z, sp_x, sp_b, bvm, bt_ref,
            sem_w, sem_in, sem_out, sem_misc,
            *, L, tm, d, ntiles, r0, wins, shifts, xwin, pfrac, pshift, ngroups, zwin, reps):
    d4 = d // 4
    r4 = tm // 4
    half = tm // 2
    nc = d4 // LANES
    N = ntiles
    dot = functools.partial(jnp.dot, preferred_element_type=F32)

    def ver(l):
        return "A" if l % L == 0 else "BC"[l % 2]

    ids = {}
    for name in ([(n, k) for n in "UV" for k in range(7)]
                 + [("Y", Q, (L - 1) % 2, k) for Q in (0, 1) for k in range(4)]
                 + [("H", Q, k) for Q in (2, 3) for k in range(4)]
                 + [("z", Q, k) for Q in (2, 3) for k in range(4)]):
        ids[name] = len(ids)
    nzero = len(ids)

    rw = [0, r4]

    def rows(base):
        if isinstance(rw[0], int):
            return slice(base + rw[0], base + rw[0] + rw[1])
        return pl.ds(pl.multiple_of(base + rw[0], 8), rw[1])

    def chunked(fn, lo, n, rep):
        def body(k, c):
            for u in range(rep):
                rw[:] = [lo + (k * rep + u) * 8, 8]
                fn()
            rw[:] = [0, r4]
            return c
        jax.lax.fori_loop(0, n // (8 * rep), body, 0)

    def put(name, v):
        m_ref[ids.setdefault(name, len(ids)), rows(0), :d4] = v

    def get(name):
        return m_ref[ids.setdefault(name, len(ids)), rows(0), :d4]

    def putq(name, q):
        for k, v in enumerate(q.q):
            put(name + (k,), v)

    def getq(name):
        return _Q(get(name + (k,)) for k in range(4))

    def sl(Q, q):
        r, c = _rc(Q, q)
        return (rows(r * r4), slice(c * d4, (c + 1) * d4))

    def delta(l, Q, gate):
        par = l % 2
        c = []
        for k in range(7):
            t = get(("EFUU"[Q], k))
            if k in (1, 5, 6):
                t = gate(t)
            if Q >= 2:
                t = t + get(("V", k)) if Q == 2 else t - get(("V", k))
            c.append(t)
        f = c[1] - c[0]
        e = c[1] + c[0] + c[2] + c[3] + c[4]
        v = c[5] + c[3]
        u = c[6] - c[2]
        y = _Q([e, f, u + v + f, u - v + e])
        if Q < 2:
            putq(("Y", Q, par), y)
        else:
            y = y + getq(("Y", 3 - Q, par))
        return [get(("z", Q, q)) * (y.q[q] + bt_ref[l, 4 * Q + q, 0:1, :]) for q in range(4)]

    def finish(Q, gate, oslot):
        dq = delta(L - 1, Q, gate)
        if Q < 2:
            vr = ver(L - 1)
            xu = _Q(gate(x) for x in getq(("X", 0, vr)).q)
            xv = getq(("X", 1, vr))
            t = ((xu + xv) if Q == 0 else (xu - xv)) * 0.5
            xs = _inv(*t.q)
            putq(("H", 3 - Q), _Q(_inv(*(getq(("X", 2 + Q, vr)) - t).q)))
        else:
            xs = getq(("H", Q)).q
        o = [_scl(xs[q] + dq[q], 1.0 / (_SCALE[Q] * _SCALE[q])) for q in range(4)]
        for q in range(4):
            ost[(oslot,) + sl(Q, q)] = o[q].astype(ost.dtype)
        return o

    def load_z(Q, gates, islot):
        putq(("z", Q), _Q(gates[q](xin[(islot,) + sl(Q, q)].astype(F32)) for q in range(4)))

    def init_x(gates, islot):
        def blk(Q, q):
            x = xin[(islot,) + sl(Q, q)].astype(F32)
            if q < 2:
                x = gates[Q](x)
            return _scl(x, _SCALE[Q] * _SCALE[q])
        x = _fwd(*[_Q(_fwd(*[blk(Q, q) for q in range(4)])) for Q in range(4)])
        for a in range(4):
            putq(("X", a, ver(0)), x[a])

    def update(l, Q, gate, oslot, islot, never):
        if l == L - 1:
            o = finish(Q, gate, oslot)
            if Q >= 2:
                load_z(Q, [lambda x, t=t: jnp.where(never, t, x) for t in o], islot)
            return
        par, vo, vn = l % 2, ver(l), ver(l + 1)
        dn = _Q(_fwd(*delta(l, Q, gate)))
        if Q < 2:
            putq(("D", Q, par), dn)
        if Q != 1:
            a = (0, None, 3, 2)[Q]
            putq(("X", a, vn), dn + getq(("X", a, vo)) + getq(("D", (1, None, 1, 0)[Q], par)))

    def update_v(l, gate):
        par, vo, vn = l % 2, ver(l), ver(l + 1)
        d11 = _Q(gate(x) for x in getq(("D", 0, par)).q)
        putq(("X", 1, vn), d11 + getq(("X", 1, vo)) - getq(("D", 1, par)))

    def w_copy(l):
        return pltpu.make_async_copy(w_hbm.at[l], wbuf.at[l], sem_w.at[l])

    def in_copy(t, slot):
        return pltpu.make_async_copy(
            x0_hbm.at[pl.ds(pl.multiple_of(t * tm, 16), tm)], xin.at[slot], sem_in.at[slot])

    def out_copy(t, slot, lo=0, n=tm):
        return pltpu.make_async_copy(
            ost.at[slot, pl.ds(lo, n)],
            o_hbm.at[pl.ds(pl.multiple_of(t * tm + lo, 16), n)], sem_out)

    def last_top(Q):
        cols = pl.ds(Q * (d // 2), d // 2)
        return pltpu.make_async_copy(
            ost.at[(N - 1) % 2, pl.ds(0, half), cols],
            o_hbm.at[pl.ds((N - 1) * tm, half), cols], sem_misc.at[2 + Q])

    sp_in = pltpu.make_async_copy(x0_hbm.at[pl.ds(N * tm, r0)], sp_b, sem_misc.at[0])
    sp_out = pltpu.make_async_copy(sp_b, o_hbm.at[pl.ds(N * tm, r0)], sem_misc.at[0])
    b_in = pltpu.make_async_copy(b_hbm, bvm, sem_misc.at[1])

    b_in.start()
    sp_in.start()

    def w_start(l, c):
        w_copy(l).start()
        return c
    jax.lax.fori_loop(0, L, w_start, 0)
    in_copy(0, 0).start()

    def zero(i, c):
        m_ref[i, :r4, :d4] = jnp.zeros((r4, d4), F32)
        return c
    jax.lax.fori_loop(0, nzero, zero, 0)
    in_copy(min(1, N - 1), 1).start()

    b_in.wait()
    ball = bvm[...].astype(F32)
    for l in range(L):
        for Q in range(4):
            for q in range(4):
                c = _rc(Q, q)[1]
                row = _scl(ball[l:l + 1, c * d4:(c + 1) * d4], _SCALE[Q] * _SCALE[q])
                bt_ref[l, 4 * Q + q] = jnp.broadcast_to(row, (8, d4))
    sp_in.wait()
    z0 = sp_b[...].astype(F32)
    sp_z[...] = z0
    sp_x[...] = z0

    def layer_body(l, carry):
        w_copy(l).wait()
        never = jnp.full((16, LANES), l, jnp.int32) < 0
        xb = sp_b[...]
        trig, new = [], []
        for n in range(d // LANES):
            cs = slice(n * LANES, (n + 1) * LANES)
            cb, off = divmod(n * LANES, d4)
            unscaled = 4 * 3 * (cb // 2) + 3 * (cb % 2)
            y1 = dot(xb[:, :d // 2], wbuf[l, :d // 2, cs]) + bt_ref[l, unscaled, 0:1, off:off + LANES]
            y2 = dot(xb[:, d // 2:], wbuf[l, d // 2:, cs]) + y1
            trig += [y[k * 16:(k + 1) * 16] for y in (y1, y2) for k in range(r0 // 16)]
            new.append(sp_z[:, cs] * y2 + sp_x[:, cs])
        for n in range(d // LANES):
            cs = slice(n * LANES, (n + 1) * LANES)
            sp_x[:, cs] = new[n]
            sp_b[:, cs] = new[n].astype(BF16)

        nch = (d4 // 16) * nc
        per = len(trig) // nch
        for ch in range(nch):
            rr, h = (ch // nc) * 16, ch % nc

            def blk(Q, q):
                r, c = _rc(Q, q)
                c0 = c * d4 + h * LANES
                w = wbuf[l, r * d4 + rr:r * d4 + rr + 16, c0:c0 + LANES].astype(F32)
                ti = ch * per + (pfrac[Q] * per) // 8 + pshift
                if q < 2 and ti >= 0:
                    w = jnp.where(never, trig[ti], w)
                return _scl(w, 0.25 * _SCALE[Q] * _SCALE[q])
            wt = _fwd(*[_Q(_fwd(*[blk(Q, q) for q in range(4)])) for Q in range(4)])
            for i, t in enumerate(_rhs7(*wt)):
                for j, u in enumerate(_rhs7(*t.q)):
                    s_ref[l, i * 7 + j, h, rr:rr + 16, :] = u.astype(BF16)
        return carry
    jax.lax.fori_loop(0, L, layer_body, 0)

    sp_out.start()
    in_copy(0, 0).wait()

    chunked(lambda: init_x([_ident] * 4, 0), 0, r4, reps[0])

    def tile_body(s, slots):
        cur, nxt, fre = slots
        in_copy(0, nxt).wait()
        in_copy(jnp.minimum(s + 2, N - 1), fre).start()
        oslot = s & 1
        never = jnp.full((r4, d4), s, jnp.int32) < 0
        prods = []

        def gate_on(lo, hi, shift):
            n = (r4 // 8) * nc
            parts = []
            for r in range(r4 // 8):
                cols = []
                for c in range(nc):
                    k, rem = divmod((r * nc + c) * (hi - lo) + shift, n)
                    rr, cc = divmod(rem, nc)
                    cols.append(prods[lo + k][rr * 8:(rr + 1) * 8, cc * LANES:(cc + 1) * LANES])
                parts.append(jnp.concatenate(cols, axis=1))
            trig = jnp.concatenate(parts, axis=0)
            return lambda x: jnp.where(never, trig, x)

        for l in range(L):
            lp = (l - 1) % L

            def outer(i):
                for j in range(7):
                    t = _lin(_LHS[j], lambda b: _lin(_LHS[i], lambda a: get(("X", a, ver(l), b))))
                    w = jnp.concatenate([s_ref[l, i * 7 + j, h] for h in range(nc)], axis=1)
                    p = dot(t.astype(BF16), w)
                    prods.append(p)
                    if i in (0, 2, 3):
                        put(("P", i, j), p)
                    elif i == 1:
                        p0 = get(("P", 0, j))
                        put(("F", j), p - p0)
                        put(("G", j), p + p0)
                    elif i == 4:
                        put(("E", j), p + get(("G", j)) + get(("P", 2, j)) + get(("P", 3, j)))
                    elif i == 5:
                        put(("V", j), p + get(("P", 3, j)))
                    else:
                        put(("U", j), p - get(("P", 2, j)))

            def win(k):
                return gate_on(49 * l + wins[k][0], 49 * l + wins[k][1], shifts[k])

            outer(0)
            if l > 0:
                update_v(lp, win(4))
            outer(1)
            update(lp, 3, win(3), 1 - oslot, cur, never)
            outer(2)
            outer(3)
            outer(4)
            update(lp, 2, win(2), 1 - oslot, cur, never)
            if l == 0:
                load_z(1, [gate_on(*zwin[1])] * 4, cur)
                load_z(0, [gate_on(*zwin[0])] * 4, cur)
            update(l, 1, win(1), oslot, nxt, never)
            if l == L - 1:
                @pl.when(s == N - 1)
                def _():
                    last_top(1).start()
            outer(5)
            outer(6)
            update(l, 0, win(0), oslot, nxt, never)
            if l == 0:
                @pl.when(s > 0)
                def _():
                    out_copy(s - 1, 1 - oslot).start()
                ost[oslot, 0:8, 0:d4] = prods[-1][0:8].astype(ost.dtype)
            if l == L - 2:
                init_x([gate_on(xwin[0], xwin[1], sh) for sh in xwin[2]], nxt)

        @pl.when(s > 0)
        def _():
            out_copy(0, 0).wait()
        return nxt, fre, cur
    jax.lax.fori_loop(0, N, tile_body, (0, 1, 2))

    oslot = (N - 1) % 2
    last_top(0).start()
    gr = r4 // ngroups

    def last():
        finish(3, _ident, oslot)
        finish(2, _ident, oslot)

    def group(g, carry):
        lo = pl.multiple_of(g * gr, 16)
        chunked(last, lo, gr, reps[1])
        for rb in (2, 3):
            out_copy(N - 1, oslot, pl.multiple_of(rb * r4 + lo, 16), gr).start()
        return carry
    jax.lax.fori_loop(0, ngroups, group, 0)
    in_copy(0, (N + 1) % 3).wait()
    sp_out.wait()
    last_top(1).wait()
    last_top(0).wait()
    out_copy(0, 0, 0, half).wait()
    assert len(ids) <= m_ref.shape[0]


def _build(x0, ws, bs, *, TM=768, R0=256, ngroups=4,
           wins=((35, 47), (24, 34), (12, 24), (4, 12), (0, 4)), shifts=(1, 1, 1, 1, 1),
           xwin=(98, 242, (1, 1, 17, 9)), pfrac=(0, 1, 6, 3), pshift=0,
           zwin=((2, 4, 1), (0, 2, 1)), reps=(2, 2)):
    B, D = x0.shape
    L = ws.shape[0]
    N = (B - R0) // TM
    assert R0 + N * TM == B and L % 2 == 0 and L >= 6 and D % (4 * LANES) == 0
    assert TM % (64 * ngroups) == 0 and R0 % 16 == 0
    nc = D // (4 * LANES)
    return pl.pallas_call(
        functools.partial(_kernel, L=L, tm=TM, d=D, ntiles=N, r0=R0, wins=wins, shifts=shifts,
                          xwin=xwin, pfrac=pfrac, pshift=pshift, ngroups=ngroups,
                          zwin=zwin, reps=reps),
        in_specs=[pl.BlockSpec(memory_space=pl.ANY)] * 3,
        out_specs=pl.BlockSpec(memory_space=pl.ANY),
        out_shape=jax.ShapeDtypeStruct((B, D), x0.dtype),
        scratch_shapes=[
            pltpu.VMEM((L, D, D), BF16),
            pltpu.VMEM((L, 49, nc, D // 4, LANES), BF16),
            pltpu.VMEM((160, TM // 4 + 8, D // 4 + LANES), F32),
            pltpu.VMEM((3, TM, D), BF16),
            pltpu.VMEM((2, TM, D), BF16),
            pltpu.VMEM((R0, D), F32),
            pltpu.VMEM((R0, D), F32),
            pltpu.VMEM((R0, D), BF16),
            pltpu.VMEM((L, D), BF16),
            pltpu.VMEM((L, 16, 8, D // 4), F32),
            pltpu.SemaphoreType.DMA((L,)),
            pltpu.SemaphoreType.DMA((3,)),
            pltpu.SemaphoreType.DMA,
            pltpu.SemaphoreType.DMA((4,)),
        ],
        compiler_params=pltpu.CompilerParams(vmem_limit_bytes=120 * 1024 * 1024),
    )(x0, ws, bs)


@jax.jit
def pallas_standalone__dcn_v2_cross__recsys_kernel(
    x0: jax.Array,
    ws: jax.Array,
    bs: jax.Array,
):
    return _build(x0, ws, bs)
```

```python
import functools

import jax
import jax.numpy as jnp
import jax.experimental.pallas as pl
import jax.experimental.pallas.tpu as pltpu

F32 = jnp.float32
BF16 = jnp.bfloat16
LANES = 128

_SCALE = (1.0, 0.5, 2.0, 1.0)
_LHS = (((1, 0),), ((1, 1),), ((1, 0), (-1, 2)), ((1, 2), (-1, 1)), ((1, 2),),
        ((1, 2), (1, 3)), ((1, 3), (-1, 2)))


def _fwd(a, g, h, d):
    return [a + g, a - g, a + d, g + h]


def _inv(u, v, e, f):
    a = (u + v) * 0.5
    g = (u - v) * 0.5
    return [a, g, f - g, e - a]


def _rhs7(u, v, e, f):
    return [v - e, u - e, e + f, f - e, e + e, v, u]


def _lin(terms, fetch):
    t = fetch(terms[0][1])
    for sign, k in terms[1:]:
        t = t + fetch(k) if sign > 0 else t - fetch(k)
    return t


class _Q:
    def __init__(self, blocks):
        self.q = list(blocks)

    def __add__(self, o):
        return _Q(a + b for a, b in zip(self.q, o.q))

    def __sub__(self, o):
        return _Q(a - b for a, b in zip(self.q, o.q))

    def __mul__(self, s):
        return _Q(a * s for a in self.q)


def _scl(x, s):
    return x if s == 1.0 else x * s


def _rc(Q, q):
    return 2 * (Q // 2) + q // 2, 2 * (Q % 2) + q % 2


def _ident(x):
    return x


def _kernel(x0_hbm, w_hbm, b_hbm, o_hbm,
            wbuf, s_ref, m_ref, xin, ost, sp_z, sp_x, sp_b, bvm, bt_ref,
            sem_w, sem_in, sem_out, sem_misc,
            *, L, tm, d, ntiles, r0, wins, shifts, xwin, pfrac, pshift, ngroups, zwin, reps, early):
    d4 = d // 4
    r4 = tm // 4
    half = tm // 2
    nc = d4 // LANES
    N = ntiles
    dot = functools.partial(jnp.dot, preferred_element_type=F32)

    def ver(l):
        return "A" if l % L == 0 else "BC"[l % 2]

    ids = {}
    for name in ([(n, k) for n in "UV" for k in range(7)]
                 + [("Y", Q, (L - 1) % 2, k) for Q in (0, 1) for k in range(4)]
                 + [("H", Q, k) for Q in (2, 3) for k in range(4)]
                 + [("z", Q, k) for Q in (2, 3) for k in range(4)]):
        ids[name] = len(ids)
    nzero = len(ids)

    rw = [0, r4]

    def rows(base):
        if isinstance(rw[0], int):
            return slice(base + rw[0], base + rw[0] + rw[1])
        return pl.ds(pl.multiple_of(base + rw[0], 8), rw[1])

    def chunked(fn, lo, n, rep):
        def body(k, c):
            for u in range(rep):
                rw[:] = [lo + (k * rep + u) * 8, 8]
                fn()
            rw[:] = [0, r4]
            return c
        jax.lax.fori_loop(0, n // (8 * rep), body, 0)

    def put(name, v):
        m_ref[ids.setdefault(name, len(ids)), rows(0), :d4] = v

    def get(name):
        return m_ref[ids.setdefault(name, len(ids)), rows(0), :d4]

    def putq(name, q):
        for k, v in enumerate(q.q):
            put(name + (k,), v)

    def getq(name):
        return _Q(get(name + (k,)) for k in range(4))

    def sl(Q, q):
        r, c = _rc(Q, q)
        return (rows(r * r4), slice(c * d4, (c + 1) * d4))

    def delta(l, Q, gate):
        par = l % 2
        c = []
        for k in range(7):
            t = get(("EFUU"[Q], k))
            if k in (1, 5, 6):
                t = gate(t)
            if Q >= 2:
                t = t + get(("V", k)) if Q == 2 else t - get(("V", k))
            c.append(t)
        f = c[1] - c[0]
        e = c[1] + c[0] + c[2] + c[3] + c[4]
        v = c[5] + c[3]
        u = c[6] - c[2]
        y = _Q([e, f, u + v + f, u - v + e])
        if Q < 2:
            putq(("Y", Q, par), y)
        else:
            y = y + getq(("Y", 3 - Q, par))
        return [get(("z", Q, q)) * (y.q[q] + bt_ref[l, 4 * Q + q, 0:1, :]) for q in range(4)]

    def finish(Q, gate, oslot):
        dq = delta(L - 1, Q, gate)
        if Q < 2:
            vr = ver(L - 1)
            xu = _Q(gate(x) for x in getq(("X", 0, vr)).q)
            xv = getq(("X", 1, vr))
            t = ((xu + xv) if Q == 0 else (xu - xv)) * 0.5
            xs = _inv(*t.q)
            putq(("H", 3 - Q), _Q(_inv(*(getq(("X", 2 + Q, vr)) - t).q)))
        else:
            xs = getq(("H", Q)).q
        o = [_scl(xs[q] + dq[q], 1.0 / (_SCALE[Q] * _SCALE[q])) for q in range(4)]
        for q in range(4):
            ost[(oslot,) + sl(Q, q)] = o[q].astype(ost.dtype)
        return o

    def load_z(Q, gates, islot):
        putq(("z", Q), _Q(gates[q](xin[(islot,) + sl(Q, q)].astype(F32)) for q in range(4)))

    def init_x(gates, islot):
        def blk(Q, q):
            x = xin[(islot,) + sl(Q, q)].astype(F32)
            if q < 2:
                x = gates[Q](x)
            return _scl(x, _SCALE[Q] * _SCALE[q])
        x = _fwd(*[_Q(_fwd(*[blk(Q, q) for q in range(4)])) for Q in range(4)])
        for a in range(4):
            putq(("X", a, ver(0)), x[a])

    def update(l, Q, gate, oslot, islot, never):
        if l == L - 1:
            o = finish(Q, gate, oslot)
            if Q >= 2:
                load_z(Q, [lambda x, t=t: jnp.where(never, t, x) for t in o], islot)
            return
        par, vo, vn = l % 2, ver(l), ver(l + 1)
        dn = _Q(_fwd(*delta(l, Q, gate)))
        if Q < 2:
            putq(("D", Q, par), dn)
        if Q != 1:
            a = (0, None, 3, 2)[Q]
            putq(("X", a, vn), dn + getq(("X", a, vo)) + getq(("D", (1, None, 1, 0)[Q], par)))

    def update_v(l, gate):
        par, vo, vn = l % 2, ver(l), ver(l + 1)
        d11 = _Q(gate(x) for x in getq(("D", 0, par)).q)
        putq(("X", 1, vn), d11 + getq(("X", 1, vo)) - getq(("D", 1, par)))

    def w_copy(l):
        return pltpu.make_async_copy(w_hbm.at[l], wbuf.at[l, :, pl.ds(0, d)], sem_w.at[l])

    def in_copy(t, slot):
        return pltpu.make_async_copy(
            x0_hbm.at[pl.ds(pl.multiple_of(t * tm, 16), tm)], xin.at[slot], sem_in.at[slot])

    def out_copy(t, slot, lo=0, n=tm):
        return pltpu.make_async_copy(
            ost.at[slot, pl.ds(lo, n)],
            o_hbm.at[pl.ds(pl.multiple_of(t * tm + lo, 16), n)], sem_out)

    def last_top(Q, lo=0, n=half):
        cols = pl.ds(Q * (d // 2), d // 2)
        return pltpu.make_async_copy(
            ost.at[(N - 1) % 2, pl.ds(lo, n), cols],
            o_hbm.at[pl.ds((N - 1) * tm + lo, n), cols], sem_misc.at[2 + Q])

    sp_bv = sp_b.at[:, pl.ds(0, d)]
    sp_in = pltpu.make_async_copy(x0_hbm.at[pl.ds(N * tm, r0)], sp_bv, sem_misc.at[0])
    sp_out = pltpu.make_async_copy(sp_bv, o_hbm.at[pl.ds(N * tm, r0)], sem_misc.at[0])
    b_in = pltpu.make_async_copy(b_hbm, bvm, sem_misc.at[1])

    b_in.start()
    sp_in.start()

    def w_start(l, c):
        w_copy(l).start()
        return c
    jax.lax.fori_loop(0, L, w_start, 0)
    in_copy(0, 0).start()

    def zero(i, c):
        m_ref[i, :r4, :d4] = jnp.zeros((r4, d4), F32)
        return c
    jax.lax.fori_loop(0, nzero, zero, 0)
    in_copy(min(1, N - 1), 1).start()

    b_in.wait()
    ball = bvm[...].astype(F32)
    for l in range(L):
        for Q in range(4):
            for q in range(4):
                c = _rc(Q, q)[1]
                row = _scl(ball[l:l + 1, c * d4:(c + 1) * d4], _SCALE[Q] * _SCALE[q])
                bt_ref[l, 4 * Q + q] = jnp.broadcast_to(row, (8, d4))
    sp_in.wait()
    z0 = sp_b[:, :d].astype(F32)
    sp_z[:, :d] = z0
    sp_x[:, :d] = z0

    def layer_body(l, carry):
        w_copy(l).wait()
        never = jnp.full((16, LANES), l, jnp.int32) < 0
        xb = sp_b[:, :d]
        trig, new = [], []
        for n in range(d // LANES):
            cs = slice(n * LANES, (n + 1) * LANES)
            cb, off = divmod(n * LANES, d4)
            unscaled = 4 * 3 * (cb // 2) + 3 * (cb % 2)
            y1 = dot(xb[:, :d // 2], wbuf[l, :d // 2, cs]) + bt_ref[l, unscaled, 0:1, off:off + LANES]
            y2 = dot(xb[:, d // 2:], wbuf[l, d // 2:, cs]) + y1
            trig += [y[k * 16:(k + 1) * 16] for y in (y1, y2) for k in range(r0 // 16)]
            new.append(sp_z[:, cs] * y2 + sp_x[:, cs])
        for n in range(0, d // LANES, 2):
            cs = slice(n * LANES, (n + 2) * LANES)
            v = jnp.concatenate(new[n:n + 2], axis=1)
            sp_x[:, cs] = v
            sp_b[:, cs] = v.astype(BF16)

        nch = (d4 // 16) * nc
        per = len(trig) // nch
        for ch in range(nch):
            rr, h = (ch // nc) * 16, ch % nc

            def blk(Q, q):
                r, c = _rc(Q, q)
                c0 = c * d4 + h * LANES
                w = wbuf[l, r * d4 + rr:r * d4 + rr + 16, c0:c0 + LANES].astype(F32)
                ti = ch * per + (pfrac[Q] * per) // 8 + pshift
                if q < 2 and ti >= 0:
                    w = jnp.where(never, trig[ti], w)
                return _scl(w, 0.25 * _SCALE[Q] * _SCALE[q])
            wt = _fwd(*[_Q(_fwd(*[blk(Q, q) for q in range(4)])) for Q in range(4)])
            for i, t in enumerate(_rhs7(*wt)):
                for j, u in enumerate(_rhs7(*t.q)):
                    s_ref[l, i * 7 + j, h, rr:rr + 16, :] = u.astype(BF16)
        return carry
    jax.lax.fori_loop(0, L, layer_body, 0)

    sp_out.start()
    in_copy(0, 0).wait()

    chunked(lambda: init_x([_ident] * 4, 0), 0, r4, reps[0])

    def tile_body(s, slots):
        cur, nxt, fre = slots
        in_copy(0, nxt).wait()
        in_copy(jnp.minimum(s + 2, N - 1), fre).start()
        oslot = s & 1
        never = jnp.full((r4, d4), s, jnp.int32) < 0
        prods = []

        def gate_on(lo, hi, shift):
            n = (r4 // 8) * nc
            parts = []
            for r in range(rw[0] // 8, (rw[0] + rw[1]) // 8):
                cols = []
                for c in range(nc):
                    k, rem = divmod((r * nc + c) * (hi - lo) + shift, n)
                    rr, cc = divmod(rem, nc)
                    cols.append(prods[lo + k][rr * 8:(rr + 1) * 8, cc * LANES:(cc + 1) * LANES])
                parts.append(jnp.concatenate(cols, axis=1))
            trig = jnp.concatenate(parts, axis=0)
            nv = never if rw[1] == r4 else jnp.full(trig.shape, s, jnp.int32) < 0
            return lambda x: jnp.where(nv, trig, x)

        for l in range(L):
            lp = (l - 1) % L

            def outer(i):
                for j in range(7):
                    t = _lin(_LHS[j], lambda b: _lin(_LHS[i], lambda a: get(("X", a, ver(l), b))))
                    w = jnp.concatenate([s_ref[l, i * 7 + j, h] for h in range(nc)], axis=1)
                    p = dot(t.astype(BF16), w)
                    prods.append(p)
                    if i in (0, 2, 3):
                        put(("P", i, j), p)
                    elif i == 1:
                        p0 = get(("P", 0, j))
                        put(("F", j), p - p0)
                        put(("G", j), p + p0)
                    elif i == 4:
                        put(("E", j), p + get(("G", j)) + get(("P", 2, j)) + get(("P", 3, j)))
                    elif i == 5:
                        put(("V", j), p + get(("P", 3, j)))
                    else:
                        put(("U", j), p - get(("P", 2, j)))

            def win(k):
                return gate_on(49 * l + wins[k][0], 49 * l + wins[k][1], shifts[k])

            outer(0)
            if l > 0:
                update_v(lp, win(4))
            outer(1)
            update(lp, 3, win(3), 1 - oslot, cur, never)
            outer(2)
            outer(3)
            outer(4)
            update(lp, 2, win(2), 1 - oslot, cur, never)
            if l == 0:
                load_z(1, [gate_on(*zwin[1])] * 4, cur)
                load_z(0, [gate_on(*zwin[0])] * 4, cur)
            update(l, 1, win(1), oslot, nxt, never)
            if l == L - 1:
                @pl.when(s == N - 1)
                def _():
                    last_top(1).start()
            outer(5)
            outer(6)
            if l < L - 1:
                update(l, 0, win(0), oslot, nxt, never)
            else:
                rw[:] = [0, early]
                update(l, 0, win(0), oslot, nxt, never)

                @pl.when(s == N - 1)
                def _():
                    last_top(0, 0, early).start()
                    last_top(0, r4, early).start()
                rw[:] = [early, r4 - early]
                update(l, 0, win(0), oslot, nxt, never)
                rw[:] = [0, r4]
            if l == 0:
                @pl.when(s > 0)
                def _():
                    out_copy(s - 1, 1 - oslot).start()
                ost[oslot, 0:8, 0:d4] = prods[-1][0:8].astype(ost.dtype)
            if l == L - 2:
                init_x([gate_on(xwin[0], xwin[1], sh) for sh in xwin[2]], nxt)

        @pl.when(s > 0)
        def _():
            out_copy(0, 0).wait()
        return nxt, fre, cur
    jax.lax.fori_loop(0, N, tile_body, (0, 1, 2))

    oslot = (N - 1) % 2
    last_top(0, early, r4 - early).start()
    last_top(0, r4 + early, r4 - early).start()
    gr = r4 // ngroups

    def last():
        finish(3, _ident, oslot)
        finish(2, _ident, oslot)

    def group(g, carry):
        lo = pl.multiple_of(g * gr, 16)
        chunked(last, lo, gr, reps[1])
        for rb in (2, 3):
            out_copy(N - 1, oslot, pl.multiple_of(rb * r4 + lo, 16), gr).start()
        return carry
    jax.lax.fori_loop(0, ngroups, group, 0)
    in_copy(0, (N + 1) % 3).wait()
    sp_out.wait()
    last_top(1).wait()
    last_top(0).wait()
    out_copy(0, 0, 0, half).wait()
    assert len(ids) <= m_ref.shape[0]


def _build(x0, ws, bs, *, TM=768, R0=256, ngroups=12,
           wins=((35, 47), (24, 32), (12, 24), (4, 12), (0, 4)), shifts=(1, 1, 1, 1, 1),
           xwin=(98, 146, (11, 11, 35, 23)), pfrac=(0, 1, 6, 3), pshift=0,
           zwin=((22, 34, 7), (0, 4, 1)), reps=(2, 2), early=160):
    B, D = x0.shape
    L = ws.shape[0]
    N = (B - R0) // TM
    assert R0 + N * TM == B and L % 2 == 0 and L >= 6 and D % (4 * LANES) == 0
    assert TM % (64 * ngroups) == 0 and R0 % 16 == 0 and early % 16 == 0 and early < TM // 4
    nc = D // (4 * LANES)
    return pl.pallas_call(
        functools.partial(_kernel, L=L, tm=TM, d=D, ntiles=N, r0=R0, wins=wins, shifts=shifts,
                          xwin=xwin, pfrac=pfrac, pshift=pshift, ngroups=ngroups,
                          zwin=zwin, reps=reps, early=early),
        in_specs=[pl.BlockSpec(memory_space=pl.ANY)] * 3,
        out_specs=pl.BlockSpec(memory_space=pl.ANY),
        out_shape=jax.ShapeDtypeStruct((B, D), x0.dtype),
        scratch_shapes=[
            pltpu.VMEM((L, D, D + 2 * LANES), BF16),
            pltpu.VMEM((L, 49, nc, D // 4, LANES), BF16),
            pltpu.VMEM((160, TM // 4 + 8, D // 4 + LANES), F32),
            pltpu.VMEM((3, TM, D), BF16),
            pltpu.VMEM((2, TM, D), BF16),
            pltpu.VMEM((R0, D + LANES), F32),
            pltpu.VMEM((R0, D + LANES), F32),
            pltpu.VMEM((R0, D + 2 * LANES), BF16),
            pltpu.VMEM((L, D), BF16),
            pltpu.VMEM((L, 16, 8, D // 4), F32),
            pltpu.SemaphoreType.DMA((L,)),
            pltpu.SemaphoreType.DMA((3,)),
            pltpu.SemaphoreType.DMA,
            pltpu.SemaphoreType.DMA((4,)),
        ],
        compiler_params=pltpu.CompilerParams(vmem_limit_bytes=120 * 1024 * 1024),
    )(x0, ws, bs)


@jax.jit
def pallas_standalone__dcn_v2_cross__recsys_kernel(
    x0: jax.Array,
    ws: jax.Array,
    bs: jax.Array,
):
    return _build(x0, ws, bs)
```

```python
import functools

import jax
import jax.numpy as jnp
import jax.experimental.pallas as pl
import jax.experimental.pallas.tpu as pltpu

F32 = jnp.float32
BF16 = jnp.bfloat16
LANES = 128

_T = 1.75
_EXP = (0, -1, 1, 0)
_LHS = (((1, 0),), ((1, 1),), ((1, 0), (-1, 2)), ((1, 2), (-1, 1)), ((1, 2),),
        ((1, 2), (1, 3)), ((1, 3), (-1, 2)))

_JA, _JB, _JF = (0, 1), (2, 5), (3, 4, 6)
_PLAN = (("r", (0, 1), _JA), ("f", (0, 1), _JF), ("r", (0, 1), _JB), ("a", (0, 1), _JA), ("a", (0, 1), _JB),
         None,
         ("r", (2, 3), _JB), ("a", (2, 3), _JB), ("r", (2, 3), _JA), ("a", (2, 3), _JA), ("f", (2, 3), _JF),
         ("f", (4,), _JB + _JA + _JF),
         None,
         ("r", (5, 6), _JA), ("f", (5, 6), _JF), ("r", (5, 6), _JB), ("a", (5, 6), _JA), ("a", (5, 6), _JB),
         None)

_WIN = dict(
    q3=(((0, 14, 8), (14, 22, 32)), (1, 5, 9)),
    q2=(((25, 33, 32), (33, 39, 24), (39, 51, 8)), (1, 5, 9)),
    q1=(((45, 51, 24), (51, 65, 8)), (5, 5, None)),
    q0=(((66, 80, 8), (80, 88, 32)), (1, 5, 9)),
    f3=(((0, 14, 8), (14, 22, 32)), (1, 5, 9)),
    f2=(((25, 33, 32), (33, 39, 24), (39, 51, 8)), (1, 5, 9)),
    f1=(((45, 51, 24), (51, 65, 8)), (5, 9, 13)),
    f0=(((66, 68, 16), (68, 80, 8), (80, 89, 24)), (1, 5, 9)),
)
_PTRIG = (0, 1, 3, 2, 4, 5, 7, 6, 8, 9, 11, 10, 12, 13, 15, 14) + tuple(range(16, 32))


def _fwd(a, g, h, d):
    return [a + g, a - g, a + d, g + h]


def _rhs7(u, v, e, f):
    return [v - e, u - e, e + f, f - e, e + e, v, u]


class _Q:
    def __init__(self, blocks):
        self.q = list(blocks)

    def __add__(self, o):
        return _Q(a + b for a, b in zip(self.q, o.q))

    def __sub__(self, o):
        return _Q(a - b for a, b in zip(self.q, o.q))


def _scl(x, s):
    return x if s == 1.0 else x * s


def _sc(*blocks):
    return _T ** sum(_EXP[b] for b in blocks)


def _rc(Q, q):
    return 2 * (Q // 2) + q // 2, 2 * (Q % 2) + q % 2


def _ident(x):
    return x


def _after(step, t, x):
    return jnp.where(jnp.full(x.shape, step, jnp.int32) < 0, t, x)


def _split(plan):
    deep = [(i, j) for st in plan if st and st[0] == "r" for i in st[1] for j in st[2]]
    return deep, [(i, j) for i in range(7) for j in range(7) if (i, j) not in deep]


def _kernel(x0_hbm, w_hbm, b_hbm, o_hbm,
            wbuf, s_ref, s3_ref, pb_ref, m_ref, xin, ost, sp_z, sp_x, sp_b, bvm, bt_ref, bp_ref,
            sem_w, sem_in, sem_out, sem_misc,
            *, L, tm, d, ntiles, r0, plan, win, ptrig, early):
    d4 = d // 4
    r4 = tm // 4
    r8 = tm // 8
    half = tm // 2
    N = ntiles
    deep, flat = _split(plan)
    djs = sorted({j for _, j in deep})
    dot = functools.partial(jnp.dot, preferred_element_type=F32)

    ids = {}
    for name in ([(n, k) for n in "UV" for k in range(7)]
                 + [("C", Q, k) for Q in range(4) for k in range(4)]
                 + [("z", Q, k) for Q in (2, 3) for k in range(4)]):
        ids[name] = len(ids)
    nzero = len(ids)

    rw = [0, r4, None]

    def rows(base):
        if isinstance(rw[0], int):
            return slice(base + rw[0], base + rw[0] + rw[1])
        return pl.ds(pl.multiple_of(base + rw[0], 8), rw[1])

    def pieces():
        if rw[2] is not None:
            return [(0, rw[1], rw[2])]
        cut = min(max(r8 - rw[0], 0), rw[1])
        return [p for p in ((0, cut, 0), (cut, rw[1], 1)) if p[1] > p[0]]

    def scaled(x, Q, q, power):
        return jnp.concatenate([jnp.concatenate(
            [_scl(x[a:b, c * LANES:(c + 1) * LANES], _sc(Q, q, 2 * rh + c) ** power) for c in range(2)],
            axis=1) for a, b, rh in pieces()], axis=0)

    def chunked(fn, lo, n):
        def body(k, c):
            for rh in range(2):
                rw[:] = [rh * r8 + lo + k * 8, 8, rh]
                fn()
            rw[:] = [0, r4, None]
            return c
        jax.lax.fori_loop(0, n // 8, body, 0)

    def loc(name, sub):
        i = ids.setdefault(name, len(ids))
        if sub is None:
            return (i, rows(0), slice(0, d4))
        return (i, slice(sub // 2 * r8, (sub // 2 + 1) * r8), slice(sub % 2 * LANES, (sub % 2 + 1) * LANES))

    def put(name, v, sub=None):
        m_ref[loc(name, sub)] = v

    def get(name, sub=None):
        return m_ref[loc(name, sub)]

    small = {}

    def putx(name, v):
        m_ref[small.setdefault(name, len(small)), 0:r8, d4:d4 + LANES] = v

    def getx(name):
        return m_ref[small[name], 0:r8, d4:d4 + LANES]

    def putq(name, q):
        for k, v in enumerate(q.q):
            put(name + (k,), v)

    def getq(name):
        return _Q(get(name + (k,)) for k in range(4))

    def sl(Q, q):
        r, c = _rc(Q, q)
        return (rows(r * r4), slice(c * d4, (c + 1) * d4))

    def new_x(l, Q, gate, gate2):
        c = []
        for k in range(7):
            t = get((("E", k), ("P", 1, k), ("U", k), ("U", k))[Q])
            if k in (1, 5, 6):
                t = gate(t) if k == 1 else gate2(t)
            if Q > 0:
                o = get(("P", 0, k) if Q == 1 else ("V", k))
                t = t + o if Q == 2 else t - o
            c.append(t)
        f = c[1] - c[0]
        e = c[1] + c[0] + c[2] + c[3] + c[4]
        v = c[5] + c[3]
        u = c[6] - c[2]
        y = _Q([e, f, u + v + f, u - v + e])
        if l > 0:
            y = y + getq(("C", Q))
        if Q < 2 or l < L - 1:
            putq(("C", Q), y)
        if Q >= 2:
            y = y + getq(("C", 3 - Q))
        return [get(("z", Q, q)) * jnp.concatenate(
            [y.q[q][a:b] + bt_ref[l, 4 * Q + q, rh, 0:1, :] for a, b, rh in pieces()], axis=0)
            for q in range(4)]

    def emit(Q, gate, gate2, oslot):
        o = [scaled(x, Q, q, -1) for q, x in enumerate(new_x(L - 1, Q, gate, gate2))]
        for q in range(4):
            ost[(oslot,) + sl(Q, q)] = o[q].astype(ost.dtype)
        return o

    def load(Q, islot, gates):
        z = [gates[q](xin[(islot,) + sl(Q, q)].astype(F32)) for q in range(4)]
        putq(("z", Q), _Q(z))
        return [scaled(z[q], Q, q, 1) for q in range(4)]

    def operands(Q, x):
        dn = _Q(_fwd(*x))
        if Q < 2:
            putq(("D", Q), dn)
        if Q != 1:
            g = getq(("D", 1))
        if Q == 0:
            putq(("S", 0), dn + g)
            putq(("S", 1), dn - g)
        elif Q == 3:
            putq(("S", 4), dn + getq(("D", 0)))
            putq(("S", 2), g - dn)
            putq(("S", 3), g + dn)
        elif Q == 2:
            f, e = dn + g, getq(("S", 4))
            putq(("S", 5), f + e)
            putq(("S", 6), f - e)

    def stage(l, Q, gates, oslot, islot):
        if l == L - 1:
            o = emit(Q, gates[0], gates[1], oslot)
            x = load(Q, islot, [functools.partial(_after, islot, t) for t in o])
        else:
            x = new_x(l, Q, gates[0], gates[1])
        operands(Q, [gates[2](x[0]), gates[2](x[1]), x[2], x[3]])

    def w_copy(l):
        return pltpu.make_async_copy(w_hbm.at[l], wbuf.at[l, :, pl.ds(0, d)], sem_w.at[l])

    def in_copy(t, slot):
        return pltpu.make_async_copy(
            x0_hbm.at[pl.ds(pl.multiple_of(t * tm, 16), tm)], xin.at[slot], sem_in.at[slot])

    def out_copy(t, slot, lo=0, n=tm):
        return pltpu.make_async_copy(
            ost.at[slot, pl.ds(lo, n)],
            o_hbm.at[pl.ds(pl.multiple_of(t * tm + lo, 16), n)], sem_out)

    def last_top(Q, lo=0, n=half):
        cols = pl.ds(Q * (d // 2), d // 2)
        return pltpu.make_async_copy(
            ost.at[(N - 1) % 2, pl.ds(lo, n), cols],
            o_hbm.at[pl.ds((N - 1) * tm + lo, n), cols], sem_misc.at[2 + Q])

    sp_bv = sp_b.at[:, pl.ds(0, d)]
    sp_in = pltpu.make_async_copy(x0_hbm.at[pl.ds(N * tm, r0)], sp_bv, sem_misc.at[0])
    sp_out = pltpu.make_async_copy(sp_bv, o_hbm.at[pl.ds(N * tm, r0)], sem_misc.at[0])
    b_in = pltpu.make_async_copy(b_hbm, bvm, sem_misc.at[1])

    b_in.start()
    sp_in.start()

    def w_start(l, c):
        w_copy(l).start()
        return c
    jax.lax.fori_loop(0, L, w_start, 0)
    in_copy(0, 0).start()

    def zero(i, c):
        m_ref[i, :r4, :d4] = jnp.zeros((r4, d4), F32)
        pb_ref[i & 1, 0, 0, 0, 0:8, :] = jnp.zeros((8, LANES), F32)
        return c
    jax.lax.fori_loop(0, nzero, zero, 0)
    in_copy(min(1, N - 1), 1).start()

    b_in.wait()
    ball = bvm[...].astype(F32)
    cum = jnp.ones((8, d), F32)
    for l in range(L):
        bl = jnp.broadcast_to(ball[l:l + 1], (8, d))
        bp_ref[l] = bl
        cum = cum + bl
        for Q in range(4):
            for q in range(4):
                c = _rc(Q, q)[1]
                for rh in range(2):
                    rw[:] = [0, 8, rh]
                    bt_ref[l, 4 * Q + q, rh] = scaled(cum[:, c * d4:(c + 1) * d4], Q, q, 1)
    rw[:] = [0, r4, None]
    sp_in.wait()
    z0 = sp_b[:, :d].astype(F32)
    sp_z[:, :d] = z0
    sp_x[:, :d] = z0

    def layer_body(l, carry):
        w_copy(l).wait()
        xb = sp_b[:, :d]
        trig, new = [], []
        for n in range(d // LANES):
            cs = slice(n * LANES, (n + 1) * LANES)
            y1 = dot(xb[:, :d // 2], wbuf[l, :d // 2, cs]) + bp_ref[l, 0:1, cs]
            y2 = dot(xb[:, d // 2:], wbuf[l, d // 2:, cs]) + y1
            trig += [y[k * 16:(k + 1) * 16] for y in (y1, y2) for k in range(r0 // 16)]
            new.append(sp_z[:, cs] * y2 + sp_x[:, cs])
        for n in range(0, d // LANES, 2):
            cs = slice(n * LANES, (n + 2) * LANES)
            v = jnp.concatenate(new[n:n + 2], axis=1)
            sp_x[:, cs] = v
            sp_b[:, cs] = v.astype(BF16)

        per = len(trig) // (LANES // 16)

        def gated(w, st, k):
            ti = st * per + ptrig[k] * per // 32
            return _after(l, trig[ti], w) if ti >= 0 else w

        def two_levels(st, sub):
            rh, h = divmod(sub, 2)
            rr = rh * LANES + st * 16

            def blk(Q, q):
                r, c = _rc(Q, q)
                c0 = c * d4 + h * LANES
                w = wbuf[l, r * d4 + rr:r * d4 + rr + 16, c0:c0 + LANES].astype(F32)
                if q == 0:
                    w = gated(w, st, 4 * sub + Q)
                return _scl(w, 0.125 * _sc(Q, q, sub))
            wt = _fwd(*[_Q(_fwd(*[blk(Q, q) for q in range(4)])) for Q in range(4)])
            for j in range(7):
                base = [t.q[2] * 4.0 if j == 4 else _rhs7(*t.q)[j] for t in wt]
                if j in djs:
                    for a in range(4):
                        pb_ref[st % 2, djs.index(j), a, sub, 0:16, :] = base[a]
                    out = [base[2] * 4.0 if i == 4 else u + u for i, u in enumerate(_rhs7(*base))]
                else:
                    out = _rhs7(*(base if j == 4 else [b + b for b in base]))
                for i, u in enumerate(out):
                    if (i, j) in flat:
                        s_ref[l, flat.index((i, j)), h, rr:rr + 16, :] = u.astype(BF16)

        def third_level(st, n, j):
            def blk(a, sub):
                w = pb_ref[st % 2, n, a, sub, 0:16, :]
                return gated(w, st, 16 + 4 * n + a) if sub == 0 else w
            wt = [_Q(_fwd(*[blk(a, sub) for sub in range(4)])) for a in range(4)]
            for i, t in enumerate(_rhs7(*wt)):
                if (i, j) in deep:
                    for k, u in enumerate(_rhs7(*t.q)):
                        s3_ref[l, 7 * deep.index((i, j)) + k, st * 16:(st + 1) * 16, :] = u.astype(BF16)

        for st in range(LANES // 16):
            for sub in range(4):
                two_levels(st, sub)
            for n, j in enumerate(djs):
                third_level(st, n, j)
        return carry
    jax.lax.fori_loop(0, L, layer_body, 0)

    sp_out.start()
    in_copy(0, 0).wait()
    chunked(lambda: [operands(Q, load(Q, 0, [_ident] * 4)) for Q in (1, 0)], 0, r8)

    def tile_body(s, slots):
        cur, nxt, fre = slots
        in_copy(0, nxt).wait()
        in_copy(jnp.minimum(s + 2, N - 1), fre).start()
        oslot = s & 1
        tl = []
        hd = r8 // 4

        def gates(t0, key):
            segs, lags = win[key]
            n = r4 // 4
            when = [k for lo, hi, sp in segs for k in range((t0 + lo) * 24, (t0 + hi) * 24, sp)]
            when = [when[k * len(when) // n] * hd // 24 for k in range(n)]

            def one(lag):
                if lag is None:
                    return _ident
                parts = []
                for r in range(rw[0] // 8, (rw[0] + rw[1]) // 8):
                    cols = []
                    for c in range(2):
                        p, rr, cc = tl[min(when[2 * r + c] + lag, len(tl) - 1)]
                        cols.append(p[rr * 8:(rr + 1) * 8, cc * LANES:(cc + 1) * LANES])
                    parts.append(jnp.concatenate(cols, axis=1))
                return functools.partial(_after, s, jnp.concatenate(parts, axis=0))
            return [one(lag) for lag in lags]

        def lhs(i, j, sub=None):
            terms = _LHS[j]
            t = get(("S", i, terms[0][1]), sub)
            for sign, b in terms[1:]:
                t = t + get(("S", i, b), sub) if sign > 0 else t - get(("S", i, b), sub)
            return t

        def arrive(i, j, p, sub=None):
            if i < 4:
                put(("P", i, j), p, sub)
            elif i == 4:
                put(("E", j), p + get(("P", 0, j)) + get(("P", 1, j)) + get(("P", 2, j)) + get(("P", 3, j)))
            elif i == 5:
                put(("V", j), p + get(("P", 3, j), sub), sub)
            else:
                put(("U", j), p - get(("P", 2, j), sub), sub)

        def products(l, kind, outer, inner):
            ps = [(i, j) for i in outer for j in inner]

            def mul(pr, k, t):
                return dot(t.astype(BF16), s3_ref[l, 7 * deep.index(pr) + k])

            def close(pr, m0, m1, m4):
                f = m1 - m0
                putx(("e", pr), m1 + m0 + m4)
                if pr[0] > 4:
                    putx(("f", pr), f)
                arrive(*pr, f, 1)

            if kind == "f":
                for pr in ps:
                    w = jnp.concatenate([s_ref[l, flat.index(pr), h] for h in range(2)], axis=1)
                    p = dot(lhs(*pr).astype(BF16), w)
                    tl.extend((p, rr, cc) for rr in range(r4 // 8) for cc in range(2))
                    arrive(*pr, p)
            elif kind == "r":
                for r in range(3):
                    a, g, dd = (lhs(*ps[r], sub) for sub in (0, 1, 3))
                    m0, m1, m4 = mul(ps[r], 0, a + g), mul(ps[r], 1, a - g), mul(ps[r], 4, a + dd)
                    a, x = lhs(*ps[3], 0), lhs(*ps[3], 3 if r == 0 else 1)
                    mx = mul(ps[3], (4, 0, 1)[r], a - x if r == 2 else a + x)
                    tl.extend((p, rr, 0) for rr in range(r8 // 8) for p in (m0, mx))
                    close(ps[r], m0, m1, m4)
                    if r < 2:
                        putx(("m", r), mx)
                    else:
                        close(ps[3], getx(("m", 1)), mx, getx(("m", 0)))
            else:
                for pr in ps:
                    a, g, h, dd = (lhs(*pr, sub) for sub in range(4))
                    e, f = a + dd, g + h
                    m2, m3, m5, m6 = mul(pr, 2, g - dd), mul(pr, 3, g + dd), mul(pr, 5, e + f), mul(pr, 6, f - e)
                    tl.extend((p, rr, 0) for rr in range(r8 // 8) for p in (m2, m6))
                    e0 = getx(("e", pr))
                    f0 = getx(("f", pr)) if pr[0] > 4 else get(("P",) + pr, 1)
                    arrive(*pr, m2 + m3 + e0, 0)
                    arrive(*pr, (m3 - m2) + (m5 + m6) + f0, 2)
                    arrive(*pr, (m6 - m5) + e0, 3)

        for l in range(L):
            t0 = len(tl) // hd
            last = l == L - 1

            def run(lay, Q, oslot, islot):
                stage(lay, Q, gates(t0, "qf"[lay == L - 1] + str(Q)), oslot, islot)

            def splice(k):
                if k == 0:
                    run((l - 1) % L, 3, 1 - oslot, cur)
                elif k == 1:
                    run((l - 1) % L, 2, 1 - oslot, cur)
                    run(l, 1, oslot, nxt)
                    if last:
                        pl.when(s == N - 1)(last_top(1).start)
                elif not last:
                    run(l, 0, oslot, nxt)
                else:
                    rw[:] = [0, early, None]
                    run(l, 0, oslot, nxt)

                    @pl.when(s == N - 1)
                    def _():
                        last_top(0, 0, early).start()
                        last_top(0, r4, early).start()
                    rw[:] = [early, r4 - early, None]
                    run(l, 0, oslot, nxt)
                    rw[:] = [0, r4, None]

            k = 0
            for st in plan:
                if st is None:
                    splice(k)
                    k += 1
                else:
                    products(l, *st)
            if l == 0:
                @pl.when(s > 0)
                def _():
                    out_copy(s - 1, 1 - oslot).start()
                ost[oslot, 0:8, 0:LANES] = tl[-1][0][0:8].astype(ost.dtype)

        @pl.when(s > 0)
        def _():
            out_copy(0, 0).wait()
        return nxt, fre, cur
    jax.lax.fori_loop(0, N, tile_body, (0, 1, 2))

    oslot = (N - 1) % 2
    last_top(0, early, r4 - early).start()
    last_top(0, r4 + early, r4 - early).start()

    def group(g, carry):
        lo = pl.multiple_of(g * 16, 16)
        chunked(lambda: [emit(Q, _ident, _ident, oslot) for Q in (3, 2)], lo, 16)
        for rb in range(4, 8):
            out_copy(N - 1, oslot, pl.multiple_of(rb * r8 + lo, 16), 16).start()
        return carry
    jax.lax.fori_loop(0, r8 // 16, group, 0)
    in_copy(0, (N + 1) % 3).wait()
    sp_out.wait()
    last_top(1).wait()
    last_top(0).wait()
    out_copy(0, 0, 0, half).wait()
    assert len(ids) <= m_ref.shape[0] and len(small) <= m_ref.shape[0]


def _build(x0, ws, bs, *, TM=768, R0=256, early=160, plan=_PLAN, ptrig=_PTRIG, **win):
    B, D = x0.shape
    L = ws.shape[0]
    N = (B - R0) // TM
    assert R0 + N * TM == B and L >= 2 and D == 8 * LANES
    assert TM % 128 == 0 and R0 % 16 == 0 and early % 16 == 0 and early < TM // 4
    deep, flat = _split(plan)
    return pl.pallas_call(
        functools.partial(_kernel, L=L, tm=TM, d=D, ntiles=N, r0=R0, plan=plan,
                          win=dict(_WIN, **win), ptrig=ptrig, early=early),
        in_specs=[pl.BlockSpec(memory_space=pl.ANY)] * 3,
        out_specs=pl.BlockSpec(memory_space=pl.ANY),
        out_shape=jax.ShapeDtypeStruct((B, D), x0.dtype),
        scratch_shapes=[
            pltpu.VMEM((L, D, D + 2 * LANES), BF16),
            pltpu.VMEM((L, len(flat), 2, D // 4, LANES), BF16),
            pltpu.VMEM((L, 7 * len(deep), LANES, LANES), BF16),
            pltpu.VMEM((2, 7, 4, 4, 24, LANES), F32),
            pltpu.VMEM((120, TM // 4 + 8, D // 4 + LANES), F32),
            pltpu.VMEM((3, TM, D), BF16),
            pltpu.VMEM((2, TM, D), BF16),
            pltpu.VMEM((R0, D + LANES), F32),
            pltpu.VMEM((R0, D + LANES), F32),
            pltpu.VMEM((R0, D + 2 * LANES), BF16),
            pltpu.VMEM((L, D), BF16),
            pltpu.VMEM((L, 16, 2, 8, D // 4), F32),
            pltpu.VMEM((L, 8, D), F32),
            pltpu.SemaphoreType.DMA((L,)),
            pltpu.SemaphoreType.DMA((3,)),
            pltpu.SemaphoreType.DMA,
            pltpu.SemaphoreType.DMA((4,)),
        ],
        compiler_params=pltpu.CompilerParams(vmem_limit_bytes=120 * 1024 * 1024),
    )(x0, ws, bs)


@jax.jit
def pallas_standalone__dcn_v2_cross__recsys_kernel(
    x0: jax.Array,
    ws: jax.Array,
    bs: jax.Array,
):
    return _build(x0, ws, bs)
```

```python
import functools

import jax
import jax.numpy as jnp
import jax.experimental.pallas as pl
import jax.experimental.pallas.tpu as pltpu

F32 = jnp.float32
BF16 = jnp.bfloat16
LANES = 128

_T = 1.75
_EXP = (0, -1, 1, 0)
_LHS = (((1, 0),), ((1, 1),), ((1, 0), (-1, 2)), ((1, 2), (-1, 1)), ((1, 2),),
        ((1, 2), (1, 3)), ((1, 3), (-1, 2)))

_JA, _JB, _JC = (0, 1), (2, 5), (3, 6)
_PLAN = (("r", (0, 1), _JA), ("f", (0, 1), (4,)), ("r", (0, 1), _JB), ("r", (0, 1), _JC),
         ("a", (0, 1), _JA), ("a", (0, 1), _JB), ("a", (0, 1), _JC),
         None,
         ("r", (2, 3), _JB), ("a", (2, 3), _JB), ("r", (2, 3), _JC), ("a", (2, 3), _JC),
         ("r", (2, 3), _JA), ("a", (2, 3), _JA), ("f", (2, 3), (4,)), ("f", (4,), _JB + _JC + _JA + (4,)),
         None,
         ("r", (5, 6), _JA), ("f", (5, 6), (4,)), ("r", (5, 6), _JB), ("r", (5, 6), _JC),
         ("a", (5, 6), _JA), ("a", (5, 6), _JB), ("a", (5, 6), _JC),
         None)
_DEEP = [(i, j) for st in _PLAN if st and st[0] == "r" for i in st[1] for j in st[2]]
_FLAT = [(i, j) for i in range(7) for j in range(7) if (i, j) not in _DEEP]

_WIN = dict(
    q3=(((0, 2, 8), (2, 5, 6), (5, 15, 12), (15, 22, 16)), (1, 5, 11)),
    q2=(((24, 38, 16), (38, 44, 12), (44, 49, 8)), (1, 5, 9)),
    q1=(((48, 64, 8),), (1, 1, None)),
    q0=(((64, 66, 8), (66, 70, 6), (70, 79, 12), (79, 87, 24)), (1, 5, 9)),
    f3=(((0, 2, 8), (2, 5, 6), (5, 15, 12), (15, 22, 16)), (1, 5, None)),
    f2=(((24, 38, 16), (38, 44, 12), (44, 49, 8)), (1, 5, None)),
    f1=(((48, 64, 8),), (1, 1, None)),
    f0=(((64, 66, 24), (66, 70, 6), (70, 79, 12), (79, 87, 16)), (1, 5, None)),
    z1=(((38, 46, 4),), (2,)),
    z0=(((48, 64, 8),), (3,)),
    x=(((49, 62, 32),), (5, 13, 29, 21), (1, 2, 3, 4, 5)),
)
_PTRIG = (0, 0, 1, 1, 2, 2, 3, 3, 4, 4, 5, 5, 6, 6, 7, 7) + tuple(range(8, 32))


def _fwd(a, g, h, d):
    return [a + g, a - g, a + d, g + h]


def _rhs7(u, v, e, f):
    return [v - e, u - e, e + f, f - e, e + e, v, u]


class _Q:
    def __init__(self, blocks):
        self.q = list(blocks)

    def __add__(self, o):
        return _Q(a + b for a, b in zip(self.q, o.q))

    def __sub__(self, o):
        return _Q(a - b for a, b in zip(self.q, o.q))


def _scl(x, s):
    return x if s == 1.0 else x * s


def _sc(*blocks):
    return _T ** sum(_EXP[b] for b in blocks)


def _rc(Q, q):
    return 2 * (Q // 2) + q // 2, 2 * (Q % 2) + q % 2


def _ident(x):
    return x


def _after(step, t, x):
    return jnp.where(jnp.full(x.shape, step, jnp.int32) < 0, t, x)


def _kernel(x0_hbm, w_hbm, b_hbm, o_hbm,
            wbuf, s_ref, s3_ref, pb_ref, m_ref, xin, ost, sp_z, sp_x, sp_b, bvm, bt_ref, bp_ref,
            sem_w, sem_in, sem_out, sem_misc,
            *, L, tm, d, ntiles, r0, win, early):
    d4 = d // 4
    r4 = tm // 4
    r8 = tm // 8
    half = tm // 2
    N = ntiles
    dot = functools.partial(jnp.dot, preferred_element_type=F32)

    def rot(k):
        return k % 4

    def unrot(ref, k):
        r = 16 * rot(k)
        return jnp.concatenate([ref[r:], ref[:r]], axis=0) if r else ref[...]

    ids = {}
    for name in ([(n, k) for n in "UV" for k in range(7)]
                 + [("C", Q, k) for Q in range(4) for k in range(4)]
                 + [("z", Q, k) for Q in (2, 3) for k in range(4)]):
        ids[name] = len(ids)
    nzero = len(ids)

    rw = [0, r4, None]

    def rows(base):
        if isinstance(rw[0], int):
            return slice(base + rw[0], base + rw[0] + rw[1])
        return pl.ds(pl.multiple_of(base + rw[0], 8), rw[1])

    def pieces():
        if rw[2] is not None:
            return [(0, rw[1], rw[2])]
        cut = min(max(r8 - rw[0], 0), rw[1])
        return [p for p in ((0, cut, 0), (cut, rw[1], 1)) if p[1] > p[0]]

    def scaled(x, Q, q, power):
        return jnp.concatenate([jnp.concatenate(
            [_scl(x[a:b, c * LANES:(c + 1) * LANES], _sc(Q, q, 2 * rh + c) ** power) for c in range(2)],
            axis=1) for a, b, rh in pieces()], axis=0)

    def chunked(fn, lo, n):
        def body(k, c):
            for rh in range(2):
                rw[:] = [rh * r8 + lo + k * 8, 8, rh]
                fn()
            rw[:] = [0, r4, None]
            return c
        jax.lax.fori_loop(0, n // 8, body, 0)

    def loc(name, sub):
        i = ids.setdefault(name, len(ids))
        if sub is None:
            return (i, rows(0), slice(0, d4))
        return (i, slice(sub // 2 * r8, (sub // 2 + 1) * r8), slice(sub % 2 * LANES, (sub % 2 + 1) * LANES))

    def put(name, v, sub=None):
        m_ref[loc(name, sub)] = v

    def get(name, sub=None):
        return m_ref[loc(name, sub)]

    small = {}

    def putx(name, v):
        m_ref[small.setdefault(name, len(small)), 0:r8, d4:d4 + LANES] = v

    def getx(name):
        return m_ref[small[name], 0:r8, d4:d4 + LANES]

    def putq(name, q):
        for k, v in enumerate(q.q):
            put(name + (k,), v)

    def getq(name):
        return _Q(get(name + (k,)) for k in range(4))

    def sl(Q, q):
        r, c = _rc(Q, q)
        return (rows(r * r4), slice(c * d4, (c + 1) * d4))

    def new_x(l, Q, gate, gate2):
        c = []
        for k in range(7):
            t = get((("E", k), ("P", 1, k), ("U", k), ("U", k))[Q])
            if k in (1, 6):
                t = gate(t) if k == 1 else gate2(t)
            if Q > 0:
                o = get(("P", 0, k) if Q == 1 else ("V", k))
                t = t + o if Q == 2 else t - o
            c.append(t)
        f = c[1] - c[0]
        e = c[1] + c[0] + c[2] + c[3] + c[4]
        v = c[5] + c[3]
        u = c[6] - c[2]
        y = _Q([e, f, u + v + f, u - v + e])
        if l > 0:
            y = y + getq(("C", Q))
        if Q < 2 or l < L - 1:
            putq(("C", Q), y)
        if Q >= 2:
            y = y + getq(("C", 3 - Q))
        return [get(("z", Q, q)) * jnp.concatenate(
            [y.q[q][a:b] + bt_ref[l, 4 * Q + q, rh, 0:1, :] for a, b, rh in pieces()], axis=0)
            for q in range(4)]

    def emit(Q, gate, gate2, oslot):
        o = [scaled(x, Q, q, -1) for q, x in enumerate(new_x(L - 1, Q, gate, gate2))]
        for q in range(4):
            ost[(oslot,) + sl(Q, q)] = o[q].astype(ost.dtype)
        return o

    def load_z(Q, islot, gates):
        putq(("z", Q), _Q(gates[q](xin[(islot,) + sl(Q, q)].astype(F32)) for q in range(4)))

    def start(islot, gates):
        def blk(Q, q):
            x = xin[(islot,) + sl(Q, q)].astype(F32)
            return scaled(gates[Q](x) if q < 2 else x, Q, q, 1)
        a, g, h, dd = [_Q(_fwd(*[blk(Q, q) for q in range(4)])) for Q in range(4)]
        e, f = a + dd, g + h
        for i, t in enumerate([a + g, a - g, g - dd, g + dd, e, e + f, f - e]):
            putq(("A", i), t)

    def operands(Q, x):
        dn = _Q(_fwd(*x))
        if Q == 1:
            putq(("D", 1), dn)
        else:
            g = getq(("D", 1))
        if Q == 0:
            putq(("S", 0), dn + g)
            putq(("S", 1), dn - g)
        elif Q == 3:
            putq(("S", 2), g - dn)
            putq(("S", 4), getq(("S", 0)) - (g - dn))
            putq(("S", 3), g + dn)
        elif Q == 2:
            f, e = dn + g, getq(("S", 4))
            putq(("S", 5), f + e)
            putq(("S", 6), f - e)

    def stage(l, Q, gates, oslot, islot):
        if l == L - 1:
            o = emit(Q, gates[0], gates[1], oslot)
            if Q >= 2:
                load_z(Q, islot, [functools.partial(_after, islot, t) for t in o])
        else:
            x = new_x(l, Q, gates[0], gates[1])
            operands(Q, [gates[2](x[0])] + x[1:])

    def w_copy(l, slot):
        return pltpu.make_async_copy(w_hbm.at[l], wbuf.at[slot, :, pl.ds(0, d)], sem_w.at[slot])

    def in_copy(t, slot):
        return pltpu.make_async_copy(
            x0_hbm.at[pl.ds(pl.multiple_of(t * tm, 16), tm)], xin.at[slot], sem_in.at[slot])

    def out_copy(t, slot, lo=0, n=tm):
        return pltpu.make_async_copy(
            ost.at[slot, pl.ds(lo, n)],
            o_hbm.at[pl.ds(pl.multiple_of(t * tm + lo, 16), n)], sem_out)

    def last_top(Q, lo=0, n=half):
        cols = pl.ds(Q * (d // 2), d // 2)
        return pltpu.make_async_copy(
            ost.at[(N - 1) % 2, pl.ds(lo, n), cols],
            o_hbm.at[pl.ds((N - 1) * tm + lo, n), cols], sem_misc.at[2 + Q])

    sp_bv = sp_b.at[:, pl.ds(0, d)]
    sp_in = pltpu.make_async_copy(x0_hbm.at[pl.ds(N * tm, r0)], sp_bv, sem_misc.at[0])
    sp_out = pltpu.make_async_copy(sp_bv, o_hbm.at[pl.ds(N * tm, r0)], sem_misc.at[0])
    b_in = pltpu.make_async_copy(b_hbm, bvm, sem_misc.at[1])

    b_in.start()
    sp_in.start()

    def w_start(l, c):
        w_copy(l, l).start()
        return c
    jax.lax.fori_loop(0, 2, w_start, 0)

    def zero(i, c):
        m_ref[i, :r4, :d4] = jnp.zeros((r4, d4), F32)
        return c
    jax.lax.fori_loop(0, nzero, zero, 0)

    b_in.wait()
    ball = bvm[...].astype(F32)
    cum = jnp.ones((8, d), F32)
    for l in range(L):
        bl = jnp.broadcast_to(ball[l:l + 1], (8, d))
        bp_ref[l] = bl
        cum = cum + bl
        for Q in range(4):
            for q in range(4):
                c = _rc(Q, q)[1]
                for rh in range(2):
                    rw[:] = [0, 8, rh]
                    bt_ref[l, 4 * Q + q, rh] = scaled(cum[:, c * d4:(c + 1) * d4], Q, q, 1)
    rw[:] = [0, r4, None]
    sp_in.wait()
    z0 = sp_b[:, :d].astype(F32)
    sp_z[:, :d] = z0
    sp_x[:, :d] = z0

    def layer_body(l, slots):
        ws, wn, wf = slots

        @pl.when(l + 2 < L)
        def _():
            w_copy(l + 2, wf).start()

        @pl.when(l + 2 >= L)
        def _():
            in_copy(jnp.minimum(l + 2 - L, N - 1), l + 2 - L).start()
        w_copy(l, ws).wait()
        xa, xb = sp_x[:, :d // 2].astype(BF16), sp_x[:, d // 2:d].astype(BF16)
        trig, new = [], []
        for n in range(d // LANES):
            cs = slice(n * LANES, (n + 1) * LANES)
            y1 = dot(xa, wbuf[ws, :d // 2, cs]) + bp_ref[l, 0:1, cs]
            y2 = dot(xb, wbuf[ws, d // 2:, cs]) + y1
            trig += [y[k * 16:(k + 1) * 16] for y in (y1, y2) for k in range(r0 // 16)]
            new.append(sp_z[:, cs] * y2 + sp_x[:, cs])
        for n in range(d // LANES):
            sp_x[:, n * LANES:(n + 1) * LANES] = new[n]

        per = len(trig) // (LANES // 16)

        chain = []

        def gated(w, st, k):
            ti = (st * per + _PTRIG[k] * per // 32) * 33 // 32 - per // 4
            if ti >= 0:
                return _after(l, trig[ti], w)
            return _after(l, chain[-1], w) if chain else w

        def two_levels(st, sub):
            rh, h = divmod(sub, 2)
            rr = rh * LANES + st * 16

            def blk(Q, q):
                r, c = _rc(Q, q)
                c0 = c * d4 + h * LANES
                w = wbuf[ws, r * d4 + rr:r * d4 + rr + 16, c0:c0 + LANES].astype(F32)
                if q == 0:
                    w = gated(w, st, 4 * sub + Q)
                return _scl(w, 0.125 * _sc(Q, q, sub))
            inner = {}
            for Q in (0, 1, 3, 2):
                inner[Q] = _Q(_fwd(*[blk(Q, q) for q in range(4)]))
                chain.append(inner[Q].q[2] if Q in (0, 2) else inner[Q].q[2] + inner[0].q[2])
            wt = _fwd(*[inner[Q] for Q in range(4)])
            chain.append(wt[3].q[2])
            for a in range(4):
                for b in range(4):
                    pb_ref[st % 2, b, a, sub, 0:16, :] = wt[a].q[b]
            e4 = [x * 4.0 for x in wt[2].q]
            out = {(4, j): u for j, u in enumerate(_rhs7(*e4))}
            col = [e4[2] if a == 2 else wt[a].q[2] * 4.0 for a in range(4)]
            out.update({(i, 4): u for i, u in enumerate(_rhs7(*col))})
            for pr in _FLAT:
                r2 = (rr + 16 * rot(_FLAT.index(pr))) % d4
                s_ref[l, _FLAT.index(pr), h, r2:r2 + 16, :] = out[pr].astype(BF16)

        def third_level(st, n, j):
            par = st % 2 + (l >> (16 + n))

            def blk(a, sub):
                w = _rhs7(*[pb_ref[par, b, a, sub, 0:16, :] for b in range(4)])[j]
                if sub == 0:
                    w = jnp.concatenate([gated(w, st, 16 + 4 * n + a)[:8], w[8:]], axis=0)
                return w
            wt = [_Q(_fwd(*[blk(a, sub) for sub in range(4)])) for a in range(4)]
            for i, t in enumerate(_rhs7(*wt)):
                if i != 4:
                    for k, u in enumerate(_rhs7(*t.q)):
                        t3 = 7 * _DEEP.index((i, j)) + k
                        r2 = (st + rot(t3)) % (LANES // 16) * 16
                        s3_ref[l, t3, r2:r2 + 16, :] = u.astype(BF16)

        for st in range(LANES // 16):
            for sub in range(4):
                two_levels(st, sub)
            for n, j in enumerate((0, 1, 2, 3, 5, 6)):
                third_level(st, n, j)
        return wn, wf, ws
    jax.lax.fori_loop(0, L, layer_body, (0, 1, 2))

    sp_b[:, :d] = sp_x[:, :d].astype(BF16)
    sp_out.start()
    in_copy(0, 0).wait()
    chunked(lambda: start(0, [_ident] * 4), 0, r8)

    def tile_body(s, slots):
        cur, nxt, fre = slots
        in_copy(0, nxt).wait()
        in_copy(jnp.minimum(s + 2, N - 1), fre).start()
        oslot = s & 1
        tl = []
        hd = r8 // 4

        def gates(t0, key):
            segs, lags = win[key]
            n = r4 // 4
            when = [k for lo, hi, sp in segs for k in range((t0 + lo) * 24, (t0 + hi) * 24, sp)]
            when = [when[k * len(when) // n] * hd // 24 for k in range(n)]

            def one(lag):
                if lag is None:
                    return _ident
                parts = []
                for r in range(rw[0] // 8, (rw[0] + rw[1]) // 8):
                    cols = []
                    for c in range(2):
                        p, rr, cc = tl[min(when[2 * r + c] + lag, len(tl) - 1)]
                        cols.append(p[rr * 8:(rr + 1) * 8, cc * LANES:(cc + 1) * LANES])
                    parts.append(jnp.concatenate(cols, axis=1))
                return functools.partial(_after, s, jnp.concatenate(parts, axis=0))
            return [one(lag) for lag in lags]

        src = ["A"]

        def lhs(i, j, sub=None):
            terms = _LHS[j]
            t = get((src[0], i, terms[0][1]), sub)
            for sign, b in terms[1:]:
                t = t + get((src[0], i, b), sub) if sign > 0 else t - get((src[0], i, b), sub)
            return t

        def arrive(i, j, p, sub=None):
            if i < 4:
                put(("P", i, j), p, sub)
            elif i == 4:
                put(("E", j), p + get(("P", 0, j)) + get(("P", 1, j)) + get(("P", 2, j)) + get(("P", 3, j)))
            elif i == 5:
                put(("V", j), p + get(("P", 3, j), sub), sub)
            else:
                put(("U", j), p - get(("P", 2, j), sub), sub)

        def products(l, kind, outer, inner):
            ps = [(i, j) for i in outer for j in inner]

            def mul(pr, k, t):
                t3 = 7 * _DEEP.index(pr) + k
                return dot(t.astype(BF16), unrot(s3_ref.at[l, t3], t3))

            def close(pr, m0, m1, m4):
                f = m1 - m0
                putx(("e", pr), m1 + m0 + m4)
                if pr[0] > 4:
                    putx(("f", pr), f)
                arrive(*pr, f, 1)

            if kind == "f":
                for pr in ps:
                    w = jnp.concatenate([unrot(s_ref.at[l, _FLAT.index(pr), h], _FLAT.index(pr)) for h in range(2)], axis=1)
                    p = dot(lhs(*pr).astype(BF16), w)
                    tl.extend((p, rr, cc) for rr in range(r4 // 8) for cc in range(2))
                    arrive(*pr, p)
            elif kind == "r":
                for r in range(3):
                    a, g, dd = (lhs(*ps[r], sub) for sub in (0, 1, 3))
                    m0, m1, m4 = mul(ps[r], 0, a + g), mul(ps[r], 1, a - g), mul(ps[r], 4, a + dd)
                    a, x = lhs(*ps[3], 0), lhs(*ps[3], 3 if r == 0 else 1)
                    mx = mul(ps[3], (4, 0, 1)[r], a - x if r == 2 else a + x)
                    tl.extend((p, rr, 0) for rr in range(r8 // 8) for p in (m0, mx))
                    close(ps[r], m0, m1, m4)
                    if r < 2:
                        putx(("m", r), mx)
                    else:
                        close(ps[3], getx(("m", 1)), mx, getx(("m", 0)))
            else:
                for pr in ps:
                    a, g, h, dd = (lhs(*pr, sub) for sub in range(4))
                    e, f = a + dd, g + h
                    m2, m3, m5, m6 = mul(pr, 2, g - dd), mul(pr, 3, g + dd), mul(pr, 5, e + f), mul(pr, 6, f - e)
                    tl.extend((p, rr, 0) for rr in range(r8 // 8) for p in (m2, m6))
                    e0 = getx(("e", pr))
                    f0 = getx(("f", pr)) if pr[0] > 4 else get(("P",) + pr, 1)
                    arrive(*pr, m2 + m3 + e0, 0)
                    arrive(*pr, (m3 - m2) + (m5 + m6) + f0, 2)
                    arrive(*pr, (m6 - m5) + e0, 3)

        for l in range(L):
            t0 = len(tl) // hd
            last = l == L - 1
            src[0] = "AS"[l > 0]

            def run(lay, Q, oslot, islot):
                stage(lay, Q, gates(t0, "qf"[lay == L - 1] + str(Q)), oslot, islot)

            def splice(k):
                if k == 0:
                    run((l - 1) % L, 3, 1 - oslot, cur)
                elif k == 1:
                    run((l - 1) % L, 2, 1 - oslot, cur)
                    if l == 0:
                        load_z(1, cur, gates(t0, "z1") * 4)
                        load_z(0, cur, gates(t0, "z0") * 4)
                    run(l, 1, oslot, nxt)
                    if last:
                        pl.when(s == N - 1)(last_top(1).start)
                elif not last:
                    run(l, 0, oslot, nxt)
                else:
                    rw[:] = [0, early, None]
                    run(l, 0, oslot, nxt)

                    @pl.when(s == N - 1)
                    def _():
                        last_top(0, 0, early).start()
                        last_top(0, r4, early).start()
                    rw[:] = [early, r4 - early, None]
                    run(l, 0, oslot, nxt)
                    rw[:] = [0, r4, None]

            k = 0
            for st in _PLAN:
                if st is None:
                    splice(k)
                    k += 1
                else:
                    products(l, *st)
            if l == 0:
                @pl.when(s > 0)
                def _():
                    out_copy(s - 1, 1 - oslot).start()
                ost[oslot, 0:8, 0:LANES] = tl[-1][0][0:8].astype(ost.dtype)

        per = len(tl) // hd // L
        segs, lags, lays = win["x"]
        win["xx"] = (tuple((lo + k * per, hi + k * per, sp) for k in lays for lo, hi, sp in segs), lags)
        start(nxt, gates(0, "xx"))

        @pl.when(s > 0)
        def _():
            out_copy(0, 0).wait()
        return nxt, fre, cur
    jax.lax.fori_loop(0, N, tile_body, (0, 1, 2))

    oslot = (N - 1) % 2
    last_top(0, early, r4 - early).start()
    last_top(0, r4 + early, r4 - early).start()

    def group(g, carry):
        lo = pl.multiple_of(g * 16, 16)
        chunked(lambda: [emit(Q, _ident, _ident, oslot) for Q in (3, 2)], lo, 16)
        for rb in range(4, 8):
            out_copy(N - 1, oslot, pl.multiple_of(rb * r8 + lo, 16), 16).start()
        return carry
    jax.lax.fori_loop(0, r8 // 16, group, 0)
    in_copy(0, (N + 1) % 3).wait()
    sp_out.wait()
    last_top(1).wait()
    last_top(0).wait()
    out_copy(0, 0, 0, half).wait()
    assert len(ids) <= m_ref.shape[0] and len(small) <= m_ref.shape[0]


def _build(x0, ws, bs, *, TM=768, R0=256, early=160, **win):
    B, D = x0.shape
    L = ws.shape[0]
    N = (B - R0) // TM
    assert R0 + N * TM == B and L >= 2 and D == 8 * LANES
    assert TM % 128 == 0 and R0 % 16 == 0 and early % 16 == 0 and early < TM // 4
    return pl.pallas_call(
        functools.partial(_kernel, L=L, tm=TM, d=D, ntiles=N, r0=R0, win=dict(_WIN, **win), early=early),
        in_specs=[pl.BlockSpec(memory_space=pl.ANY)] * 3,
        out_specs=pl.BlockSpec(memory_space=pl.ANY),
        out_shape=jax.ShapeDtypeStruct((B, D), x0.dtype),
        scratch_shapes=[
            pltpu.VMEM((3, D, D + 2 * LANES), BF16),
            pltpu.VMEM((L, len(_FLAT), 2, D // 4, LANES), BF16),
            pltpu.VMEM((L, 7 * len(_DEEP), LANES, LANES), BF16),
            pltpu.VMEM((2, 4, 4, 5, 24, LANES), F32),
            pltpu.VMEM((144, TM // 4 + 8, D // 4 + LANES), F32),
            pltpu.VMEM((3, TM, D), BF16),
            pltpu.VMEM((2, TM, D), BF16),
            pltpu.VMEM((R0, D + LANES), F32),
            pltpu.VMEM((R0, D + LANES), F32),
            pltpu.VMEM((R0, D + 2 * LANES), BF16),
            pltpu.VMEM((L, D), BF16),
            pltpu.VMEM((L, 16, 2, 8, D // 4), F32),
            pltpu.VMEM((L, 8, D), F32),
            pltpu.SemaphoreType.DMA((3,)),
            pltpu.SemaphoreType.DMA((3,)),
            pltpu.SemaphoreType.DMA,
            pltpu.SemaphoreType.DMA((4,)),
        ],
        compiler_params=pltpu.CompilerParams(vmem_limit_bytes=126 * 1024 * 1024),
    )(x0, ws, bs)


@jax.jit
def pallas_standalone__dcn_v2_cross__recsys_kernel(
    x0: jax.Array,
    ws: jax.Array,
    bs: jax.Array,
):
    return _build(x0, ws, bs)
```

```python
import functools

import jax
import jax.numpy as jnp
import jax.experimental.pallas as pl
import jax.experimental.pallas.tpu as pltpu

F32 = jnp.float32
BF16 = jnp.bfloat16
LANES = 128

_T = 1.75
_EXP = (0, -1, 1, 0)
_LHS = (((1, 0),), ((1, 1),), ((1, 0), (-1, 2)), ((1, 2), (-1, 1)), ((1, 2),),
        ((1, 2), (1, 3)), ((1, 3), (-1, 2)))

_JA, _JB, _JC = (0, 1), (2, 5), (3, 6)
_PLAN = (("r", (0, 1), _JA), ("f", (0, 1), (4,)), ("r", (0, 1), _JB), ("r", (0, 1), _JC),
         ("a", (0, 1), _JA), ("a", (0, 1), _JB), ("a", (0, 1), _JC),
         None,
         ("r", (2, 3), _JB), ("a", (2, 3), _JB), ("r", (2, 3), _JC), ("a", (2, 3), _JC),
         ("r", (2, 3), _JA), ("a", (2, 3), _JA), ("f", (2, 3), (4,)), ("f", (4,), _JB + _JC + _JA + (4,)),
         None,
         ("r", (5, 6), _JA), ("f", (5, 6), (4,)), ("r", (5, 6), _JB), ("r", (5, 6), _JC),
         ("a", (5, 6), _JA), ("a", (5, 6), _JB), ("a", (5, 6), _JC),
         None)
_DEEP = [(i, j) for st in _PLAN if st and st[0] == "r" for i in st[1] for j in st[2]]
_FLAT = [(i, j) for i in range(7) for j in range(7) if (i, j) not in _DEEP]

_WIN = dict(
    q3=(((0, 1, 8), (1, 4, 6), (4, 15, 12), (15, 22, 16)), (5, 7, 15)),
    q2=(((24, 38, 16), (38, 44, 12), (44, 49, 8)), (1, 5, 9)),
    q1=(((48, 64, 8),), (1, 1, None)),
    q0=(((64, 66, 8), (66, 70, 6), (70, 79, 12), (79, 87, 24)), (1, 5, 9)),
    f3=(((0, 3, 8), (3, 5, 6), (5, 15, 12), (15, 22, 16)), (5, 9, None)),
    f2=(((24, 36, 16), (36, 44, 12), (44, 49, 8)), (1, 5, None)),
    f1=(((47, 63, 8),), (1, 1, None)),
    f0=(((64, 66, 24), (66, 70, 6), (70, 79, 12), (79, 87, 16)), (1, 9, None)),
    z1=(((38, 46, 4),), (4,)),
    z0=(((47, 63, 8),), (1,)),
    x=(((49, 62, 32),), (5, 13, 29, 21), (1, 2, 3, 4, 5)),
)
_PTRIG = (0, 0, 1, 1, 2, 2, 3, 3, 4, 4, 5, 5, 6, 6, 7, 7) + tuple(range(8, 32))


def _fwd(a, g, h, d):
    return [a + g, a - g, a + d, g + h]


def _rhs7(u, v, e, f):
    return [v - e, u - e, e + f, f - e, e + e, v, u]


class _Q:
    def __init__(self, blocks):
        self.q = list(blocks)

    def __add__(self, o):
        return _Q(a + b for a, b in zip(self.q, o.q))

    def __sub__(self, o):
        return _Q(a - b for a, b in zip(self.q, o.q))


def _scl(x, s):
    return x if s == 1.0 else x * s


def _sc(*blocks):
    return _T ** sum(_EXP[b] for b in blocks)


def _rc(Q, q):
    return 2 * (Q // 2) + q // 2, 2 * (Q % 2) + q % 2


def _ident(x):
    return x


def _after(step, t, x):
    return jnp.where(jnp.full(x.shape, step, jnp.int32) < 0, t, x)


def _kernel(x0_hbm, w_hbm, b_hbm, o_hbm,
            wbuf, s_ref, s3_ref, pb_ref, m_ref, xin, ost, sp_z, sp_x, sp_b, bvm, bt_ref, bp_ref,
            sem_w, sem_in, sem_out, sem_misc,
            *, L, tm, d, ntiles, r0, win, early):
    d4 = d // 4
    r4 = tm // 4
    r8 = tm // 8
    half = tm // 2
    N = ntiles
    dot = functools.partial(jnp.dot, preferred_element_type=F32)

    def rot(k):
        return k % 4

    def unrot(ref, k):
        r = 16 * rot(k)
        return jnp.concatenate([ref[r:], ref[:r]], axis=0) if r else ref[...]

    ids = {}
    for name in ([(n, k) for n in "UV" for k in range(7)]
                 + [("C", Q, k) for Q in range(4) for k in range(4)]
                 + [("z", Q, k) for Q in (2, 3) for k in range(4)]):
        ids[name] = len(ids)
    nzero = len(ids)

    rw = [0, r4, None]

    def rows(base):
        if isinstance(rw[0], int):
            return slice(base + rw[0], base + rw[0] + rw[1])
        return pl.ds(pl.multiple_of(base + rw[0], 8), rw[1])

    def pieces():
        if rw[2] is not None:
            return [(0, rw[1], rw[2])]
        cut = min(max(r8 - rw[0], 0), rw[1])
        return [p for p in ((0, cut, 0), (cut, rw[1], 1)) if p[1] > p[0]]

    def scaled(x, Q, q, power):
        return jnp.concatenate([jnp.concatenate(
            [_scl(x[a:b, c * LANES:(c + 1) * LANES], _sc(Q, q, 2 * rh + c) ** power) for c in range(2)],
            axis=1) for a, b, rh in pieces()], axis=0)

    def chunked(fn, lo, n):
        def body(k, c):
            for rh in range(2):
                rw[:] = [rh * r8 + lo + k * 8, 8, rh]
                fn()
            rw[:] = [0, r4, None]
            return c
        jax.lax.fori_loop(0, n // 8, body, 0)

    def loc(name, sub):
        i = ids.setdefault(name, len(ids))
        if sub is None:
            return (i, rows(0), slice(0, d4))
        return (i, slice(sub // 2 * r8, (sub // 2 + 1) * r8), slice(sub % 2 * LANES, (sub % 2 + 1) * LANES))

    def put(name, v, sub=None):
        m_ref[loc(name, sub)] = v

    def get(name, sub=None):
        return m_ref[loc(name, sub)]

    small = {}

    def putx(name, v):
        m_ref[small.setdefault(name, len(small)), 0:r8, d4:d4 + LANES] = v

    def getx(name):
        return m_ref[small[name], 0:r8, d4:d4 + LANES]

    def putq(name, q):
        for k, v in enumerate(q.q):
            put(name + (k,), v)

    def getq(name):
        return _Q(get(name + (k,)) for k in range(4))

    def sl(Q, q):
        r, c = _rc(Q, q)
        return (rows(r * r4), slice(c * d4, (c + 1) * d4))

    def new_x(l, Q, gate, gate2):
        c = []
        for k in range(7):
            t = get((("E", k), ("P", 1, k), ("U", k), ("U", k))[Q])
            if k in (1, 6):
                t = gate(t) if k == 1 else gate2(t)
            if Q > 0:
                o = get(("P", 0, k) if Q == 1 else ("V", k))
                t = t + o if Q == 2 else t - o
            c.append(t)
        f = c[1] - c[0]
        e = c[1] + c[0] + c[2] + c[3] + c[4]
        v = c[5] + c[3]
        u = c[6] - c[2]
        y = _Q([e, f, u + v + f, u - v + e])
        if l > 0:
            y = y + getq(("C", Q))
        if Q < 2 or l < L - 1:
            putq(("C", Q), y)
        if Q >= 2:
            y = y + getq(("C", 3 - Q))
        return [get(("z", Q, q)) * jnp.concatenate(
            [y.q[q][a:b] + bt_ref[l, 4 * Q + q, rh, 0:1, :] for a, b, rh in pieces()], axis=0)
            for q in range(4)]

    def emit(Q, gate, gate2, oslot):
        o = [scaled(x, Q, q, -1) for q, x in enumerate(new_x(L - 1, Q, gate, gate2))]
        for q in range(4):
            ost[(oslot,) + sl(Q, q)] = o[q].astype(ost.dtype)
        return o

    def load_z(Q, islot, gates):
        putq(("z", Q), _Q(gates[q](xin[(islot,) + sl(Q, q)].astype(F32)) for q in range(4)))

    def start(islot, gates):
        def blk(Q, q):
            x = xin[(islot,) + sl(Q, q)].astype(F32)
            return scaled(gates[Q](x) if q < 2 else x, Q, q, 1)
        a, g, h, dd = [_Q(_fwd(*[blk(Q, q) for q in range(4)])) for Q in range(4)]
        e, f = a + dd, g + h
        for i, t in enumerate([a + g, a - g, g - dd, g + dd, e, e + f, f - e]):
            putq(("A", i), t)

    def operands(Q, x):
        dn = _Q(_fwd(*x))
        if Q == 1:
            putq(("D", 1), dn)
        else:
            g = getq(("D", 1))
        if Q == 0:
            putq(("S", 0), dn + g)
            putq(("S", 1), dn - g)
        elif Q == 3:
            putq(("S", 2), g - dn)
            putq(("S", 4), getq(("S", 0)) - (g - dn))
            putq(("S", 3), g + dn)
        elif Q == 2:
            f, e = dn + g, getq(("S", 4))
            putq(("S", 5), f + e)
            putq(("S", 6), f - e)

    def stage(l, Q, gates, oslot, islot):
        if l == L - 1:
            o = emit(Q, gates[0], gates[1], oslot)
            if Q >= 2:
                load_z(Q, islot, [functools.partial(_after, islot, t) for t in o])
        else:
            x = new_x(l, Q, gates[0], gates[1])
            operands(Q, [gates[2](x[0])] + x[1:])

    def w_copy(l, slot):
        return pltpu.make_async_copy(w_hbm.at[l], wbuf.at[slot, :, pl.ds(0, d)], sem_w.at[slot])

    def in_copy(t, slot):
        return pltpu.make_async_copy(
            x0_hbm.at[pl.ds(pl.multiple_of(t * tm, 16), tm)], xin.at[slot], sem_in.at[slot])

    def out_copy(t, slot, lo=0, n=tm):
        return pltpu.make_async_copy(
            ost.at[slot, pl.ds(lo, n)],
            o_hbm.at[pl.ds(pl.multiple_of(t * tm + lo, 16), n)], sem_out)

    def last_top(Q, lo=0, n=half):
        cols = pl.ds(Q * (d // 2), d // 2)
        return pltpu.make_async_copy(
            ost.at[(N - 1) % 2, pl.ds(lo, n), cols],
            o_hbm.at[pl.ds((N - 1) * tm + lo, n), cols], sem_misc.at[2 + Q])

    sp_bv = sp_b.at[:, pl.ds(0, d)]
    sp_in = pltpu.make_async_copy(x0_hbm.at[pl.ds(N * tm, r0)], sp_bv, sem_misc.at[0])
    sp_out = pltpu.make_async_copy(sp_bv, o_hbm.at[pl.ds(N * tm, r0)], sem_misc.at[0])
    b_in = pltpu.make_async_copy(b_hbm, bvm, sem_misc.at[1])

    b_in.start()
    sp_in.start()

    def w_start(l, c):
        w_copy(l, l).start()
        return c
    jax.lax.fori_loop(0, 2, w_start, 0)

    def zero(i, c):
        m_ref[i, :r4, :d4] = jnp.zeros((r4, d4), F32)
        return c
    jax.lax.fori_loop(0, nzero, zero, 0)

    b_in.wait()
    ball = bvm[...].astype(F32)
    cum = jnp.ones((8, d), F32)
    for l in range(L):
        bl = jnp.broadcast_to(ball[l:l + 1], (8, d))
        bp_ref[l] = bl
        cum = cum + bl
        for Q in range(4):
            for q in range(4):
                c = _rc(Q, q)[1]
                for rh in range(2):
                    rw[:] = [0, 8, rh]
                    bt_ref[l, 4 * Q + q, rh] = scaled(cum[:, c * d4:(c + 1) * d4], Q, q, 1)
    rw[:] = [0, r4, None]
    sp_in.wait()
    z0 = sp_b[:, :d].astype(F32)
    sp_z[:, :d] = z0
    sp_x[:, :d] = z0

    def layer_body(l, slots):
        ws, wn, wf = slots

        @pl.when(l + 2 < L)
        def _():
            w_copy(l + 2, wf).start()

        @pl.when(l + 2 >= L)
        def _():
            in_copy(jnp.minimum(l + 2 - L, N - 1), l + 2 - L).start()
        w_copy(l, ws).wait()
        xa, xb = sp_x[:, :d // 2].astype(BF16), sp_x[:, d // 2:d].astype(BF16)
        trig, new = [], []
        for n in range(d // LANES):
            cs = slice(n * LANES, (n + 1) * LANES)
            y1 = dot(xa, wbuf[ws, :d // 2, cs]) + bp_ref[l, 0:1, cs]
            y2 = dot(xb, wbuf[ws, d // 2:, cs]) + y1
            trig += [y[k * 16:(k + 1) * 16] for y in (y1, y2) for k in range(r0 // 16)]
            new.append(sp_z[:, cs] * y2 + sp_x[:, cs])
        for n in range(d // LANES):
            sp_x[:, n * LANES:(n + 1) * LANES] = new[n]

        per = len(trig) // (LANES // 16)
        chain = []

        def gated(w, st, k):
            ti = (st * per + _PTRIG[k] * per // 32) * 33 // 32 - per // 4
            if ti >= 0:
                return _after(l, trig[ti], w)
            return _after(l, chain[-1], w) if chain else w

        def two_levels(st, sub):
            rh, h = divmod(sub, 2)
            rr = rh * LANES + st * 16

            def blk(Q, q):
                r, c = _rc(Q, q)
                c0 = c * d4 + h * LANES
                w = wbuf[ws, r * d4 + rr:r * d4 + rr + 16, c0:c0 + LANES].astype(F32)
                if q == 0:
                    w = gated(w, st, 4 * sub + Q)
                return _scl(w, 0.125 * _sc(Q, q, sub))
            inner = {}
            for Q in (0, 1, 3, 2):
                inner[Q] = _Q(_fwd(*[blk(Q, q) for q in range(4)]))
                chain.append(inner[Q].q[2] if Q in (0, 2) else inner[Q].q[2] + inner[0].q[2])
            wt = _fwd(*[inner[Q] for Q in range(4)])
            chain.append(wt[3].q[2])
            for a in range(4):
                for b in range(4):
                    pb_ref[st % 2, b, a, sub, 0:16, :] = wt[a].q[b]
            e4 = [x * 4.0 for x in wt[2].q]
            out = {(4, j): u for j, u in enumerate(_rhs7(*e4))}
            col = [e4[2] if a == 2 else wt[a].q[2] * 4.0 for a in range(4)]
            out.update({(i, 4): u for i, u in enumerate(_rhs7(*col))})
            for pr in _FLAT:
                r2 = (rr + 16 * rot(_FLAT.index(pr))) % d4
                s_ref[l, _FLAT.index(pr), h, r2:r2 + 16, :] = out[pr].astype(BF16)

        def third_level(st, n, j):
            par = st % 2 + (l >> (16 + n))

            def blk(a, sub):
                w = _rhs7(*[pb_ref[par, b, a, sub, 0:16, :] for b in range(4)])[j]
                if sub == 0:
                    w = jnp.concatenate([gated(w, st, 16 + 4 * n + a)[:8], w[8:]], axis=0)
                return w
            wt = [_Q(_fwd(*[blk(a, sub) for sub in range(4)])) for a in range(4)]
            for i, t in enumerate(_rhs7(*wt)):
                if i != 4:
                    for k, u in enumerate(_rhs7(*t.q)):
                        t3 = 7 * _DEEP.index((i, j)) + k
                        r2 = (st + rot(t3)) % (LANES // 16) * 16
                        s3_ref[l, t3, r2:r2 + 16, :] = u.astype(BF16)

        for st in range(LANES // 16):
            for sub in range(4):
                two_levels(st, sub)
            for n, j in enumerate((0, 1, 2, 3, 5, 6)):
                third_level(st, n, j)
        return wn, wf, ws
    jax.lax.fori_loop(0, L, layer_body, (0, 1, 2))

    sp_b[:, :d] = sp_x[:, :d].astype(BF16)
    sp_out.start()
    in_copy(0, 0).wait()
    chunked(lambda: start(0, [_ident] * 4), 0, r8)

    def tile_body(s, slots):
        cur, nxt, fre = slots
        in_copy(0, nxt).wait()
        in_copy(jnp.minimum(s + 2, N - 1), fre).start()
        oslot = s & 1
        tl = []
        hd = r8 // 4

        def gates(t0, key):
            segs, lags = win[key]
            n = r4 // 4
            when = [k for lo, hi, sp in segs for k in range((t0 + lo) * 24, (t0 + hi) * 24, sp)]
            when = [when[k * len(when) // n] * hd // 24 for k in range(n)]

            def one(lag):
                if lag is None:
                    return _ident
                parts = []
                for r in range(rw[0] // 8, (rw[0] + rw[1]) // 8):
                    cols = []
                    for c in range(2):
                        p, rr, cc = tl[min(when[2 * r + c] + lag, len(tl) - 1)]
                        cols.append(p[rr * 8:(rr + 1) * 8, cc * LANES:(cc + 1) * LANES])
                    parts.append(jnp.concatenate(cols, axis=1))
                return functools.partial(_after, s, jnp.concatenate(parts, axis=0))
            return [one(lag) for lag in lags]

        src = ["A"]

        def lhs(i, j, sub=None):
            terms = _LHS[j]
            t = get((src[0], i, terms[0][1]), sub)
            for sign, b in terms[1:]:
                t = t + get((src[0], i, b), sub) if sign > 0 else t - get((src[0], i, b), sub)
            return t

        def arrive(i, j, p, sub=None):
            if i < 4:
                put(("P", i, j), p, sub)
            elif i == 4:
                put(("E", j), p + get(("P", 0, j)) + get(("P", 1, j)) + get(("P", 2, j)) + get(("P", 3, j)))
            elif i == 5:
                put(("V", j), p + get(("P", 3, j), sub), sub)
            else:
                put(("U", j), p - get(("P", 2, j), sub), sub)

        def products(l, kind, outer, inner):
            ps = [(i, j) for i in outer for j in inner]

            def mul(pr, k, t):
                t3 = 7 * _DEEP.index(pr) + k
                return dot(t.astype(BF16), unrot(s3_ref.at[l, t3], t3))

            def close(pr, m0, m1, m4):
                f = m1 - m0
                putx(("e", pr), m1 + m0 + m4)
                if pr[0] > 4:
                    putx(("f", pr), f)
                arrive(*pr, f, 1)

            if kind == "f":
                for pr in ps:
                    k = _FLAT.index(pr)
                    w = jnp.concatenate([unrot(s_ref.at[l, k, h], k) for h in range(2)], axis=1)
                    p = dot(lhs(*pr).astype(BF16), w)
                    tl.extend((p, rr, cc) for rr in range(r4 // 8) for cc in range(2))
                    arrive(*pr, p)
            elif kind == "r":
                for r in range(3):
                    a, g, dd = (lhs(*ps[r], sub) for sub in (0, 1, 3))
                    m0, m1, m4 = mul(ps[r], 0, a + g), mul(ps[r], 1, a - g), mul(ps[r], 4, a + dd)
                    a, x = lhs(*ps[3], 0), lhs(*ps[3], 3 if r == 0 else 1)
                    mx = mul(ps[3], (4, 0, 1)[r], a - x if r == 2 else a + x)
                    tl.extend((p, rr, 0) for rr in range(r8 // 8) for p in (m0, mx))
                    close(ps[r], m0, m1, m4)
                    if r < 2:
                        putx(("m", r), mx)
                    else:
                        close(ps[3], getx(("m", 1)), mx, getx(("m", 0)))
            else:
                for pr in ps:
                    a, g, h, dd = (lhs(*pr, sub) for sub in range(4))
                    e, f = a + dd, g + h
                    m2, m3, m5, m6 = mul(pr, 2, g - dd), mul(pr, 3, g + dd), mul(pr, 5, e + f), mul(pr, 6, f - e)
                    tl.extend((p, rr, 0) for rr in range(r8 // 8) for p in (m2, m6))
                    e0 = getx(("e", pr))
                    f0 = getx(("f", pr)) if pr[0] > 4 else get(("P",) + pr, 1)
                    arrive(*pr, m2 + m3 + e0, 0)
                    arrive(*pr, (m3 - m2) + (m5 + m6) + f0, 2)
                    arrive(*pr, (m6 - m5) + e0, 3)

        for l in range(L):
            t0 = len(tl) // hd
            last = l == L - 1
            src[0] = "AS"[l > 0]

            def run(lay, Q, oslot, islot):
                stage(lay, Q, gates(t0, "qf"[lay == L - 1] + str(Q)), oslot, islot)

            def splice(k):
                if k == 0:
                    run((l - 1) % L, 3, 1 - oslot, cur)
                elif k == 1:
                    run((l - 1) % L, 2, 1 - oslot, cur)
                    if l == 0:
                        load_z(1, cur, gates(t0, "z1") * 4)
                        load_z(0, cur, gates(t0, "z0") * 4)
                    run(l, 1, oslot, nxt)
                    if last:
                        pl.when(s == N - 1)(last_top(1).start)
                elif not last:
                    run(l, 0, oslot, nxt)
                else:
                    rw[:] = [0, early, None]
                    run(l, 0, oslot, nxt)

                    @pl.when(s == N - 1)
                    def _():
                        last_top(0, 0, early).start()
                        last_top(0, r4, early).start()
                    rw[:] = [early, r4 - early, None]
                    run(l, 0, oslot, nxt)
                    rw[:] = [0, r4, None]

            k = 0
            for st in _PLAN:
                if st is None:
                    splice(k)
                    k += 1
                else:
                    products(l, *st)
            if l == 0:
                @pl.when(s > 0)
                def _():
                    out_copy(s - 1, 1 - oslot).start()
                ost[oslot, 0:8, 0:LANES] = tl[-1][0][0:8].astype(ost.dtype)

        per = len(tl) // hd // L
        segs, lags, lays = win["x"]
        win["xx"] = (tuple((lo + k * per, hi + k * per, sp) for k in lays for lo, hi, sp in segs), lags)
        start(nxt, gates(0, "xx"))

        @pl.when(s > 0)
        def _():
            out_copy(0, 0).wait()
        return nxt, fre, cur
    jax.lax.fori_loop(0, N, tile_body, (0, 1, 2))

    oslot = (N - 1) % 2
    last_top(0, early, r4 - early).start()
    last_top(0, r4 + early, r4 - early).start()

    def group(g, carry):
        lo = pl.multiple_of(g * 16, 16)
        chunked(lambda: [emit(Q, _ident, _ident, oslot) for Q in (3, 2)], lo, 16)
        for rb in range(4, 8):
            out_copy(N - 1, oslot, pl.multiple_of(rb * r8 + lo, 16), 16).start()
        return carry
    jax.lax.fori_loop(0, r8 // 16, group, 0)
    in_copy(0, (N + 1) % 3).wait()
    sp_out.wait()
    last_top(1).wait()
    last_top(0).wait()
    out_copy(0, 0, 0, half).wait()
    assert len(ids) <= m_ref.shape[0] and len(small) <= m_ref.shape[0]


def _build(x0, ws, bs, *, TM=768, R0=256, early=160, **win):
    B, D = x0.shape
    L = ws.shape[0]
    N = (B - R0) // TM
    assert R0 + N * TM == B and L >= 2 and D == 8 * LANES and x0.dtype == BF16
    assert TM % 128 == 0 and R0 % 16 == 0 and early % 16 == 0 and early < TM // 4
    return pl.pallas_call(
        functools.partial(_kernel, L=L, tm=TM, d=D, ntiles=N, r0=R0, win=dict(_WIN, **win), early=early),
        in_specs=[pl.BlockSpec(memory_space=pl.ANY)] * 3,
        out_specs=pl.BlockSpec(memory_space=pl.ANY),
        out_shape=jax.ShapeDtypeStruct((B, D), x0.dtype),
        scratch_shapes=[
            pltpu.VMEM((3, D, D + 2 * LANES), BF16),
            pltpu.VMEM((L, len(_FLAT), 2, D // 4, LANES), BF16),
            pltpu.VMEM((L, 7 * len(_DEEP), LANES, LANES), BF16),
            pltpu.VMEM((2, 4, 4, 5, 24, LANES), F32),
            pltpu.VMEM((144, TM // 4 + 8, D // 4 + LANES), F32),
            pltpu.VMEM((3, TM, D), BF16),
            pltpu.VMEM((2, TM, D), BF16),
            pltpu.VMEM((R0, D + LANES), F32),
            pltpu.VMEM((R0, D + LANES), F32),
            pltpu.VMEM((R0, D + 2 * LANES), BF16),
            pltpu.VMEM((L, D), BF16),
            pltpu.VMEM((L, 16, 2, 8, D // 4), F32),
            pltpu.VMEM((L, 8, D), F32),
            pltpu.SemaphoreType.DMA((3,)),
            pltpu.SemaphoreType.DMA((3,)),
            pltpu.SemaphoreType.DMA,
            pltpu.SemaphoreType.DMA((4,)),
        ],
        compiler_params=pltpu.CompilerParams(vmem_limit_bytes=126 * 1024 * 1024),
    )(x0, ws, bs)


@jax.jit
def pallas_standalone__dcn_v2_cross__recsys_kernel(
    x0: jax.Array,
    ws: jax.Array,
    bs: jax.Array,
):
    return _build(x0, ws, bs)
```

```python
import functools

import jax
import jax.numpy as jnp
import jax.experimental.pallas as pl
import jax.experimental.pallas.tpu as pltpu

F32 = jnp.float32
BF16 = jnp.bfloat16
LANES = 128

_T = 1.75
_EXP = (0, -1, 1, 0)
_LHS = (((1, 0),), ((1, 1),), ((1, 0), (-1, 2)), ((1, 2), (-1, 1)), ((1, 2),),
        ((1, 2), (1, 3)), ((1, 3), (-1, 2)))

_JA, _JB, _JC = (0, 1), (2, 5), (3, 6)
_PLAN = (("r", (0, 1), _JA), ("f", (0, 1), (4,)), ("r", (0, 1), _JB), ("r", (0, 1), _JC),
         ("a", (0, 1), _JA), ("a", (0, 1), _JB), ("a", (0, 1), _JC),
         None,
         ("r", (2, 3), _JB), ("a", (2, 3), _JB), ("r", (2, 3), _JC), ("a", (2, 3), _JC),
         ("r", (2, 3), _JA), ("a", (2, 3), _JA), ("f", (2, 3), (4,)), ("f", (4,), _JB + _JC + _JA + (4,)),
         None,
         ("r", (5, 6), _JA), ("f", (5, 6), (4,)), ("r", (5, 6), _JB), ("r", (5, 6), _JC),
         ("a", (5, 6), _JA), ("a", (5, 6), _JB), ("a", (5, 6), _JC),
         None)
_DEEP = [(i, j) for st in _PLAN if st and st[0] == "r" for i in st[1] for j in st[2]]
_FLAT = [(i, j) for i in range(7) for j in range(7) if (i, j) not in _DEEP]

_WIN = dict(
    q3=(((0, 1, 8), (1, 4, 6), (4, 15, 12), (15, 22, 16)), (5, 7, 15)),
    q2=(((24, 38, 16), (38, 44, 12), (44, 49, 8)), (1, 5, 9)),
    q1=(((48, 64, 8),), (1, 1, None)),
    q0=(((64, 66, 8), (66, 70, 6), (70, 79, 12), (79, 87, 24)), (1, 5, 9)),
    f3=(((0, 3, 8), (3, 5, 6), (5, 15, 12), (15, 22, 16)), (5, 9, None)),
    f2=(((24, 36, 16), (36, 44, 12), (44, 49, 8)), (1, 5, None)),
    f1=(((47, 63, 8),), (1, 1, None)),
    f0=(((64, 66, 24), (66, 70, 6), (70, 79, 12), (79, 87, 16)), (1, 9, None)),
    z1=(((38, 46, 4),), (4,)),
    z0=(((47, 63, 8),), (0,)),
    x=(((49, 62, 32),), (7, 13, 29, 21), (1, 2, 3, 4, 5)),
)
_PTRIG = (0, 0, 1, 1, 2, 2, 3, 3, 4, 4, 5, 5, 6, 6, 7, 7) + tuple(range(8, 32))


def _fwd(a, g, h, d):
    return [a + g, a - g, a + d, g + h]


def _rhs7(u, v, e, f):
    return [v - e, u - e, e + f, f - e, e + e, v, u]


class _Q:
    def __init__(self, blocks):
        self.q = list(blocks)

    def __add__(self, o):
        return _Q(a + b for a, b in zip(self.q, o.q))

    def __sub__(self, o):
        return _Q(a - b for a, b in zip(self.q, o.q))


def _scl(x, s):
    return x if s == 1.0 else x * s


def _sc(*blocks):
    return _T ** sum(_EXP[b] for b in blocks)


def _rc(Q, q):
    return 2 * (Q // 2) + q // 2, 2 * (Q % 2) + q % 2


def _ident(x):
    return x


def _after(step, t, x):
    return jnp.where(jnp.full(x.shape, step, jnp.int32) < 0, t, x)


def _kernel(x0_hbm, w_hbm, b_hbm, o_hbm,
            wbuf, s_ref, s3_ref, pb_ref, m_ref, xin, ost, sp_z, sp_x, sp_b, bvm, bt_ref, bp_ref,
            sem_w, sem_in, sem_out, sem_misc,
            *, L, tm, d, ntiles, r0, win, early):
    d4 = d // 4
    r4 = tm // 4
    r8 = tm // 8
    half = tm // 2
    N = ntiles
    dot = functools.partial(jnp.dot, preferred_element_type=F32)

    def rot(k):
        return k % 4

    def unrot(ref, k):
        r = 16 * rot(k)
        return jnp.concatenate([ref[r:], ref[:r]], axis=0) if r else ref[...]

    ids = {}
    for name in ([(n, k) for n in "UV" for k in range(7)]
                 + [("C", Q, k) for Q in range(4) for k in range(4)]
                 + [("z", Q, k) for Q in (2, 3) for k in range(4)]):
        ids[name] = len(ids)
    nzero = len(ids)

    rw = [0, r4, None]

    def rows(base):
        if isinstance(rw[0], int):
            return slice(base + rw[0], base + rw[0] + rw[1])
        return pl.ds(pl.multiple_of(base + rw[0], 8), rw[1])

    def pieces():
        if rw[2] is not None:
            return [(0, rw[1], rw[2])]
        cut = min(max(r8 - rw[0], 0), rw[1])
        return [p for p in ((0, cut, 0), (cut, rw[1], 1)) if p[1] > p[0]]

    def scaled(x, Q, q, power):
        return jnp.concatenate([jnp.concatenate(
            [_scl(x[a:b, c * LANES:(c + 1) * LANES], _sc(Q, q, 2 * rh + c) ** power) for c in range(2)],
            axis=1) for a, b, rh in pieces()], axis=0)

    def chunked(fn, lo, n):
        def body(k, c):
            for rh in range(2):
                rw[:] = [rh * r8 + lo + k * 8, 8, rh]
                fn()
            rw[:] = [0, r4, None]
            return c
        jax.lax.fori_loop(0, n // 8, body, 0)

    def loc(name, sub):
        i = ids.setdefault(name, len(ids))
        if sub is None:
            return (i, rows(0), slice(0, d4))
        return (i, slice(sub // 2 * r8, (sub // 2 + 1) * r8), slice(sub % 2 * LANES, (sub % 2 + 1) * LANES))

    def put(name, v, sub=None):
        m_ref[loc(name, sub)] = v

    def get(name, sub=None):
        return m_ref[loc(name, sub)]

    small = {}

    def putx(name, v):
        m_ref[small.setdefault(name, len(small)), 0:r8, d4:d4 + LANES] = v

    def getx(name):
        return m_ref[small[name], 0:r8, d4:d4 + LANES]

    def putq(name, q):
        for k, v in enumerate(q.q):
            put(name + (k,), v)

    def getq(name):
        return _Q(get(name + (k,)) for k in range(4))

    def sl(Q, q):
        r, c = _rc(Q, q)
        return (rows(r * r4), slice(c * d4, (c + 1) * d4))

    def new_x(l, Q, gate, gate2):
        c = []
        for k in range(7):
            t = get((("E", k), ("P", 1, k), ("U", k), ("U", k))[Q])
            if k in (1, 6):
                t = gate(t) if k == 1 else gate2(t)
            if Q > 0:
                o = get(("P", 0, k) if Q == 1 else ("V", k))
                t = t + o if Q == 2 else t - o
            c.append(t)
        f = c[1] - c[0]
        e = c[1] + c[0] + c[2] + c[3] + c[4]
        v = c[5] + c[3]
        u = c[6] - c[2]
        y = _Q([e, f, u + v + f, u - v + e])
        if l > 0:
            y = y + getq(("C", Q))
        if Q < 2 or l < L - 1:
            putq(("C", Q), y)
        if Q >= 2:
            y = y + getq(("C", 3 - Q))
        return [get(("z", Q, q)) * jnp.concatenate(
            [y.q[q][a:b] + bt_ref[l, 4 * Q + q, rh, 0:1, :] for a, b, rh in pieces()], axis=0)
            for q in range(4)]

    def emit(Q, gate, gate2, oslot):
        o = [scaled(x, Q, q, -1) for q, x in enumerate(new_x(L - 1, Q, gate, gate2))]
        for q in range(4):
            ost[(oslot,) + sl(Q, q)] = o[q].astype(ost.dtype)
        return o

    def load_z(Q, islot, gates):
        putq(("z", Q), _Q(gates[q](xin[(islot,) + sl(Q, q)].astype(F32)) for q in range(4)))

    def start(islot, gates):
        def blk(Q, q):
            x = xin[(islot,) + sl(Q, q)].astype(F32)
            return scaled(gates[Q](x) if q < 2 else x, Q, q, 1)
        a, g, h, dd = [_Q(_fwd(*[blk(Q, q) for q in range(4)])) for Q in range(4)]
        e, f = a + dd, g + h
        for i, t in enumerate([a + g, a - g, g - dd, g + dd, e, e + f, f - e]):
            putq(("A", i), t)

    def operands(Q, x):
        dn = _Q(_fwd(*x))
        if Q == 1:
            putq(("D", 1), dn)
        else:
            g = getq(("D", 1))
        if Q == 0:
            putq(("S", 0), dn + g)
            putq(("S", 1), dn - g)
        elif Q == 3:
            putq(("S", 2), g - dn)
            putq(("S", 4), getq(("S", 0)) - (g - dn))
            putq(("S", 3), g + dn)
        elif Q == 2:
            f, e = dn + g, getq(("S", 4))
            putq(("S", 5), f + e)
            putq(("S", 6), f - e)

    def stage(l, Q, gates, oslot, islot):
        if l == L - 1:
            o = emit(Q, gates[0], gates[1], oslot)
            if Q >= 2:
                load_z(Q, islot, [functools.partial(_after, islot, t) for t in o])
        else:
            x = new_x(l, Q, gates[0], gates[1])
            operands(Q, [gates[2](x[0])] + x[1:])

    def w_copy(l, slot):
        return pltpu.make_async_copy(w_hbm.at[l], wbuf.at[slot, :, pl.ds(0, d)], sem_w.at[slot])

    def in_copy(t, slot):
        return pltpu.make_async_copy(
            x0_hbm.at[pl.ds(pl.multiple_of(t * tm, 16), tm)], xin.at[slot], sem_in.at[slot])

    def out_copy(t, slot, lo=0, n=tm):
        return pltpu.make_async_copy(
            ost.at[slot, pl.ds(lo, n)],
            o_hbm.at[pl.ds(pl.multiple_of(t * tm + lo, 16), n)], sem_out)

    def last_top(Q, lo=0, n=half):
        cols = pl.ds(Q * (d // 2), d // 2)
        return pltpu.make_async_copy(
            ost.at[(N - 1) % 2, pl.ds(lo, n), cols],
            o_hbm.at[pl.ds((N - 1) * tm + lo, n), cols], sem_misc.at[2 + Q])

    sp_bv = sp_b.at[:, pl.ds(0, d)]
    sp_in = pltpu.make_async_copy(x0_hbm.at[pl.ds(N * tm, r0)], sp_bv, sem_misc.at[0])
    sp_out = pltpu.make_async_copy(sp_bv, o_hbm.at[pl.ds(N * tm, r0)], sem_misc.at[0])
    b_in = pltpu.make_async_copy(b_hbm, bvm, sem_misc.at[1])

    b_in.start()
    sp_in.start()

    def w_start(l, c):
        w_copy(l, l).start()
        return c
    jax.lax.fori_loop(0, 2, w_start, 0)

    def zero(i, c):
        m_ref[i, :r4, :d4] = jnp.zeros((r4, d4), F32)
        return c
    jax.lax.fori_loop(0, nzero, zero, 0)

    b_in.wait()
    ball = bvm[...].astype(F32)
    cum = jnp.ones((8, d), F32)
    for l in range(L):
        bl = jnp.broadcast_to(ball[l:l + 1], (8, d))
        bp_ref[l] = bl
        cum = cum + bl
        for Q in range(4):
            for q in range(4):
                c = _rc(Q, q)[1]
                for rh in range(2):
                    rw[:] = [0, 8, rh]
                    bt_ref[l, 4 * Q + q, rh] = scaled(cum[:, c * d4:(c + 1) * d4], Q, q, 1)
    rw[:] = [0, r4, None]
    sp_in.wait()
    z0 = sp_b[:, :d].astype(F32)
    sp_z[:, :d] = z0
    sp_x[:, :d] = z0

    def layer_body(l, slots):
        ws, wn, wf = slots

        @pl.when(l + 2 < L)
        def _():
            w_copy(l + 2, wf).start()

        @pl.when(l + 2 >= L)
        def _():
            in_copy(jnp.minimum(l + 2 - L, N - 1), l + 2 - L).start()
        w_copy(l, ws).wait()
        xa, xb = sp_x[:, :d // 2].astype(BF16), sp_x[:, d // 2:d].astype(BF16)
        trig, new = [], []
        for n in range(d // LANES):
            cs = slice(n * LANES, (n + 1) * LANES)
            y1 = dot(xa, wbuf[ws, :d // 2, cs]) + bp_ref[l, 0:1, cs]
            y2 = dot(xb, wbuf[ws, d // 2:, cs]) + y1
            trig += [y[k * 16:(k + 1) * 16] for y in (y1, y2) for k in range(r0 // 16)]
            new.append(sp_z[:, cs] * y2 + sp_x[:, cs])
        for n in range(d // LANES):
            sp_x[:, n * LANES:(n + 1) * LANES] = new[n]

        per = len(trig) // (LANES // 16)

        def delayed(v, n):
            v = v[0:8]
            for _ in range(n):
                v = v * 1.0001
            return jnp.concatenate([v, v], axis=0)

        chain = [delayed(sp_z[0:8, 0:LANES], 5)]

        def gated(w, st, k):
            ti = (st * per + _PTRIG[k] * per // 32) * 131 // 128 - per // 4
            return _after(l, trig[ti] if ti >= 0 else delayed(chain[-1], 3), w)

        def two_levels(st, sub):
            rh, h = divmod(sub, 2)
            rr = rh * LANES + st * 16

            def blk(Q, q):
                r, c = _rc(Q, q)
                c0 = c * d4 + h * LANES
                w = wbuf[ws, r * d4 + rr:r * d4 + rr + 16, c0:c0 + LANES].astype(F32)
                if q == 0:
                    w = gated(w, st, 4 * sub + Q)
                return _scl(w, 0.125 * _sc(Q, q, sub))
            inner = {}
            for Q in (0, 1, 3, 2):
                inner[Q] = _Q(_fwd(*[blk(Q, q) for q in range(4)]))
                chain.append(inner[Q].q[2] if Q in (0, 2) else inner[Q].q[2] + inner[0].q[2])
            wt = _fwd(*[inner[Q] for Q in range(4)])
            chain.append(wt[3].q[2])
            for a in range(4):
                for b in range(4):
                    pb_ref[st % 2, b, a, sub, 0:16, :] = wt[a].q[b]
            e4 = [x * 4.0 for x in wt[2].q]
            out = {(4, j): u for j, u in enumerate(_rhs7(*e4))}
            col = [e4[2] if a == 2 else wt[a].q[2] * 4.0 for a in range(4)]
            out.update({(i, 4): u for i, u in enumerate(_rhs7(*col))})
            for pr in _FLAT:
                r2 = (rr + 16 * rot(_FLAT.index(pr))) % d4
                s_ref[l, _FLAT.index(pr), h, r2:r2 + 16, :] = out[pr].astype(BF16)

        def third_level(st, n, j):
            par = st % 2 + (l >> (16 + n))

            def blk(a, sub):
                w = _rhs7(*[pb_ref[par, b, a, sub, 0:16, :] for b in range(4)])[j]
                if sub == 0:
                    w = jnp.concatenate([gated(w, st, 16 + 4 * n + a)[:8], w[8:]], axis=0)
                return w
            wt = [_Q(_fwd(*[blk(a, sub) for sub in range(4)])) for a in range(4)]
            for i, t in enumerate(_rhs7(*wt)):
                if i != 4:
                    for k, u in enumerate(_rhs7(*t.q)):
                        t3 = 7 * _DEEP.index((i, j)) + k
                        r2 = (st + rot(t3)) % (LANES // 16) * 16
                        s3_ref[l, t3, r2:r2 + 16, :] = u.astype(BF16)

        for st in range(LANES // 16):
            for sub in range(4):
                two_levels(st, sub)
            for n, j in enumerate((0, 1, 2, 3, 5, 6)):
                third_level(st, n, j)
        return wn, wf, ws
    jax.lax.fori_loop(0, L, layer_body, (0, 1, 2))

    sp_b[:, :d] = sp_x[:, :d].astype(BF16)
    sp_out.start()
    in_copy(0, 0).wait()
    chunked(lambda: start(0, [_ident] * 4), 0, r8)

    def tile_body(s, slots):
        cur, nxt, fre = slots
        in_copy(0, nxt).wait()
        in_copy(jnp.minimum(s + 2, N - 1), fre).start()
        oslot = s & 1
        tl = []
        hd = r8 // 4

        def gates(t0, key):
            segs, lags = win[key]
            n = r4 // 4
            when = [k for lo, hi, sp in segs for k in range((t0 + lo) * 24, (t0 + hi) * 24, sp)]
            when = [when[k * len(when) // n] * hd // 24 for k in range(n)]

            def one(lag):
                if lag is None:
                    return _ident
                parts = []
                for r in range(rw[0] // 8, (rw[0] + rw[1]) // 8):
                    cols = []
                    for c in range(2):
                        p, rr, cc = tl[min(when[2 * r + c] + lag, len(tl) - 1)]
                        cols.append(p[rr * 8:(rr + 1) * 8, cc * LANES:(cc + 1) * LANES])
                    parts.append(jnp.concatenate(cols, axis=1))
                return functools.partial(_after, s, jnp.concatenate(parts, axis=0))
            return [one(lag) for lag in lags]

        src = ["A"]

        def lhs(i, j, sub=None):
            terms = _LHS[j]
            t = get((src[0], i, terms[0][1]), sub)
            for sign, b in terms[1:]:
                t = t + get((src[0], i, b), sub) if sign > 0 else t - get((src[0], i, b), sub)
            return t

        def arrive(i, j, p, sub=None):
            if i < 4:
                put(("P", i, j), p, sub)
            elif i == 4:
                put(("E", j), p + get(("P", 0, j)) + get(("P", 1, j)) + get(("P", 2, j)) + get(("P", 3, j)))
            elif i == 5:
                put(("V", j), p + get(("P", 3, j), sub), sub)
            else:
                put(("U", j), p - get(("P", 2, j), sub), sub)

        def products(l, kind, outer, inner):
            ps = [(i, j) for i in outer for j in inner]

            def mul(pr, k, t):
                t3 = 7 * _DEEP.index(pr) + k
                return dot(t.astype(BF16), unrot(s3_ref.at[l, t3], t3))

            def close(pr, m0, m1, m4):
                f = m1 - m0
                putx(("e", pr), m1 + m0 + m4)
                if pr[0] > 4:
                    putx(("f", pr), f)
                arrive(*pr, f, 1)

            if kind == "f":
                for pr in ps:
                    k = _FLAT.index(pr)
                    w = jnp.concatenate([unrot(s_ref.at[l, k, h], k) for h in range(2)], axis=1)
                    p = dot(lhs(*pr).astype(BF16), w)
                    tl.extend((p, rr, cc) for rr in range(r4 // 8) for cc in range(2))
                    arrive(*pr, p)
            elif kind == "r":
                for r in range(3):
                    a, g, dd = (lhs(*ps[r], sub) for sub in (0, 1, 3))
                    m0, m1, m4 = mul(ps[r], 0, a + g), mul(ps[r], 1, a - g), mul(ps[r], 4, a + dd)
                    a, x = lhs(*ps[3], 0), lhs(*ps[3], 3 if r == 0 else 1)
                    mx = mul(ps[3], (4, 0, 1)[r], a - x if r == 2 else a + x)
                    tl.extend((p, rr, 0) for rr in range(r8 // 8) for p in (m0, mx))
                    close(ps[r], m0, m1, m4)
                    if r < 2:
                        putx(("m", r), mx)
                    else:
                        close(ps[3], getx(("m", 1)), mx, getx(("m", 0)))
            else:
                for pr in ps:
                    a, g, h, dd = (lhs(*pr, sub) for sub in range(4))
                    e, f = a + dd, g + h
                    m2, m3, m5, m6 = mul(pr, 2, g - dd), mul(pr, 3, g + dd), mul(pr, 5, e + f), mul(pr, 6, f - e)
                    tl.extend((p, rr, 0) for rr in range(r8 // 8) for p in (m2, m6))
                    e0 = getx(("e", pr))
                    f0 = getx(("f", pr)) if pr[0] > 4 else get(("P",) + pr, 1)
                    arrive(*pr, m2 + m3 + e0, 0)
                    arrive(*pr, (m3 - m2) + (m5 + m6) + f0, 2)
                    arrive(*pr, (m6 - m5) + e0, 3)

        for l in range(L):
            t0 = len(tl) // hd
            last = l == L - 1
            src[0] = "AS"[l > 0]

            def run(lay, Q, oslot, islot):
                stage(lay, Q, gates(t0, "qf"[lay == L - 1] + str(Q)), oslot, islot)

            def splice(k):
                if k == 0:
                    run((l - 1) % L, 3, 1 - oslot, cur)
                elif k == 1:
                    run((l - 1) % L, 2, 1 - oslot, cur)
                    if l == 0:
                        load_z(1, cur, gates(t0, "z1") * 4)
                        load_z(0, cur, gates(t0, "z0") * 4)
                    run(l, 1, oslot, nxt)
                    if last:
                        pl.when(s == N - 1)(last_top(1).start)
                elif not last:
                    run(l, 0, oslot, nxt)
                else:
                    rw[:] = [0, early, None]
                    run(l, 0, oslot, nxt)

                    @pl.when(s == N - 1)
                    def _():
                        last_top(0, 0, early).start()
                        last_top(0, r4, early).start()
                    rw[:] = [early, r4 - early, None]
                    run(l, 0, oslot, nxt)
                    rw[:] = [0, r4, None]

            k = 0
            for st in _PLAN:
                if st is None:
                    splice(k)
                    k += 1
                else:
                    products(l, *st)
            if l == 0:
                @pl.when(s > 0)
                def _():
                    out_copy(s - 1, 1 - oslot).start()
                ost[oslot, 0:8, 0:LANES] = tl[-1][0][0:8].astype(ost.dtype)

        per = len(tl) // hd // L
        segs, lags, lays = win["x"]
        win["xx"] = (tuple((lo + k * per, hi + k * per, sp) for k in lays for lo, hi, sp in segs), lags)
        start(nxt, gates(0, "xx"))

        @pl.when(s > 0)
        def _():
            out_copy(0, 0).wait()
        return nxt, fre, cur
    jax.lax.fori_loop(0, N, tile_body, (0, 1, 2))

    oslot = (N - 1) % 2
    last_top(0, early, r4 - early).start()
    last_top(0, r4 + early, r4 - early).start()

    def group(g, carry):
        lo = pl.multiple_of(g * 16, 16)
        chunked(lambda: [emit(Q, _ident, _ident, oslot) for Q in (3, 2)], lo, 16)
        for rb in range(4, 8):
            out_copy(N - 1, oslot, pl.multiple_of(rb * r8 + lo, 16), 16).start()
        return carry
    jax.lax.fori_loop(0, r8 // 16, group, 0)
    in_copy(0, (N + 1) % 3).wait()
    sp_out.wait()
    last_top(1).wait()
    last_top(0).wait()
    out_copy(0, 0, 0, half).wait()
    assert len(ids) <= m_ref.shape[0] and len(small) <= m_ref.shape[0]


def _build(x0, ws, bs, *, TM=768, R0=256, early=160, **win):
    B, D = x0.shape
    L = ws.shape[0]
    N = (B - R0) // TM
    assert R0 + N * TM == B and L >= 2 and D == 8 * LANES and x0.dtype == BF16
    assert TM % 128 == 0 and R0 % 16 == 0 and early % 16 == 0 and early < TM // 4
    return pl.pallas_call(
        functools.partial(_kernel, L=L, tm=TM, d=D, ntiles=N, r0=R0, win=dict(_WIN, **win), early=early),
        in_specs=[pl.BlockSpec(memory_space=pl.ANY)] * 3,
        out_specs=pl.BlockSpec(memory_space=pl.ANY),
        out_shape=jax.ShapeDtypeStruct((B, D), x0.dtype),
        scratch_shapes=[
            pltpu.VMEM((3, D, D + 2 * LANES), BF16),
            pltpu.VMEM((L, len(_FLAT), 2, D // 4, LANES), BF16),
            pltpu.VMEM((L, 7 * len(_DEEP), LANES, LANES), BF16),
            pltpu.VMEM((2, 4, 4, 5, 24, LANES), F32),
            pltpu.VMEM((144, TM // 4 + 8, D // 4 + LANES), F32),
            pltpu.VMEM((3, TM, D), BF16),
            pltpu.VMEM((2, TM, D), BF16),
            pltpu.VMEM((R0, D + LANES), F32),
            pltpu.VMEM((R0, D + LANES), F32),
            pltpu.VMEM((R0, D + 2 * LANES), BF16),
            pltpu.VMEM((L, D), BF16),
            pltpu.VMEM((L, 16, 2, 8, D // 4), F32),
            pltpu.VMEM((L, 8, D), F32),
            pltpu.SemaphoreType.DMA((3,)),
            pltpu.SemaphoreType.DMA((3,)),
            pltpu.SemaphoreType.DMA,
            pltpu.SemaphoreType.DMA((4,)),
        ],
        compiler_params=pltpu.CompilerParams(vmem_limit_bytes=126 * 1024 * 1024),
    )(x0, ws, bs)


@jax.jit
def pallas_standalone__dcn_v2_cross__recsys_kernel(
    x0: jax.Array,
    ws: jax.Array,
    bs: jax.Array,
):
    return _build(x0, ws, bs)
```

```python
import functools

import jax
import jax.numpy as jnp
import jax.experimental.pallas as pl
import jax.experimental.pallas.tpu as pltpu

F32 = jnp.float32
BF16 = jnp.bfloat16
LANES = 128

_T = 1.75
_EXP = (0, -1, 1, 0)
_LHS = (((1, 0),), ((1, 1),), ((1, 0), (-1, 2)), ((1, 2), (-1, 1)), ((1, 2),),
        ((1, 2), (1, 3)), ((1, 3), (-1, 2)))

_JA, _JB, _JC = (0, 1), (2, 5), (3, 6)
_PLAN = (("r", (0, 1), _JA), ("f", (0, 1), (4,)), ("r", (0, 1), _JB), ("r", (0, 1), _JC),
         ("a", (0, 1), _JA), ("a", (0, 1), _JB), ("a", (0, 1), _JC),
         None,
         ("r", (2, 3), _JB), ("a", (2, 3), _JB), ("r", (2, 3), _JC), ("a", (2, 3), _JC),
         ("r", (2, 3), _JA), ("a", (2, 3), _JA), ("f", (2, 3), (4,)), ("f", (4,), _JB + _JC + _JA + (4,)),
         None,
         ("r", (5, 6), _JA), ("f", (5, 6), (4,)), ("r", (5, 6), _JB), ("r", (5, 6), _JC),
         ("a", (5, 6), _JA), ("a", (5, 6), _JB), ("a", (5, 6), _JC),
         None)
_DEEP = [(i, j) for st in _PLAN if st and st[0] == "r" for i in st[1] for j in st[2]]
_FLAT = [(i, j) for i in range(7) for j in range(7) if (i, j) not in _DEEP]

_WIN = dict(
    q3=(((0, 1, 8), (1, 4, 6), (4, 15, 12), (15, 22, 16)), (5, 7, 15)),
    q2=(((24, 38, 16), (38, 44, 12), (44, 49, 8)), (1, 5, 9)),
    q1=(((48, 64, 8),), (1, 1, None)),
    q0=(((64, 66, 8), (66, 70, 6), (70, 79, 12), (79, 87, 24)), (1, 5, 9)),
    f3=(((0, 3, 8), (3, 5, 6), (5, 15, 12), (15, 22, 16)), (5, 9, None)),
    f2=(((24, 36, 16), (36, 44, 12), (44, 49, 8)), (1, 5, None)),
    f1=(((47, 63, 8),), (1, 1, None)),
    f0=(((64, 66, 24), (66, 70, 6), (70, 79, 12), (79, 87, 16)), (1, 9, None)),
    z1=(((38, 46, 4),), (4,)),
    z0=(((47, 63, 8),), (0,)),
    x=(((49, 62, 32),), (7, 13, 29, 21)),
)
_PTRIG = (0, 0, -1, 0, 1, 1, 2, 3, 4, 4, 4, 5, 7, 6, 6, 7) + tuple(range(8, 24)) + (25,) + tuple(range(25, 32))


def _fwd(a, g, h, d):
    return [a + g, a - g, a + d, g + h]


def _rhs7(u, v, e, f):
    return [v - e, u - e, e + f, f - e, e + e, v, u]


class _Q:
    def __init__(self, blocks):
        self.q = list(blocks)

    def __add__(self, o):
        return _Q(a + b for a, b in zip(self.q, o.q))

    def __sub__(self, o):
        return _Q(a - b for a, b in zip(self.q, o.q))


def _scl(x, s):
    return x if s == 1.0 else x * s


def _sc(*blocks):
    return _T ** sum(_EXP[b] for b in blocks)


def _rc(Q, q):
    return 2 * (Q // 2) + q // 2, 2 * (Q % 2) + q % 2


def _ident(x):
    return x


def _after(step, t, x):
    return jnp.where(jnp.full(x.shape, step, jnp.int32) < 0, t, x)


def _kernel(x0_hbm, w_hbm, b_hbm, o_hbm,
            wbuf, s_ref, s3_ref, pb_ref, m_ref, xin, ost, sp_z, sp_x, sp_b, bvm, bt_ref, bp_ref,
            sem_w, sem_in, sem_out, sem_misc,
            *, L, tm, d, ntiles, r0, win, early):
    d4 = d // 4
    r4 = tm // 4
    r8 = tm // 8
    half = tm // 2
    N = ntiles
    dot = functools.partial(jnp.dot, preferred_element_type=F32)

    def rot(k):
        return k % 4

    def unrot(ref, k):
        r = 16 * rot(k)
        return jnp.concatenate([ref[r:], ref[:r]], axis=0) if r else ref[...]

    ids = {}
    for name in ([(n, k) for n in "UV" for k in range(7)]
                 + [("C", Q, k) for Q in range(4) for k in range(4)]
                 + [("z", Q, k) for Q in (2, 3) for k in range(4)]):
        ids[name] = len(ids)
    nzero = len(ids)

    rw = [0, r4, None]

    def rows(base):
        if isinstance(rw[0], int):
            return slice(base + rw[0], base + rw[0] + rw[1])
        return pl.ds(pl.multiple_of(base + rw[0], 8), rw[1])

    def pieces():
        if rw[2] is not None:
            return [(0, rw[1], rw[2])]
        cut = min(max(r8 - rw[0], 0), rw[1])
        return [p for p in ((0, cut, 0), (cut, rw[1], 1)) if p[1] > p[0]]

    def scaled(x, Q, q, power):
        return jnp.concatenate([jnp.concatenate(
            [_scl(x[a:b, c * LANES:(c + 1) * LANES], _sc(Q, q, 2 * rh + c) ** power) for c in range(2)],
            axis=1) for a, b, rh in pieces()], axis=0)

    def chunked(fn, lo, n):
        def body(k, c):
            for rh in range(2):
                rw[:] = [rh * r8 + lo + k * 8, 8, rh]
                fn()
            rw[:] = [0, r4, None]
            return c
        jax.lax.fori_loop(0, n // 8, body, 0)

    def loc(name, sub):
        i = ids.setdefault(name, len(ids))
        if sub is None:
            return (i, rows(0), slice(0, d4))
        return (i, slice(sub // 2 * r8, (sub // 2 + 1) * r8), slice(sub % 2 * LANES, (sub % 2 + 1) * LANES))

    def put(name, v, sub=None):
        m_ref[loc(name, sub)] = v

    def get(name, sub=None):
        return m_ref[loc(name, sub)]

    small = {}

    def putx(name, v):
        m_ref[small.setdefault(name, len(small)), 0:r8, d4:d4 + LANES] = v

    def getx(name):
        return m_ref[small[name], 0:r8, d4:d4 + LANES]

    def putq(name, q):
        for k, v in enumerate(q.q):
            put(name + (k,), v)

    def getq(name):
        return _Q(get(name + (k,)) for k in range(4))

    def sl(Q, q):
        r, c = _rc(Q, q)
        return (rows(r * r4), slice(c * d4, (c + 1) * d4))

    def new_x(l, Q, gate, gate2):
        c = []
        for k in range(7):
            t = get((("E", k), ("P", 1, k), ("U", k), ("U", k))[Q])
            if k in (1, 6):
                t = gate(t) if k == 1 else gate2(t)
            if Q > 0:
                o = get(("P", 0, k) if Q == 1 else ("V", k))
                t = t + o if Q == 2 else t - o
            c.append(t)
        f = c[1] - c[0]
        e = c[1] + c[0] + c[2] + c[3] + c[4]
        v = c[5] + c[3]
        u = c[6] - c[2]
        y = _Q([e, f, u + v + f, u - v + e])
        if l > 0:
            y = y + getq(("C", Q))
        if Q < 2 or l < L - 1:
            putq(("C", Q), y)
        if Q >= 2:
            y = y + getq(("C", 3 - Q))
        return [get(("z", Q, q)) * jnp.concatenate(
            [y.q[q][a:b] + bt_ref[l, 4 * Q + q, rh, 0:1, :] for a, b, rh in pieces()], axis=0)
            for q in range(4)]

    def emit(Q, gate, gate2, oslot):
        o = [scaled(x, Q, q, -1) for q, x in enumerate(new_x(L - 1, Q, gate, gate2))]
        for q in range(4):
            ost[(oslot,) + sl(Q, q)] = o[q].astype(ost.dtype)
        return o

    def load_z(Q, islot, gates):
        putq(("z", Q), _Q(gates[q](xin[(islot,) + sl(Q, q)].astype(F32)) for q in range(4)))

    def start(islot, gates):
        def blk(Q, q):
            x = xin[(islot,) + sl(Q, q)].astype(F32)
            return scaled(gates[Q](x) if q < 2 else x, Q, q, 1)
        a, g, h, dd = [_Q(_fwd(*[blk(Q, q) for q in range(4)])) for Q in range(4)]
        e, f = a + dd, g + h
        for i, t in enumerate([a + g, a - g, g - dd, g + dd, e, e + f, f - e]):
            putq(("A", i), t)

    def operands(Q, x):
        dn = _Q(_fwd(*x))
        if Q == 1:
            putq(("D", 1), dn)
        else:
            g = getq(("D", 1))
        if Q == 0:
            putq(("S", 0), dn + g)
            putq(("S", 1), dn - g)
        elif Q == 3:
            putq(("S", 2), g - dn)
            putq(("S", 4), getq(("S", 0)) - (g - dn))
            putq(("S", 3), g + dn)
        elif Q == 2:
            f, e = dn + g, getq(("S", 4))
            putq(("S", 5), f + e)
            putq(("S", 6), f - e)

    def stage(l, Q, gates, oslot, islot):
        if l == L - 1:
            o = emit(Q, gates[0], gates[1], oslot)
            if Q >= 2:
                load_z(Q, islot, [functools.partial(_after, islot, t) for t in o])
        else:
            x = new_x(l, Q, gates[0], gates[1])
            operands(Q, [gates[2](x[0])] + x[1:])

    def w_copy(l, slot):
        return pltpu.make_async_copy(w_hbm.at[l], wbuf.at[slot, :, pl.ds(0, d)], sem_w.at[slot])

    def in_copy(t, slot):
        return pltpu.make_async_copy(
            x0_hbm.at[pl.ds(pl.multiple_of(t * tm, 16), tm)], xin.at[slot], sem_in.at[slot])

    def out_copy(t, slot, lo=0, n=tm):
        return pltpu.make_async_copy(
            ost.at[slot, pl.ds(lo, n)],
            o_hbm.at[pl.ds(pl.multiple_of(t * tm + lo, 16), n)], sem_out)

    def last_top(Q, lo=0, n=half):
        cols = pl.ds(Q * (d // 2), d // 2)
        return pltpu.make_async_copy(
            ost.at[(N - 1) % 2, pl.ds(lo, n), cols],
            o_hbm.at[pl.ds((N - 1) * tm + lo, n), cols], sem_misc.at[2 + Q])

    sp_bv = sp_b.at[:, pl.ds(0, d)]
    sp_in = pltpu.make_async_copy(x0_hbm.at[pl.ds(N * tm, r0)], sp_bv, sem_misc.at[0])
    sp_out = pltpu.make_async_copy(sp_bv, o_hbm.at[pl.ds(N * tm, r0)], sem_misc.at[0])
    b_in = pltpu.make_async_copy(b_hbm, bvm, sem_misc.at[1])

    b_in.start()
    sp_in.start()

    def w_start(l, c):
        w_copy(l, l).start()
        return c
    jax.lax.fori_loop(0, 2, w_start, 0)

    def zero(i, c):
        m_ref[i, :r4, :d4] = jnp.zeros((r4, d4), F32)
        return c
    jax.lax.fori_loop(0, nzero, zero, 0)

    b_in.wait()
    ball = bvm[...].astype(F32)
    cum = jnp.ones((8, d), F32)
    for l in range(L):
        bl = jnp.broadcast_to(ball[l:l + 1], (8, d))
        bp_ref[l] = bl
        cum = cum + bl
        for Q in range(4):
            for q in range(4):
                c = _rc(Q, q)[1]
                for rh in range(2):
                    rw[:] = [0, 8, rh]
                    bt_ref[l, 4 * Q + q, rh] = scaled(cum[:, c * d4:(c + 1) * d4], Q, q, 1)
    rw[:] = [0, r4, None]
    sp_in.wait()
    z0 = sp_b[:, :d].astype(F32)
    sp_z[:, :d] = z0
    sp_x[:, :d] = z0

    def layer_body(l, slots):
        ws, wn, wf = slots

        @pl.when(l + 2 < L)
        def _():
            w_copy(l + 2, wf).start()

        @pl.when(l + 2 >= L)
        def _():
            in_copy(jnp.minimum(l + 2 - L, N - 1), l + 2 - L).start()
        w_copy(l, ws).wait()
        xa, xb = sp_x[:, :d // 2].astype(BF16), sp_x[:, d // 2:d].astype(BF16)
        trig, new = [], []
        for n in range(d // LANES):
            cs = slice(n * LANES, (n + 1) * LANES)
            y1 = dot(xa, wbuf[ws, :d // 2, cs]) + bp_ref[l, 0:1, cs]
            y2 = dot(xb, wbuf[ws, d // 2:, cs]) + y1
            trig += [y[k * 16:(k + 1) * 16] for y in (y1, y2) for k in range(r0 // 16)]
            new.append(sp_z[:, cs] * y2 + sp_x[:, cs])
        for n in range(d // LANES):
            sp_x[:, n * LANES:(n + 1) * LANES] = new[n]

        per = len(trig) // (LANES // 16)

        def delayed(v, n):
            v = v[0:8]
            for _ in range(n):
                v = v * 1.0001
            return jnp.concatenate([v, v], axis=0)

        chain = [delayed(sp_z[0:8, 0:LANES], 4)]

        def gated(w, st, k):
            ti = (st * per + _PTRIG[k] * per // 32) * 33 // 32 - per // 4
            return _after(l, trig[ti] if ti >= 0 else delayed(chain[-1], 3), w)

        def two_levels(st, sub):
            rh, h = divmod(sub, 2)
            rr = rh * LANES + st * 16

            def blk(Q, q):
                r, c = _rc(Q, q)
                c0 = c * d4 + h * LANES
                w = wbuf[ws, r * d4 + rr:r * d4 + rr + 16, c0:c0 + LANES].astype(F32)
                if q == 0:
                    w = gated(w, st, 4 * sub + Q)
                return _scl(w, 0.125 * _sc(Q, q, sub))
            inner = {}
            for Q in (0, 1, 3, 2):
                inner[Q] = _Q(_fwd(*[blk(Q, q) for q in range(4)]))
                chain.append(inner[Q].q[2] if Q in (0, 2) else inner[Q].q[2] + inner[0].q[2])
            wt = _fwd(*[inner[Q] for Q in range(4)])
            chain.append(wt[3].q[2])
            for a in range(4):
                for b in range(4):
                    pb_ref[st % 2, b, a, sub, 0:16, :] = wt[a].q[b]
            e4 = [x * 4.0 for x in wt[2].q]
            out = {(4, j): u for j, u in enumerate(_rhs7(*e4))}
            col = [e4[2] if a == 2 else wt[a].q[2] * 4.0 for a in range(4)]
            out.update({(i, 4): u for i, u in enumerate(_rhs7(*col))})
            for pr in _FLAT:
                r2 = (rr + 16 * rot(_FLAT.index(pr))) % d4
                s_ref[l, _FLAT.index(pr), h, r2:r2 + 16, :] = out[pr].astype(BF16)

        def third_level(st, n, j):
            par = st % 2 + (l >> (16 + n))

            def blk(a, sub):
                w = _rhs7(*[pb_ref[par, b, a, sub, 0:16, :] for b in range(4)])[j]
                if sub == 0:
                    w = jnp.concatenate([gated(w, st, 16 + 4 * n + a)[:8], w[8:]], axis=0)
                return w
            wt = [_Q(_fwd(*[blk(a, sub) for sub in range(4)])) for a in range(4)]
            for i, t in enumerate(_rhs7(*wt)):
                if i != 4:
                    for k, u in enumerate(_rhs7(*t.q)):
                        t3 = 7 * _DEEP.index((i, j)) + k
                        r2 = (st + rot(t3)) % (LANES // 16) * 16
                        s3_ref[l, t3, r2:r2 + 16, :] = u.astype(BF16)

        for st in range(LANES // 16):
            for sub in range(4):
                two_levels(st, sub)
            for n, j in enumerate((0, 1, 2, 3, 5, 6)):
                third_level(st, n, j)
        return wn, wf, ws
    jax.lax.fori_loop(0, L, layer_body, (0, 1, 2))

    sp_b[:, :d] = sp_x[:, :d].astype(BF16)
    sp_out.start()
    in_copy(0, 0).wait()
    chunked(lambda: start(0, [_ident] * 4), 0, r8)

    def tile_body(s, slots):
        cur, nxt, fre = slots
        in_copy(0, nxt).wait()
        in_copy(jnp.minimum(s + 2, N - 1), fre).start()
        oslot = s & 1
        tl = []
        hd = r8 // 4

        def gates(t0, key):
            segs, lags = win[key]
            n = r4 // 4
            when = [k for lo, hi, sp in segs for k in range((t0 + lo) * 24, (t0 + hi) * 24, sp)]
            when = [when[k * len(when) // n] * hd // 24 for k in range(n)]

            def one(lag):
                if lag is None:
                    return _ident
                parts = []
                for r in range(rw[0] // 8, (rw[0] + rw[1]) // 8):
                    cols = []
                    for c in range(2):
                        p, rr, cc = tl[min(when[2 * r + c] + lag, len(tl) - 1)]
                        cols.append(p[rr * 8:(rr + 1) * 8, cc * LANES:(cc + 1) * LANES])
                    parts.append(jnp.concatenate(cols, axis=1))
                return functools.partial(_after, s, jnp.concatenate(parts, axis=0))
            return [one(lag) for lag in lags]

        src = ["A"]

        def lhs(i, j, sub=None):
            terms = _LHS[j]
            t = get((src[0], i, terms[0][1]), sub)
            for sign, b in terms[1:]:
                t = t + get((src[0], i, b), sub) if sign > 0 else t - get((src[0], i, b), sub)
            return t

        def arrive(i, j, p, sub=None):
            if i < 4:
                put(("P", i, j), p, sub)
            elif i == 4:
                put(("E", j), p + get(("P", 0, j)) + get(("P", 1, j)) + get(("P", 2, j)) + get(("P", 3, j)))
            elif i == 5:
                put(("V", j), p + get(("P", 3, j), sub), sub)
            else:
                put(("U", j), p - get(("P", 2, j), sub), sub)

        def products(l, kind, outer, inner):
            ps = [(i, j) for i in outer for j in inner]

            def mul(pr, k, t):
                t3 = 7 * _DEEP.index(pr) + k
                return dot(t.astype(BF16), unrot(s3_ref.at[l, t3], t3))

            def close(pr, m0, m1, m4):
                f = m1 - m0
                putx(("e", pr), m1 + m0 + m4)
                if pr[0] > 4:
                    putx(("f", pr), f)
                arrive(*pr, f, 1)

            if kind == "f":
                for pr in ps:
                    k = _FLAT.index(pr)
                    w = jnp.concatenate([unrot(s_ref.at[l, k, h], k) for h in range(2)], axis=1)
                    p = dot(lhs(*pr).astype(BF16), w)
                    tl.extend((p, rr, cc) for rr in range(r4 // 8) for cc in range(2))
                    arrive(*pr, p)
            elif kind == "r":
                for r in range(3):
                    a, g, dd = (lhs(*ps[r], sub) for sub in (0, 1, 3))
                    m0, m1, m4 = mul(ps[r], 0, a + g), mul(ps[r], 1, a - g), mul(ps[r], 4, a + dd)
                    a, x = lhs(*ps[3], 0), lhs(*ps[3], 3 if r == 0 else 1)
                    mx = mul(ps[3], (4, 0, 1)[r], a - x if r == 2 else a + x)
                    tl.extend((p, rr, 0) for rr in range(r8 // 8) for p in (m0, mx))
                    close(ps[r], m0, m1, m4)
                    if r < 2:
                        putx(("m", r), mx)
                    else:
                        close(ps[3], getx(("m", 1)), mx, getx(("m", 0)))
            else:
                for pr in ps:
                    a, g, h, dd = (lhs(*pr, sub) for sub in range(4))
                    e, f = a + dd, g + h
                    m2, m3, m5, m6 = mul(pr, 2, g - dd), mul(pr, 3, g + dd), mul(pr, 5, e + f), mul(pr, 6, f - e)
                    tl.extend((p, rr, 0) for rr in range(r8 // 8) for p in (m2, m6))
                    e0 = getx(("e", pr))
                    f0 = getx(("f", pr)) if pr[0] > 4 else get(("P",) + pr, 1)
                    arrive(*pr, m2 + m3 + e0, 0)
                    arrive(*pr, (m3 - m2) + (m5 + m6) + f0, 2)
                    arrive(*pr, (m6 - m5) + e0, 3)

        for l in range(L):
            t0 = len(tl) // hd
            last = l == L - 1
            src[0] = "AS"[l > 0]

            def run(lay, Q, oslot, islot):
                stage(lay, Q, gates(t0, "qf"[lay == L - 1] + str(Q)), oslot, islot)

            def splice(k):
                if k == 0:
                    run((l - 1) % L, 3, 1 - oslot, cur)
                elif k == 1:
                    run((l - 1) % L, 2, 1 - oslot, cur)
                    if l == 0:
                        load_z(1, cur, gates(t0, "z1") * 4)
                        load_z(0, cur, gates(t0, "z0") * 4)
                    run(l, 1, oslot, nxt)
                    if last:
                        pl.when(s == N - 1)(last_top(1).start)
                elif not last:
                    run(l, 0, oslot, nxt)
                else:
                    rw[:] = [0, early, None]
                    run(l, 0, oslot, nxt)

                    @pl.when(s == N - 1)
                    def _():
                        last_top(0, 0, early).start()
                        last_top(0, r4, early).start()
                    rw[:] = [early, r4 - early, None]
                    run(l, 0, oslot, nxt)
                    rw[:] = [0, r4, None]

            k = 0
            for st in _PLAN:
                if st is None:
                    splice(k)
                    k += 1
                else:
                    products(l, *st)
            if l == 0:
                @pl.when(s > 0)
                def _():
                    out_copy(s - 1, 1 - oslot).start()
                ost[oslot, 0:8, 0:LANES] = tl[-1][0][0:8].astype(ost.dtype)

        per = len(tl) // hd // L
        segs, lags = win["x"]
        win["xx"] = (tuple((lo + k * per, hi + k * per, sp) for k in range(1, L) for lo, hi, sp in segs), lags)
        start(nxt, gates(0, "xx"))

        @pl.when(s > 0)
        def _():
            out_copy(0, 0).wait()
        return nxt, fre, cur
    jax.lax.fori_loop(0, N, tile_body, (0, 1, 2))

    oslot = (N - 1) % 2
    last_top(0, early, r4 - early).start()
    last_top(0, r4 + early, r4 - early).start()

    for lo in range(0, r8, 16):
        chunked(lambda: [emit(Q, _ident, _ident, oslot) for Q in (3, 2)], lo, 16)
        for rb in range(4, 8):
            out_copy(N - 1, oslot, rb * r8 + lo, 16).start()
    in_copy(0, (N + 1) % 3).wait()
    sp_out.wait()
    last_top(1).wait()
    last_top(0).wait()
    out_copy(0, 0, 0, half).wait()
    assert len(ids) <= m_ref.shape[0] and len(small) <= m_ref.shape[0]


def _build(x0, ws, bs, *, TM=768, R0=256, early=160, **win):
    B, D = x0.shape
    L = ws.shape[0]
    N = (B - R0) // TM
    assert R0 + N * TM == B and L >= 2 and D == 8 * LANES and x0.dtype == BF16
    assert TM % 128 == 0 and R0 % 16 == 0 and early % 16 == 0 and early < TM // 4
    return pl.pallas_call(
        functools.partial(_kernel, L=L, tm=TM, d=D, ntiles=N, r0=R0, win=dict(_WIN, **win), early=early),
        in_specs=[pl.BlockSpec(memory_space=pl.ANY)] * 3,
        out_specs=pl.BlockSpec(memory_space=pl.ANY),
        out_shape=jax.ShapeDtypeStruct((B, D), x0.dtype),
        scratch_shapes=[
            pltpu.VMEM((3, D, D + 2 * LANES), BF16),
            pltpu.VMEM((L, len(_FLAT), 2, D // 4, LANES), BF16),
            pltpu.VMEM((L, 7 * len(_DEEP), LANES, LANES), BF16),
            pltpu.VMEM((2, 4, 4, 5, 24, LANES), F32),
            pltpu.VMEM((144, TM // 4 + 8, D // 4 + LANES), F32),
            pltpu.VMEM((3, TM, D), BF16),
            pltpu.VMEM((2, TM, D), BF16),
            pltpu.VMEM((R0, D + LANES), F32),
            pltpu.VMEM((R0, D + LANES), F32),
            pltpu.VMEM((R0, D + 2 * LANES), BF16),
            pltpu.VMEM((L, D), BF16),
            pltpu.VMEM((L, 16, 2, 8, D // 4), F32),
            pltpu.VMEM((L, 8, D), F32),
            pltpu.SemaphoreType.DMA((3,)),
            pltpu.SemaphoreType.DMA((3,)),
            pltpu.SemaphoreType.DMA,
            pltpu.SemaphoreType.DMA((4,)),
        ],
        compiler_params=pltpu.CompilerParams(vmem_limit_bytes=126 * 1024 * 1024),
    )(x0, ws, bs)


@jax.jit
def pallas_standalone__dcn_v2_cross__recsys_kernel(
    x0: jax.Array,
    ws: jax.Array,
    bs: jax.Array,
):
    return _build(x0, ws, bs)
```
